```python
import jax
import jax.numpy as jnp

def _softmax(x, axis=-1):
    return jax.nn.softmax(x, axis=axis)

def _gelu(x):
    return jax.nn.gelu(x, approximate=True)

def _silu(x):
    return jax.nn.silu(x)

def _sigmoid(x):
    return jax.nn.sigmoid(x)

def _layernorm(x, axis=-1, eps=1e-05):
    m = jnp.mean(x, axis=axis, keepdims=True)
    v = jnp.var(x, axis=axis, keepdims=True)
    return (x - m) / jnp.sqrt(v + eps)

def _scatter_add(tgt, idx, src, axis=0):
    return tgt.at[idx].add(src)

def _segment_sum(src, seg, n):
    return jax.ops.segment_sum(src, seg, n)

class _Rng:

    def __init__(self, key):
        self._k = key

    def _next(self):
        self._k, sub = jax.random.split(self._k)
        return sub

    def normal(self, shape):
        return jax.random.normal(self._next(), shape, dtype=jnp.bfloat16)

    def randint(self, lo, hi, shape):
        return jax.random.randint(self._next(), shape, lo, hi, dtype=jnp.int32)

    def uniform(self, shape, lo=0.0, hi=1.0):
        return jax.random.uniform(self._next(), shape, jnp.bfloat16, lo, hi)

    def permutation(self, n):
        return jax.random.permutation(self._next(), n)
kernel_name = 'interleave_layers__memory_aug_recurrent_mem_tr__ssm_conv_h3__prompt'

def setup_inputs():
    _rng = _Rng(jax.random.key(int.from_bytes(__import__("os").urandom(4), "little")))
    _w = lambda a: (lambda t: t.astype(jnp.bfloat16) if jnp.issubdtype(t.dtype, jnp.floating) else t)(jnp.asarray(a))

    def _A_setup():
        B, S, Dm = (1, 2048, 640)
        H, Dh = (32, 128)
        M, seg = (8, 32)
        seg = min(seg, S)
        S = S // seg * seg
        return {'x': _w((lambda *s: _rng.normal(s) * 0.05)(B, S, Dm)), 'mem0': _w((lambda *s: _rng.normal(s) * 0.05)(B, M, Dm)), 'Wq': _w((lambda *s: _rng.normal(s) * 0.05)(Dm, H, Dh) * Dm ** (-0.5)), 'Wk': _w((lambda *s: _rng.normal(s) * 0.05)(Dm, H, Dh) * Dm ** (-0.5)), 'Wv': _w((lambda *s: _rng.normal(s) * 0.05)(Dm, H, Dh) * Dm ** (-0.5)), 'Wo': _w((lambda *s: _rng.normal(s) * 0.05)(H, Dh, Dm) * (H * Dh) ** (-0.5)), 'seg_len': seg}
    _A_in = _A_setup()

    def _B_setup():
        B, S, D = (1, 2048, 640)
        ks = 4
        return {'q': _w((lambda *s: _rng.normal(s) * 0.05)(B, S, D)), 'k': _w((lambda *s: _rng.normal(s) * 0.05)(B, S, D)), 'v': _w((lambda *s: _rng.normal(s) * 0.05)(B, S, D)), 'shift_k': _w((lambda *s: _rng.normal(s) * 0.05)(D, ks) * 0.5), 'ssm_k': _w((lambda *s: _rng.normal(s) * 0.05)(D, S) * (1.0 / S ** 0.5)), 'ssm_D': _w((lambda *s: _rng.normal(s) * 0.05)(D))}
    _B_in = _B_setup()
    return {'A_x': _A_in['x'], 'A_mem0': _A_in['mem0'], 'A_Wq': _A_in['Wq'], 'A_Wk': _A_in['Wk'], 'A_Wv': _A_in['Wv'], 'A_Wo': _A_in['Wo'], 'A_seg_len': _A_in['seg_len'], 'B_q': _B_in['q'], 'B_k': _B_in['k'], 'B_v': _B_in['v'], 'B_shift_k': _B_in['shift_k'], 'B_ssm_k': _B_in['ssm_k'], 'B_ssm_D': _B_in['ssm_D']}

def reference(A_x, A_mem0, A_Wq, A_Wk, A_Wv, A_Wo, A_seg_len, B_q, B_k, B_v, B_shift_k, B_ssm_k, B_ssm_D):

    def _A_ref(x, mem0, Wq, Wk, Wv, Wo, seg_len):
        B, S, Dm = x.shape
        H, Dh = (Wq.shape[1], Wq.shape[2])
        M = mem0.shape[1]
        scale = Dh ** (-0.5)
        n_seg = S // seg_len
        L = M + seg_len
        idx = jnp.arange(L)
        mask = (idx[:, None] < M) | (idx[:, None] >= idx[None, :])
        mem = mem0
        outs = []
        for s in range(n_seg):
            xs = x[:, s * seg_len:(s + 1) * seg_len, :].copy()
            h = jnp.concatenate([mem, xs], axis=1)
            q = jnp.einsum('btd,dhe->bhte', h, Wq)
            k = jnp.einsum('btd,dhe->bhte', h, Wk)
            v = jnp.einsum('btd,dhe->bhte', h, Wv)
            scores = jnp.einsum('bhqe,bhke->bhqk', q, k) * scale
            scores = jnp.where(mask[None, None], scores, -1000000000.0)
            p = _softmax(scores, axis=-1)
            o = jnp.einsum('bhqk,bhke->bhqe', p, v)
            o = jnp.einsum('bhte,hed->btd', o, Wo)
            mem = o[:, :M, :].copy()
            outs.append(o[:, M:, :])
        return jnp.concatenate(outs, axis=1)

    def _B_ref(q, k, v, shift_k, ssm_k, ssm_D):
        B, S, D = q.shape
        ks = shift_k.shape[-1]
        k_pad = jnp.pad(k, ((0, 0), (ks - 1, 0), (0, 0)))
        k_shift = jnp.zeros_like(k)
        for t in range(ks):
            k_shift = k_shift + k_pad[:, t:t + S, :] * shift_k[:, ks - 1 - t][None, None, :]
        kv = k_shift * v
        L = 2 * S
        kv_pad = jnp.pad(kv, ((0, 0), (0, S), (0, 0)))
        kf_pad = jnp.pad(ssm_k, ((0, 0), (0, S)))
        kv_f = (lambda x, axes=(-2, -1): jnp.fft.rfft2(x.astype(jnp.float32), axes=axes))(kv_pad[:, None, :, :], axes=(1, 2))
        kf_f = (lambda x, axes=(-2, -1): jnp.fft.rfft2(x.astype(jnp.float32), axes=axes))(kf_pad[:, None, :], axes=(1, 2))
        kf_f = (lambda x, *d: x.transpose(*d))(kf_f, 1, 2, 0)
        y_f = kv_f * kf_f[None, :, :, :]
        y = (lambda x, s, axes=(-2, -1): jnp.fft.irfft2(x, s=s, axes=axes).astype(jnp.bfloat16))(y_f, (1, L), axes=(1, 2))[:, 0, :S, :]
        y = y + kv * ssm_D[None, None, :]
        return q * y
    x = A_x
    x = x + _A_ref(_layernorm(x, axis=-1), A_mem0, A_Wq, A_Wk, A_Wv, A_Wo, A_seg_len)
    x = x + _B_ref(_layernorm(x, axis=-1), B_k, B_v, B_shift_k, B_ssm_k, B_ssm_D)
    x = x + _A_ref(_layernorm(x, axis=-1), A_mem0, A_Wq, A_Wk, A_Wv, A_Wo, A_seg_len)
    x = x + _B_ref(_layernorm(x, axis=-1), B_k, B_v, B_shift_k, B_ssm_k, B_ssm_D)
    return x
```

```python
import functools

import jax
import jax.numpy as jnp
import numpy as np
from jax import lax
from jax.experimental import pallas as pl
from jax.experimental.pallas import tpu as pltpu

F32, BF16, U32 = jnp.float32, jnp.bfloat16, jnp.uint32

LOG2E = 1.4426950408889634
LN_EPS = 1e-5
CH = 128
LAG = 2
KPAD = 16


def _np_bf16(a):
    return np.asarray(a, dtype=np.float32).astype(BF16)


def _dft_mats():
    n2 = 2 * CH
    karr = np.concatenate([np.arange(0, CH, 2), np.arange(1, CH, 2)])
    n = np.arange(CH)
    th = 2.0 * np.pi * n[None, :] * (karr[:, None] + 0.5) / n2
    fa = np.concatenate([np.cos(th), -np.sin(th)], axis=0)
    fi = np.concatenate([np.cos(th).T, -np.sin(th).T], axis=1) * (2.0 / n2)
    return _np_bf16(fa), _np_bf16(fi)


def _attn_bias(m, seg):
    rows = 2 * (m + seg)
    idx = np.arange(128)

    def stream(i):
        return np.where(i < m, 0, np.where(i < 2 * m, 1, np.where(
            i < 2 * m + seg, 0, np.where(i < rows, 1, 2))))

    def ismem(i):
        return i < 2 * m

    def pos(i):
        return np.where(i < 2 * m + seg, i - 2 * m, i - 2 * m - seg)

    r, c = idx[:rows, None], idx[None, :]
    same = stream(r) == stream(c)
    keep = ismem(r) | ismem(c) | (pos(r) >= pos(c))
    fill = np.where(same, -1e9 * LOG2E, -1e30)
    return np.where(same & keep, 0.0, fill).astype(np.float32)


def _ln(x):
    m = jnp.mean(x, axis=-1, keepdims=True)
    xc = x - m
    v = jnp.mean(xc * xc, axis=-1, keepdims=True)
    return xc * lax.rsqrt(v + LN_EPS)


def _pack16(x):
    return pltpu.bitcast(x.astype(BF16), U32)


def _build(S, Dm, H, Dh, M, seg, KS, cfg):
    assert Dh == 128 and Dm % 128 == 0 and S % CH == 0 and H % 16 == 0
    assert M == 8 and seg == 32 and KS <= 8
    NSEG = S // seg
    NCH = S // CH
    NT = Dm // 128
    R = 2 * (M + seg)
    HP = H // 2
    qk_scale = float(Dh ** -0.5) * LOG2E
    lS, lP, lW = cfg.get("lS", 1), cfg.get("lP", 2), cfg.get("lW", 8)
    order = cfg.get("order", "qSkPvW")
    extras = cfg.get("extras", (3, 11, 19))
    nsteps = NSEG + LAG

    def kernel(x_hbm, mem0_hbm, wq_hbm, wk_hbm, wv_hbm, wo_hbm, k_hbm, v_hbm, sh_hbm, h_hbm,
               d_hbm, fa_hbm, fi_hbm, bias_hbm, o_hbm,
               wqkv, wstage, wo, x0, kb, vb, hb, ub, Ub, Gb, Ap, yb,
               hbuf, acc, x2buf, ox, ob, fa, fi, bias, mem0, shv, dv,
               sem_c, sem_k, sem_v, sem_h, sem_w, sem_o, sem_x, sem_out):
        c_fa = pltpu.make_async_copy(fa_hbm, fa, sem_c.at[0])
        c_sh = pltpu.make_async_copy(sh_hbm, shv, sem_c.at[1])
        c_fi = pltpu.make_async_copy(fi_hbm, fi, sem_c.at[2])
        c_d = pltpu.make_async_copy(d_hbm, dv, sem_c.at[3])
        c_bias = pltpu.make_async_copy(bias_hbm, bias, sem_c.at[4])
        c_mem0 = pltpu.make_async_copy(mem0_hbm, mem0, sem_c.at[5])

        def cp_k(j):
            return pltpu.make_async_copy(
                k_hbm.at[pl.ds(j * CH, CH)], kb.at[pl.ds(KPAD + j * CH, CH)], sem_k.at[j])

        def cp_v(j):
            return pltpu.make_async_copy(
                v_hbm.at[pl.ds(j * CH, CH)], vb.at[pl.ds(j * CH, CH)], sem_v.at[j])

        def cp_h(j):
            return pltpu.make_async_copy(
                h_hbm.at[:, pl.ds(j * CH, CH)], hb.at[j], sem_h.at[j])

        w32 = [w.bitcast(U32) for w in (wq_hbm, wk_hbm, wv_hbm)]

        def cp_w(j, s):
            return pltpu.make_async_copy(w32[j].at[:, s, :], wstage.at[j, s], sem_w.at[j, s])

        wo32 = wo_hbm.bitcast(U32)
        NWO = 4
        c_wo = [pltpu.make_async_copy(wo32.at[pl.ds(i * (H // NWO), H // NWO)],
                                      wo.at[pl.ds(i * (H // NWO), H // NWO)], sem_o.at[i])
                for i in range(NWO)]
        c_x = pltpu.make_async_copy(x_hbm, x0, sem_x.at[0])

        c_fa.start()
        c_sh.start()
        for j in range(NCH):
            cp_k(j).start()
            cp_v(j).start()
            cp_h(j).start()
        c_fi.start()
        c_d.start()
        c_bias.start()
        c_mem0.start()
        for s in range(HP):
            for j in range(3):
                cp_w(j, s).start()
        for c in c_wo:
            c.start()
        c_x.start()

        kb[0:KPAD, :] = jnp.zeros((KPAD, Dm), BF16)
        Ap[...] = jnp.zeros(Ap.shape, F32)
        c_fa.wait()
        c_sh.wait()
        sh = shv[...].astype(F32)

        def fwd(j, carry):
            cp_k(j).wait()
            cp_v(j).wait()
            cp_h(j).wait()
            r0 = pl.multiple_of(j * CH, CH)
            kf = kb[pl.ds(r0, CH + KPAD), :].astype(F32)
            ks = kf[KPAD:KPAD + CH] * sh[0:1]
            for dlt in range(1, KS):
                ks = ks + kf[KPAD - dlt:KPAD - dlt + CH] * sh[dlt:dlt + 1]
            u = (ks * vb[pl.ds(r0, CH), :].astype(F32)).astype(BF16)
            ub[pl.ds(r0, CH), :] = u
            fav = fa[...]
            Ub[j] = jnp.dot(fav, u, preferred_element_type=F32)
            a = lax.dot_general(fav, hb[j], (((1,), (1,)), ((), ())),
                                preferred_element_type=F32)
            p = Ap[...]
            hh = CH // 2
            Gb[j, 0:hh] = a[0:hh] - p[CH:CH + hh]
            Gb[j, hh:CH] = a[hh:CH] + p[CH + hh:2 * CH]
            Gb[j, CH:CH + hh] = a[CH:CH + hh] + p[0:hh]
            Gb[j, CH + hh:2 * CH] = a[CH + hh:2 * CH] - p[hh:CH]
            Ap[...] = a
            return carry
        lax.fori_loop(0, NCH, fwd, 0)

        BL = 4

        def mac(f, carry):
            rr = pl.multiple_of(f * 8, 8)
            ri = pl.multiple_of(CH + f * 8, 8)
            for c in range(NT):
                cs = slice(c * 128, (c + 1) * 128)
                for ib in reversed(range(NCH // BL)):
                    yr = [None] * BL
                    yi = [None] * BL
                    for jb in range(ib + 1):
                        for jj in range(BL):
                            J = jb * BL + jj
                            ur = Ub[J, pl.ds(rr, 8), cs]
                            ui = Ub[J, pl.ds(ri, 8), cs]
                            for ii in range(BL):
                                I = ib * BL + ii
                                if I < J:
                                    continue
                                gr = Gb[I - J, pl.ds(rr, 8), cs]
                                gi = Gb[I - J, pl.ds(ri, 8), cs]
                                tr = gr * ur - gi * ui
                                ti = gr * ui + gi * ur
                                yr[ii] = tr if yr[ii] is None else yr[ii] + tr
                                yi[ii] = ti if yi[ii] is None else yi[ii] + ti
                    for ii in range(BL):
                        Ub[ib * BL + ii, pl.ds(rr, 8), cs] = yr[ii]
                        Ub[ib * BL + ii, pl.ds(ri, 8), cs] = yi[ii]
            return carry
        lax.fori_loop(0, CH // 8, mac, 0)

        c_fi.wait()
        c_d.wait()
        dvec = dv[...].astype(F32).reshape(1, Dm)

        def inv(i, carry):
            r0 = pl.multiple_of(i * CH, CH)
            y = jnp.dot(fi[...], Ub[i].astype(BF16), preferred_element_type=F32)
            yb[pl.ds(r0, CH), :] = y + ub[pl.ds(r0, CH), :].astype(F32) * dvec
            return carry
        lax.fori_loop(0, NCH, inv, 0)

        def repack(s, carry):
            for j in range(3):
                cp_w(j, s).wait()
                a = wstage[j, s, pl.ds(0, Dm // 2, stride=2), :]
                b = wstage[j, s, pl.ds(1, Dm // 2, stride=2), :]
                wqkv[j, 2 * s] = (a & jnp.uint32(0xFFFF)) | (b << 16)
                wqkv[j, 2 * s + 1] = (a >> 16) | (b & jnp.uint32(0xFFFF0000))
            return carry
        lax.fori_loop(0, HP, repack, 0)

        hbuf[...] = jnp.zeros(hbuf.shape, U32)
        x2buf[...] = jnp.zeros(x2buf.shape, F32)
        ox[...] = jnp.zeros(ox.shape, F32)
        c_bias.wait()
        c_mem0.wait()
        c_x.wait()
        for c in c_wo:
            c.wait()
        hbuf[0, 0:M // 2, :] = _pack16(mem0[...].astype(F32))
        hbuf[0, M:M + seg // 2, :] = _pack16(_ln(x0[0:seg, :].astype(F32)))

        def finish(s, r0):
            x3 = x2buf[s + 1] + ox[seg:2 * seg, :]
            x4 = x3 + _ln(x3) * yb[pl.ds(r0, seg), :]
            ob[pl.ds(r0, seg), :] = x4.astype(BF16)

        def step(t, carry):
            par = t & 1
            npar = 1 - par
            hh = pltpu.bitcast(hbuf[par], BF16)

            def proj(h, j):
                return jnp.dot(hh, pltpu.bitcast(wqkv[j, h], BF16), preferred_element_type=F32)
            zpad = jnp.zeros((128 - R, Dh), F32)

            def pad(x):
                return jnp.concatenate([x, zpad], axis=0).astype(BF16)

            def scores(q, k):
                s = lax.dot_general(q, k, (((1,), (1,)), ((), ())), preferred_element_type=F32)
                s = s * qk_scale + bias[...]
                m = jnp.max(s, axis=-1, keepdims=True)
                p = jnp.exp2(s - m)
                l = jnp.sum(p, axis=-1, keepdims=True)
                r = pl.reciprocal(l, approx=True)
                r = r * (2.0 - l * r)
                return (p * r).astype(BF16)

            def pv(p, v):
                return jnp.dot(p, v, preferred_element_type=F32).astype(BF16)

            def wout(h, z):
                r = jnp.dot(z, pltpu.bitcast(wo[h], BF16), preferred_element_type=F32)
                if h == 0:
                    acc[...] = r
                else:
                    acc[...] += r

            def post1():
                s = jnp.maximum(t - 1, 0)
                r0 = pl.multiple_of(s * seg, seg)
                x1 = x0[pl.ds(r0, seg), :].astype(F32) + ox[0:seg, :]
                x2 = x1 + _ln(x1) * yb[pl.ds(r0, seg), :]
                x2buf[t] = x2
                hbuf[npar, M + seg // 2:M + seg, :] = _pack16(_ln(x2))

            def post2():
                s = jnp.maximum(t - 1 - LAG, 0)
                finish(s, pl.multiple_of(s * seg, seg))

            def pre1():
                s = jnp.minimum(t + 1, NSEG - 1)
                r0 = pl.multiple_of(s * seg, seg)
                hbuf[npar, M:M + seg // 2, :] = _pack16(_ln(x0[pl.ds(r0, seg), :].astype(F32)))
            extra = {extras[0]: post1, extras[1]: post2, extras[2]: pre1}

            q, k, v, p, z = {}, {}, {}, {}, {}
            for i in range(H + lW):
                for op in order:
                    if op == 'q' and i < H:
                        q[i] = proj(i, 0).astype(BF16)
                    if op == 'k' and i < H:
                        k[i] = pad(proj(i, 1))
                    if op == 'v' and i < H:
                        v[i] = pad(proj(i, 2))
                    if op == 'S' and 0 <= i - lS < H:
                        p[i - lS] = scores(q.pop(i - lS), k.pop(i - lS))
                    if op == 'P' and 0 <= i - lP < H:
                        z[i - lP] = pv(p.pop(i - lP), v.pop(i - lP))
                    if op == 'W' and 0 <= i - lW < H:
                        wout(i - lW, z.pop(i - lW))
                if i in extra:
                    extra[i]()
            assert not (q or k or v or p or z)
            a = acc[...]
            mp = _pack16(a[0:2 * M, :])
            m0p = _pack16(mem0[...].astype(F32))
            hbuf[npar, 0:M // 2, :] = mp[0:M // 2]
            hbuf[npar, M // 2:M, :] = jnp.where(t + 1 == LAG, m0p, mp[M // 2:M])
            ox[...] = a[2 * M:R, :]
            return carry
        lax.fori_loop(0, nsteps, step, 0)
        finish(NSEG - 1, (NSEG - 1) * seg)
        c_out = pltpu.make_async_copy(ob, o_hbm, sem_out.at[0])
        c_out.start()
        c_out.wait()

    scratch = [
        pltpu.VMEM((3, H, Dm // 2, Dh), U32),
        pltpu.VMEM((3, HP, Dm, Dh), U32),
        pltpu.VMEM((H, Dh // 2, Dm), U32),
        pltpu.VMEM((S, Dm), BF16),
        pltpu.VMEM((KPAD + S, Dm), BF16),
        pltpu.VMEM((S, Dm), BF16),
        pltpu.VMEM((NCH, Dm, CH), BF16),
        pltpu.VMEM((S, Dm), BF16),
        pltpu.VMEM((NCH, 2 * CH, Dm), F32),
        pltpu.VMEM((NCH, 2 * CH, Dm), F32),
        pltpu.VMEM((2 * CH, Dm), F32),
        pltpu.VMEM((S, Dm), F32),
        pltpu.VMEM((2, R // 2, Dm), U32),
        pltpu.VMEM((R, Dm), F32),
        pltpu.VMEM((NSEG + LAG + 1, seg, Dm), F32),
        pltpu.VMEM((2 * seg, Dm), F32),
        pltpu.VMEM((S, Dm), BF16),
        pltpu.VMEM((2 * CH, CH), BF16),
        pltpu.VMEM((CH, 2 * CH), BF16),
        pltpu.VMEM((R, 128), F32),
        pltpu.VMEM((M, Dm), BF16),
        pltpu.VMEM((KS, Dm), BF16),
        pltpu.VMEM((Dm,), BF16),
        pltpu.SemaphoreType.DMA((6,)),
        pltpu.SemaphoreType.DMA((NCH,)),
        pltpu.SemaphoreType.DMA((NCH,)),
        pltpu.SemaphoreType.DMA((NCH,)),
        pltpu.SemaphoreType.DMA((3, HP)),
        pltpu.SemaphoreType.DMA((4,)),
        pltpu.SemaphoreType.DMA((1,)),
        pltpu.SemaphoreType.DMA((1,)),
    ]
    return kernel, scratch


def _run(A_x, A_mem0, A_Wq, A_Wk, A_Wv, A_Wo, A_seg_len, B_k, B_v, B_shift_k, B_ssm_k, B_ssm_D,
         cfg=None):
    B, S, Dm = A_x.shape
    assert B == 1
    _, H, Dh = A_Wq.shape
    M = A_mem0.shape[1]
    seg = int(A_seg_len)
    KS = B_shift_k.shape[-1]
    kernel, scratch = _build(S, Dm, H, Dh, M, seg, KS, cfg or {})
    fa_np, fi_np = _dft_mats()
    bias_np = _attn_bias(M, seg)
    args = (A_x.reshape(S, Dm), A_mem0.reshape(M, Dm), A_Wq, A_Wk, A_Wv, A_Wo,
            B_k.reshape(S, Dm), B_v.reshape(S, Dm), B_shift_k.T, B_ssm_k, B_ssm_D,
            fa_np, fi_np, bias_np)
    out = pl.pallas_call(
        kernel,
        out_shape=jax.ShapeDtypeStruct((S, Dm), BF16),
        in_specs=[pl.BlockSpec(memory_space=pl.ANY)] * len(args),
        out_specs=pl.BlockSpec(memory_space=pl.ANY),
        scratch_shapes=scratch,
        compiler_params=pltpu.CompilerParams(vmem_limit_bytes=110 * 1024 * 1024),
    )(*args)
    return out.reshape(B, S, Dm)


@functools.partial(jax.jit, static_argnames=("A_seg_len",))
def pallas_interleave_layers__memory_aug_recurrent_mem_tr__ssm_conv_h3__prompt_kernel(
    A_x: jax.Array,
    A_mem0: jax.Array,
    A_Wq: jax.Array,
    A_Wk: jax.Array,
    A_Wv: jax.Array,
    A_Wo: jax.Array,
    A_seg_len: int,
    B_q: jax.Array,
    B_k: jax.Array,
    B_v: jax.Array,
    B_shift_k: jax.Array,
    B_ssm_k: jax.Array,
    B_ssm_D: jax.Array,
):
    del B_q
    return _run(A_x, A_mem0, A_Wq, A_Wk, A_Wv, A_Wo, A_seg_len, B_k, B_v, B_shift_k,
                B_ssm_k, B_ssm_D)
```

```python
import functools

import jax
import jax.numpy as jnp
import numpy as np
from jax import lax
from jax.experimental import pallas as pl
from jax.experimental.pallas import tpu as pltpu

F32, BF16, U32 = jnp.float32, jnp.bfloat16, jnp.uint32

LOG2E = 1.4426950408889634
LN_EPS = 1e-5
CH = 128
LAG = 2
KPAD = 16


def _np_bf16(a):
    return np.asarray(a, dtype=np.float32).astype(BF16)


def _dft_mats():
    n2 = 2 * CH
    karr = np.concatenate([np.arange(0, CH, 2), np.arange(1, CH, 2)])
    n = np.arange(CH)
    th = 2.0 * np.pi * n[None, :] * (karr[:, None] + 0.5) / n2
    fa = np.concatenate([np.cos(th), -np.sin(th)], axis=0)
    fi = np.concatenate([np.cos(th).T, -np.sin(th).T], axis=1) * (2.0 / n2)
    return _np_bf16(fa), _np_bf16(fi)


def _attn_bias(m, seg):
    rows = 2 * (m + seg)
    idx = np.arange(128)

    def stream(i):
        return np.where(i < m, 0, np.where(i < 2 * m, 1, np.where(
            i < 2 * m + seg, 0, np.where(i < rows, 1, 2))))

    def ismem(i):
        return i < 2 * m

    def pos(i):
        return np.where(i < 2 * m + seg, i - 2 * m, i - 2 * m - seg)

    r, c = idx[:rows, None], idx[None, :]
    same = stream(r) == stream(c)
    keep = ismem(r) | ismem(c) | (pos(r) >= pos(c))
    fill = np.where(same, -1e9 * LOG2E, -1e30)
    both = np.where(same & keep, 0.0, fill).astype(np.float32)
    sel = np.concatenate([np.arange(2 * m), np.arange(2 * m + seg, rows)])
    only2 = np.full((2 * m + seg, 128), -1e30, np.float32)
    only2[:, :2 * m + seg] = both[sel][:, sel]
    return np.concatenate([both, only2], axis=0)


def _ln(x):
    m = jnp.mean(x, axis=-1, keepdims=True)
    xc = x - m
    v = jnp.mean(xc * xc, axis=-1, keepdims=True)
    return xc * lax.rsqrt(v + LN_EPS)


def _pack16(x):
    return pltpu.bitcast(x.astype(BF16), U32)


def _build(S, Dm, H, Dh, M, seg, KS, cfg):
    assert Dh == 128 and Dm % 128 == 0 and S % CH == 0 and H % 16 == 0
    assert M == 8 and seg == 32 and KS <= 8
    NSEG = S // seg
    NCH = S // CH
    NT = Dm // 128
    R = 2 * (M + seg)
    HP = H // 2
    qk_scale = float(Dh ** -0.5) * LOG2E
    LAGS = {"b": (2, 4, 12, (3, 2, 1)), "bp": (2, 4, 12, (3, 2, 1, 1)), "1": (2, 5, 14, (4, 3, 2, 1)),
            "2": (2, 4, 12, (4, 3, 2, 1))}
    order = cfg.get("order", "qSkPvW")
    extras = cfg.get("extras", (3, 11, 19))
    nsteps = cfg.get("nsteps", NSEG + LAG)
    skip = cfg.get("skip", "")
    NS = cfg.get("ns", 7)
    assert LAG < NS <= NSEG - 1

    def kernel(x_hbm, mem0_hbm, wq_hbm, wk_hbm, wv_hbm, wo_hbm, k_hbm, v_hbm, sh_hbm, h_hbm,
               d_hbm, fa_hbm, fi_hbm, bias_hbm, o_hbm,
               wqkv, wstage, wo, x0, kb, vb, hb, ub, Ub, Gb, Ap, yb,
               hbuf, hx, qkvx, acc, x2buf, ox, ob, fa, fi, bias, mem0, shv, dv,
               sem_c, sem_k, sem_v, sem_h, sem_w, sem_o, sem_x, sem_out):
        c_fa = pltpu.make_async_copy(fa_hbm, fa, sem_c.at[0])
        c_sh = pltpu.make_async_copy(sh_hbm, shv, sem_c.at[1])
        c_fi = pltpu.make_async_copy(fi_hbm, fi, sem_c.at[2])
        c_d = pltpu.make_async_copy(d_hbm, dv, sem_c.at[3])
        c_bias = pltpu.make_async_copy(bias_hbm, bias, sem_c.at[4])
        c_mem0 = pltpu.make_async_copy(mem0_hbm, mem0, sem_c.at[5])

        def cp_k(j):
            return pltpu.make_async_copy(
                k_hbm.at[pl.ds(j * CH, CH)], kb.at[pl.ds(KPAD + j * CH, CH)], sem_k.at[j])

        def cp_v(j):
            return pltpu.make_async_copy(
                v_hbm.at[pl.ds(j * CH, CH)], vb.at[pl.ds(j * CH, CH)], sem_v.at[j])

        def cp_h(j):
            return pltpu.make_async_copy(
                h_hbm.at[:, pl.ds(j * CH, CH)], hb.at[j], sem_h.at[j])

        w32 = [w.bitcast(U32) for w in (wq_hbm, wk_hbm, wv_hbm)]

        def cp_w(j, s):
            return pltpu.make_async_copy(w32[j].at[:, s, :], wstage.at[j, s], sem_w.at[j, s])

        wo32 = wo_hbm.bitcast(U32)
        NWO = 4
        c_wo = [pltpu.make_async_copy(wo32.at[pl.ds(i * (H // NWO), H // NWO)],
                                      wo.at[pl.ds(i * (H // NWO), H // NWO)], sem_o.at[i])
                for i in range(NWO)]
        XA = NS * seg
        c_xa = pltpu.make_async_copy(x_hbm.at[pl.ds(0, XA)], x0.at[pl.ds(0, XA)], sem_x.at[0])
        c_xb = pltpu.make_async_copy(x_hbm.at[pl.ds(XA, S - XA)], x0.at[pl.ds(XA, S - XA)],
                                     sem_x.at[1])

        WIN = cfg.get("win", 4)
        WST = cfg.get("wst", NCH - 4)
        WW = cfg.get("ww", 3)

        def start_chunk(j):
            cp_k(j).start()
            cp_v(j).start()
            cp_h(j).start()

        def start_slab(s):
            for j in range(3):
                cp_w(j, s).start()

        start_chunk(0)
        c_fa.start()
        c_sh.start()
        for j in range(1, WIN):
            start_chunk(j)
        c_fi.start()
        c_d.start()
        c_bias.start()
        c_mem0.start()
        c_xa.start()

        kb[0:KPAD, :] = jnp.zeros((KPAD, Dm), BF16)
        Ap[...] = jnp.zeros(Ap.shape, F32)
        c_fa.wait()
        c_sh.wait()
        sh = shv[...].astype(F32)

        def fwd(j, carry):
            cp_k(j).wait()
            cp_v(j).wait()
            cp_h(j).wait()

            @pl.when(j + WIN < NCH)
            def _():
                start_chunk(j + WIN)

            @pl.when(j >= WST)
            def _():
                @pl.when(j < WST + WW)
                def _():
                    start_slab(j - WST)
            r0 = pl.multiple_of(j * CH, CH)
            kf = kb[pl.ds(r0, CH + KPAD), :].astype(F32)
            ks = kf[KPAD:KPAD + CH] * sh[0:1]
            for dlt in range(1, KS):
                ks = ks + kf[KPAD - dlt:KPAD - dlt + CH] * sh[dlt:dlt + 1]
            u = (ks * vb[pl.ds(r0, CH), :].astype(F32)).astype(BF16)
            ub[pl.ds(r0, CH), :] = u
            fav = fa[...]
            Ub[j] = jnp.dot(fav, u, preferred_element_type=F32)
            a = lax.dot_general(fav, hb[j], (((1,), (1,)), ((), ())),
                                preferred_element_type=F32)
            p = Ap[...]
            hh = CH // 2
            Gb[j, 0:hh] = a[0:hh] - p[CH:CH + hh]
            Gb[j, hh:CH] = a[hh:CH] + p[CH + hh:2 * CH]
            Gb[j, CH:CH + hh] = a[CH:CH + hh] + p[0:hh]
            Gb[j, CH + hh:2 * CH] = a[CH + hh:2 * CH] - p[hh:CH]
            Ap[...] = a
            return carry
        lax.fori_loop(0, NCH, fwd, 0)

        BL = 4

        c_xa.wait()
        for i in range(NS):
            hx[i * seg // 2:(i + 1) * seg // 2, :] = _pack16(
                _ln(x0[i * seg:(i + 1) * seg, :].astype(F32)))

        def repack(s, j):
            a = wstage[j, s, pl.ds(0, Dm // 2, stride=2), :]
            b = wstage[j, s, pl.ds(1, Dm // 2, stride=2), :]
            wqkv[j, 2 * s] = (a & jnp.uint32(0xFFFF)) | (b << 16)
            wqkv[j, 2 * s + 1] = (a >> 16) | (b & jnp.uint32(0xFFFF0000))

        def run_ahead(s, j, hh):
            w = pltpu.bitcast(wqkv[j, 2 * s + hh], BF16)
            qkvx[j, 2 * s + hh] = jnp.dot(pltpu.bitcast(hx[...], BF16), w,
                                          preferred_element_type=F32)

        assert HP == CH // 8

        def mac(f, carry):
            for j in range(3):
                cp_w(j, f).wait()

            @pl.when(f + WW < HP)
            def _():
                start_slab(f + WW)

            @pl.when(f + WW == HP)
            def _():
                for c in c_wo:
                    c.start()
            rr = pl.multiple_of(f * 8, 8)
            ri = pl.multiple_of(CH + f * 8, 8)

            def mac_piece(c, ib):
                cs = slice(c * 128, (c + 1) * 128)
                yr = [None] * BL
                yi = [None] * BL
                for jb in range(ib + 1):
                    for jj in range(BL):
                        J = jb * BL + jj
                        ur = Ub[J, pl.ds(rr, 8), cs]
                        ui = Ub[J, pl.ds(ri, 8), cs]
                        for ii in range(BL):
                            I = ib * BL + ii
                            if I < J:
                                continue
                            gr = Gb[I - J, pl.ds(rr, 8), cs]
                            gi = Gb[I - J, pl.ds(ri, 8), cs]
                            tr = gr * ur - gi * ui
                            ti = gr * ui + gi * ur
                            yr[ii] = tr if yr[ii] is None else yr[ii] + tr
                            yi[ii] = ti if yi[ii] is None else yi[ii] + ti
                for ii in range(BL):
                    Ub[ib * BL + ii, pl.ds(rr, 8), cs] = yr[ii]
                    Ub[ib * BL + ii, pl.ds(ri, 8), cs] = yi[ii]

            vpu = [(c, ib, min(ib, 1) * 16 * ib + 10) for c in range(NT if 'm' not in skip else 0)
                   for ib in reversed(range(NCH // BL))]
            mxu = []
            for j in range(3):
                mxu.append(((repack, f, j), 0))
                for hh in range(2):
                    mxu.append(((run_ahead, f, j, hh), 1))
            tot = sum(w for *_, w in vpu)
            done = 0
            nm = sum(w for _, w in mxu)
            dm = 0
            vi = 0
            for (fn, *args), w in mxu:
                fn(*args)
                dm += w
                while vi < len(vpu) and done < tot * dm / nm:
                    mac_piece(*vpu[vi][:2])
                    done += vpu[vi][2]
                    vi += 1
            assert vi == len(vpu)
            return carry
        lax.fori_loop(0, CH // 8, mac, 0)

        c_fi.wait()
        c_d.wait()
        dvec = dv[...].astype(F32).reshape(1, Dm)

        def inv(i, carry):
            r0 = pl.multiple_of(i * CH, CH)
            y = jnp.dot(fi[...], Ub[i].astype(BF16), preferred_element_type=F32)
            yb[pl.ds(r0, CH), :] = y + ub[pl.ds(r0, CH), :].astype(F32) * dvec
            return carry
        if 'i' not in skip:
            lax.fori_loop(0, NCH, inv, 0)

        hbuf[...] = jnp.zeros(hbuf.shape, U32)
        x2buf[0] = jnp.zeros(x2buf.shape[1:], F32)
        ox[...] = jnp.zeros(ox.shape, F32)
        c_bias.wait()
        c_mem0.wait()
        for c in c_wo:
            c.wait()
        c_xb.start()
        hbuf[0, 0:M // 2, :] = _pack16(mem0[...].astype(F32))
        MB = M
        XB = seg // 2

        def finish(s, r0):
            x3 = x2buf[s + 1] + ox[seg:2 * seg, :]
            x4 = x3 + _ln(x3) * yb[pl.ds(r0, seg), :]
            ob[pl.ds(r0, seg), :] = x4.astype(BF16)

        def make_step(act1, act2, pre):
            rows = 2 * M + seg * (int(act1) + int(act2))
            b0 = 0 if act1 else R
            x1_in_lhs = act1 and not pre

            key = "b" if (act1 and act2 and not pre) else "bp" if (act1 and act2) else "1" if act1 else "2"
            lS, lP, lW, tail = cfg.get("lag_" + key, LAGS[key])

            def step(t, carry):
                par = t & 1
                npar = 1 - par
                parts = [hbuf[par, 0:MB, :]]
                if x1_in_lhs:
                    parts.append(hbuf[par, MB:MB + XB, :])
                if act2:
                    parts.append(hbuf[par, MB + XB:MB + 2 * XB, :])
                hh = pltpu.bitcast(parts[0] if len(parts) == 1 else jnp.concatenate(parts, axis=0), BF16)
                zpad = jnp.zeros((128 - rows, Dh), F32)

                def proj(h, j, padded):
                    r = jnp.dot(hh, pltpu.bitcast(wqkv[j, h], BF16), preferred_element_type=F32)
                    blocks = [r]
                    if pre:
                        x1p = qkvx[j, h, pl.ds(pl.multiple_of(t * seg, seg), seg), :]
                        blocks = [r[0:2 * M], x1p] + ([r[2 * M:]] if act2 else [])
                    if padded:
                        blocks.append(zpad)
                    u = blocks[0] if len(blocks) == 1 else jnp.concatenate(blocks, axis=0)
                    return u.astype(BF16)

                def scores(q, k):
                    s = lax.dot_general(q, k, (((1,), (1,)), ((), ())), preferred_element_type=F32)
                    s = s * qk_scale + bias[b0:b0 + rows, :]
                    m = jnp.max(s, axis=-1, keepdims=True)
                    p = jnp.exp2(s - m)
                    l = jnp.sum(p, axis=-1, keepdims=True)
                    r = pl.reciprocal(l, approx=True)
                    r = r * (2.0 - l * r)
                    return (p * r).astype(BF16)

                def pv(p, v):
                    return jnp.dot(p, v, preferred_element_type=F32).astype(BF16)

                def wout(h, z):
                    return jnp.dot(z, pltpu.bitcast(wo[h], BF16), preferred_element_type=F32)

                def post1():
                    s = jnp.minimum(jnp.maximum(t - 1, 0), NSEG - 1)
                    r0 = pl.multiple_of(s * seg, seg)
                    x1 = x0[pl.ds(r0, seg), :].astype(F32) + ox[0:seg, :]
                    x2 = x1 + _ln(x1) * yb[pl.ds(r0, seg), :]
                    x2buf[t] = x2
                    hbuf[npar, MB + XB:MB + 2 * XB, :] = _pack16(_ln(x2))

                def post2():
                    s = jnp.maximum(t - 1 - LAG, 0)
                    finish(s, pl.multiple_of(s * seg, seg))

                def pre1():
                    s = jnp.minimum(t + 1, NSEG - 1)
                    r0 = pl.multiple_of(s * seg, seg)
                    hbuf[npar, MB:MB + XB, :] = _pack16(_ln(x0[pl.ds(r0, seg), :].astype(F32)))
                extra = {extras[0]: post1}
                if act2:
                    extra[extras[1]] = post2
                if act1 and act2:
                    extra[extras[2]] = pre1

                q, k, v, p, z = {}, {}, {}, {}, {}
                s_at = {h: h + lS for h in range(H)}
                p_at = {h: h + lP for h in range(H)}
                w_at = {h: h + lW for h in range(H)}
                for d, extra_lag in enumerate(tail):
                    p_at[H - 1 - d] += extra_lag
                fin = []
                accv = acc.at[0:rows]
                for i in range(max(w_at.values()) + 1):
                    for op in order:
                        if op == 'q' and i < H:
                            q[i] = proj(i, 0, False)
                        if op == 'k' and i < H:
                            k[i] = proj(i, 1, True)
                        if op == 'v' and i < H:
                            v[i] = proj(i, 2, True)
                        for h in range(H):
                            if op == 'S' and s_at[h] == i:
                                p[h] = scores(q.pop(h), k.pop(h))
                            if op == 'P' and p_at[h] == i:
                                z[h] = pv(p.pop(h), v.pop(h))
                            if op == 'W' and w_at[h] == i:
                                r = wout(h, z.pop(h))
                                if h == 0:
                                    accv[...] = r
                                elif h == H - 1:
                                    fin.append(accv[...] + r)
                                else:
                                    accv[...] += r
                    if i in extra:
                        extra[i]()
                assert not (q or k or v or p or z)
                a = fin[0]
                mp = _pack16(a[0:2 * M, :])
                if act2:
                    hbuf[npar, 0:MB, :] = mp
                else:
                    hbuf[npar, 0:MB // 2, :] = mp[0:MB // 2]
                    hbuf[npar, MB // 2:MB, :] = _pack16(mem0[...].astype(F32))
                if act1 and act2:
                    ox[...] = a[2 * M:R, :]
                elif act1:
                    ox[0:seg, :] = a[2 * M:, :]
                else:
                    ox[seg:2 * seg, :] = a[2 * M:, :]
                return carry
            return step

        lax.fori_loop(0, LAG, make_step(True, False, True), 0)
        c_xb.wait()
        nboth = nsteps - LAG
        lax.fori_loop(LAG, min(NS, nboth), make_step(True, True, True), 0)
        lax.fori_loop(NS, nboth, make_step(True, True, False), 0)
        OA = (NSEG - LAG - 1) * seg
        c_oa = pltpu.make_async_copy(ob.at[pl.ds(0, OA)], o_hbm.at[pl.ds(0, OA)], sem_out.at[0])
        c_oa.start()
        lax.fori_loop(NSEG, NSEG + LAG, make_step(False, True, False), 0)
        finish(NSEG - 1, (NSEG - 1) * seg)
        c_ob = pltpu.make_async_copy(ob.at[pl.ds(OA, S - OA)], o_hbm.at[pl.ds(OA, S - OA)],
                                     sem_out.at[1])
        c_ob.start()
        c_oa.wait()
        c_ob.wait()

    scratch = [
        pltpu.VMEM((3, H, Dm // 2, Dh), U32),
        pltpu.VMEM((3, HP, Dm, Dh), U32),
        pltpu.VMEM((H, Dh // 2, Dm), U32),
        pltpu.VMEM((S, Dm), BF16),
        pltpu.VMEM((KPAD + S, Dm), BF16),
        pltpu.VMEM((S, Dm), BF16),
        pltpu.VMEM((NCH, Dm, CH), BF16),
        pltpu.VMEM((S, Dm), BF16),
        pltpu.VMEM((NCH, 2 * CH, Dm), F32),
        pltpu.VMEM((NCH, 2 * CH, Dm), F32),
        pltpu.VMEM((2 * CH, Dm), F32),
        pltpu.VMEM((S, Dm), F32),
        pltpu.VMEM((2, R // 2, Dm), U32),
        pltpu.VMEM((NS * seg // 2, Dm), U32),
        pltpu.VMEM((3, H, NS * seg, Dh), F32),
        pltpu.VMEM((R, Dm), F32),
        pltpu.VMEM((NSEG + LAG + 1, seg, Dm), F32),
        pltpu.VMEM((2 * seg, Dm), F32),
        pltpu.VMEM((S, Dm), BF16),
        pltpu.VMEM((2 * CH, CH), BF16),
        pltpu.VMEM((CH, 2 * CH), BF16),
        pltpu.VMEM((R + 2 * M + seg, 128), F32),
        pltpu.VMEM((M, Dm), BF16),
        pltpu.VMEM((KS, Dm), BF16),
        pltpu.VMEM((Dm,), BF16),
        pltpu.SemaphoreType.DMA((6,)),
        pltpu.SemaphoreType.DMA((NCH,)),
        pltpu.SemaphoreType.DMA((NCH,)),
        pltpu.SemaphoreType.DMA((NCH,)),
        pltpu.SemaphoreType.DMA((3, HP)),
        pltpu.SemaphoreType.DMA((4,)),
        pltpu.SemaphoreType.DMA((2,)),
        pltpu.SemaphoreType.DMA((2,)),
    ]
    return kernel, scratch


def _run(A_x, A_mem0, A_Wq, A_Wk, A_Wv, A_Wo, A_seg_len, B_k, B_v, B_shift_k, B_ssm_k, B_ssm_D,
         cfg=None):
    B, S, Dm = A_x.shape
    assert B == 1
    _, H, Dh = A_Wq.shape
    M = A_mem0.shape[1]
    seg = int(A_seg_len)
    KS = B_shift_k.shape[-1]
    kernel, scratch = _build(S, Dm, H, Dh, M, seg, KS, cfg or {})
    fa_np, fi_np = _dft_mats()
    bias_np = _attn_bias(M, seg)
    args = (A_x.reshape(S, Dm), A_mem0.reshape(M, Dm), A_Wq, A_Wk, A_Wv, A_Wo,
            B_k.reshape(S, Dm), B_v.reshape(S, Dm), B_shift_k.T, B_ssm_k, B_ssm_D,
            fa_np, fi_np, bias_np)
    out = pl.pallas_call(
        kernel,
        out_shape=jax.ShapeDtypeStruct((S, Dm), BF16),
        in_specs=[pl.BlockSpec(memory_space=pl.ANY)] * len(args),
        out_specs=pl.BlockSpec(memory_space=pl.ANY),
        scratch_shapes=scratch,
        compiler_params=pltpu.CompilerParams(vmem_limit_bytes=110 * 1024 * 1024,
                                             flags=(cfg or {}).get("flags")),
    )(*args)
    return out.reshape(B, S, Dm)


@functools.partial(jax.jit, static_argnames=("A_seg_len",))
def pallas_interleave_layers__memory_aug_recurrent_mem_tr__ssm_conv_h3__prompt_kernel(
    A_x: jax.Array,
    A_mem0: jax.Array,
    A_Wq: jax.Array,
    A_Wk: jax.Array,
    A_Wv: jax.Array,
    A_Wo: jax.Array,
    A_seg_len: int,
    B_q: jax.Array,
    B_k: jax.Array,
    B_v: jax.Array,
    B_shift_k: jax.Array,
    B_ssm_k: jax.Array,
    B_ssm_D: jax.Array,
):
    del B_q
    return _run(A_x, A_mem0, A_Wq, A_Wk, A_Wv, A_Wo, A_seg_len, B_k, B_v, B_shift_k,
                B_ssm_k, B_ssm_D)
```

```python
import functools

import jax
import jax.numpy as jnp
import numpy as np
from jax import lax
from jax.experimental import pallas as pl
from jax.experimental.pallas import tpu as pltpu

F32, BF16, U32 = jnp.float32, jnp.bfloat16, jnp.uint32

LOG2E = 1.4426950408889634
LN_EPS = 1e-5
CH = 128
LAG = 2
KPAD = 16


def _np_bf16(a):
    return np.asarray(a, dtype=np.float32).astype(BF16)


def _dft_mats():
    n2 = 2 * CH
    karr = np.concatenate([np.arange(0, CH, 2), np.arange(1, CH, 2)])
    n = np.arange(CH)
    th = 2.0 * np.pi * n[None, :] * (karr[:, None] + 0.5) / n2
    fa = np.concatenate([np.cos(th), -np.sin(th)], axis=0)
    fi = np.concatenate([np.cos(th).T, -np.sin(th).T], axis=1) * (2.0 / n2)
    return _np_bf16(fa), _np_bf16(fi)


def _attn_bias(m, seg):
    stream = np.concatenate([np.zeros(seg), np.ones(seg), np.zeros(m), np.ones(m)])
    ismem = np.concatenate([np.zeros(2 * seg), np.ones(2 * m)]).astype(bool)
    pos = np.concatenate([np.arange(seg), np.arange(seg), np.zeros(2 * m)])
    same = stream[:, None] == stream[None, :]
    keep = ismem[:, None] | ismem[None, :] | (pos[:, None] >= pos[None, :])
    full = np.where(same & keep, 0.0, np.where(same, -1e9 * LOG2E, -1e30))
    s1, s2, mm = np.arange(seg), np.arange(seg, 2 * seg), np.arange(2 * seg, 2 * seg + 2 * m)
    out = []
    for sel in (np.concatenate([s1, s2, mm]), np.concatenate([s1, mm]), np.concatenate([s2, mm])):
        b = np.full((len(sel), 128), -1e30, np.float32)
        b[:, :len(sel)] = full[sel][:, sel]
        out.append(b)
    return np.concatenate(out, axis=0)


def _ln(x):
    m = jnp.mean(x, axis=-1, keepdims=True)
    xc = x - m
    v = jnp.mean(xc * xc, axis=-1, keepdims=True)
    return xc * lax.rsqrt(v + LN_EPS)


def _pack16(x):
    return pltpu.bitcast(x.astype(BF16), U32)


def _build(S, Dm, H, Dh, M, seg, KS, cfg):
    assert Dh == 128 and Dm % 128 == 0 and S % CH == 0 and H % 16 == 0
    assert M == 8 and seg == 32 and KS <= 8
    NSEG = S // seg
    NCH = S // CH
    NT = Dm // 128
    R = 2 * (M + seg)
    HP = H // 2
    qk_scale = float(Dh ** -0.5) * LOG2E
    LAGS = {"b": (2, 4, 12, (3, 2, 1)), "bp": (2, 4, 12, (3, 2, 1, 1)), "1": (2, 5, 14, (4, 3, 2, 1)),
            "2": (2, 4, 12, (4, 3, 2, 1))}
    order = cfg.get("order", "qSkPvW")
    extras = cfg.get("extras", (3, 11, 19))
    nsteps = cfg.get("nsteps", NSEG + LAG)
    skip = cfg.get("skip", "")
    NS = cfg.get("ns", 6)
    assert LAG < NS <= NSEG - 1

    def kernel(x_hbm, mem0_hbm, wq_hbm, wk_hbm, wv_hbm, wo_hbm, k_hbm, v_hbm, sh_hbm, h_hbm,
               d_hbm, fa_hbm, fi_hbm, bias_hbm, o_hbm,
               wqkv, wstage, wo, x0, kb, vb, hb, ub, Ub, Gb, Ap, yb,
               hbuf, hx, qkvx, acc, x2buf, ox, ob, fa, fi, bias, mem0, shv, dv,
               sem_c, sem_k, sem_v, sem_h, sem_w, sem_o, sem_x, sem_out):
        c_fa = pltpu.make_async_copy(fa_hbm, fa, sem_c.at[0])
        c_sh = pltpu.make_async_copy(sh_hbm, shv, sem_c.at[1])
        c_fi = pltpu.make_async_copy(fi_hbm, fi, sem_c.at[2])
        c_d = pltpu.make_async_copy(d_hbm, dv, sem_c.at[3])
        c_bias = pltpu.make_async_copy(bias_hbm, bias, sem_c.at[4])
        c_mem0 = pltpu.make_async_copy(mem0_hbm, mem0, sem_c.at[5])

        def cp_k(j):
            return pltpu.make_async_copy(
                k_hbm.at[pl.ds(j * CH, CH)], kb.at[pl.ds(KPAD + j * CH, CH)], sem_k.at[j])

        def cp_v(j):
            return pltpu.make_async_copy(
                v_hbm.at[pl.ds(j * CH, CH)], vb.at[pl.ds(j * CH, CH)], sem_v.at[j])

        def cp_h(j):
            return pltpu.make_async_copy(
                h_hbm.at[:, pl.ds(j * CH, CH)], hb.at[j], sem_h.at[j])

        w32 = [w.bitcast(U32) for w in (wq_hbm, wk_hbm, wv_hbm)]

        def cp_w(j, s):
            return pltpu.make_async_copy(w32[j].at[:, s, :], wstage.at[j, s], sem_w.at[j, s])

        wo32 = wo_hbm.bitcast(U32)
        NWO = 4
        c_wo = [pltpu.make_async_copy(wo32.at[pl.ds(i * (H // NWO), H // NWO)],
                                      wo.at[pl.ds(i * (H // NWO), H // NWO)], sem_o.at[i])
                for i in range(NWO)]
        XA = NS * seg
        c_xa = pltpu.make_async_copy(x_hbm.at[pl.ds(0, XA)], x0.at[pl.ds(0, XA)], sem_x.at[0])
        c_xb = pltpu.make_async_copy(x_hbm.at[pl.ds(XA, S - XA)], x0.at[pl.ds(XA, S - XA)],
                                     sem_x.at[1])

        WIN = cfg.get("win", 4)
        WST = cfg.get("wst", NCH - 4)
        WW = cfg.get("ww", 3)

        def start_chunk(j):
            cp_k(j).start()
            cp_v(j).start()
            cp_h(j).start()

        def start_slab(s):
            for j in range(3):
                cp_w(j, s).start()

        start_chunk(0)
        c_fa.start()
        c_sh.start()
        for j in range(1, WIN):
            start_chunk(j)
        c_fi.start()
        c_d.start()
        c_bias.start()
        c_mem0.start()
        c_xa.start()

        kb[0:KPAD, :] = jnp.zeros((KPAD, Dm), BF16)
        Ap[...] = jnp.zeros(Ap.shape, F32)
        c_fa.wait()
        c_sh.wait()
        sh = shv[...].astype(F32)

        def fwd(j, carry):
            cp_k(j).wait()
            cp_v(j).wait()
            cp_h(j).wait()

            @pl.when(j + WIN < NCH)
            def _():
                start_chunk(j + WIN)

            @pl.when(j >= WST)
            def _():
                @pl.when(j < WST + WW)
                def _():
                    start_slab(j - WST)
            r0 = pl.multiple_of(j * CH, CH)
            kf = kb[pl.ds(r0, CH + KPAD), :].astype(F32)
            ks = kf[KPAD:KPAD + CH] * sh[0:1]
            for dlt in range(1, KS):
                ks = ks + kf[KPAD - dlt:KPAD - dlt + CH] * sh[dlt:dlt + 1]
            u = (ks * vb[pl.ds(r0, CH), :].astype(F32)).astype(BF16)
            ub[pl.ds(r0, CH), :] = u
            fav = fa[...]
            Ub[j] = jnp.dot(fav, u, preferred_element_type=F32)
            a = lax.dot_general(fav, hb[j], (((1,), (1,)), ((), ())),
                                preferred_element_type=F32)
            p = Ap[...]
            hh = CH // 2
            Gb[j, 0:hh] = a[0:hh] - p[CH:CH + hh]
            Gb[j, hh:CH] = a[hh:CH] + p[CH + hh:2 * CH]
            Gb[j, CH:CH + hh] = a[CH:CH + hh] + p[0:hh]
            Gb[j, CH + hh:2 * CH] = a[CH + hh:2 * CH] - p[hh:CH]
            Ap[...] = a
            return carry
        lax.fori_loop(0, NCH, fwd, 0)

        BL = 4

        c_xa.wait()
        for i in range(NS):
            hx[i * seg // 2:(i + 1) * seg // 2, :] = _pack16(
                _ln(x0[i * seg:(i + 1) * seg, :].astype(F32)))

        def repack(s, j):
            a = wstage[j, s, pl.ds(0, Dm // 2, stride=2), :]
            b = wstage[j, s, pl.ds(1, Dm // 2, stride=2), :]
            wqkv[j, 2 * s] = (a & jnp.uint32(0xFFFF)) | (b << 16)
            wqkv[j, 2 * s + 1] = (a >> 16) | (b & jnp.uint32(0xFFFF0000))

        def run_ahead(s, j, hh):
            w = pltpu.bitcast(wqkv[j, 2 * s + hh], BF16)
            qkvx[j, 2 * s + hh] = jnp.dot(pltpu.bitcast(hx[...], BF16), w,
                                          preferred_element_type=F32)

        assert HP == CH // 8

        def mac(f, carry):
            for j in range(3):
                cp_w(j, f).wait()

            @pl.when(f + WW < HP)
            def _():
                start_slab(f + WW)

            @pl.when(f + WW == HP)
            def _():
                for c in c_wo:
                    c.start()
            rr = pl.multiple_of(f * 8, 8)
            ri = pl.multiple_of(CH + f * 8, 8)

            def mac_piece(c, ib):
                cs = slice(c * 128, (c + 1) * 128)
                yr = [None] * BL
                yi = [None] * BL
                for jb in range(ib + 1):
                    for jj in range(BL):
                        J = jb * BL + jj
                        ur = Ub[J, pl.ds(rr, 8), cs]
                        ui = Ub[J, pl.ds(ri, 8), cs]
                        for ii in range(BL):
                            I = ib * BL + ii
                            if I < J:
                                continue
                            gr = Gb[I - J, pl.ds(rr, 8), cs]
                            gi = Gb[I - J, pl.ds(ri, 8), cs]
                            tr = gr * ur - gi * ui
                            ti = gr * ui + gi * ur
                            yr[ii] = tr if yr[ii] is None else yr[ii] + tr
                            yi[ii] = ti if yi[ii] is None else yi[ii] + ti
                for ii in range(BL):
                    Ub[ib * BL + ii, pl.ds(rr, 8), cs] = yr[ii]
                    Ub[ib * BL + ii, pl.ds(ri, 8), cs] = yi[ii]

            vpu = [(c, ib, min(ib, 1) * 16 * ib + 10) for c in range(NT if 'm' not in skip else 0)
                   for ib in reversed(range(NCH // BL))]
            mxu = []
            for j in range(3):
                mxu.append(((repack, f, j), 0))
                for hh in range(2):
                    mxu.append(((run_ahead, f, j, hh), 1))
            tot = sum(w for *_, w in vpu)
            done = 0
            nm = sum(w for _, w in mxu)
            dm = 0
            vi = 0
            for (fn, *args), w in mxu:
                fn(*args)
                dm += w
                while vi < len(vpu) and done < tot * dm / nm:
                    mac_piece(*vpu[vi][:2])
                    done += vpu[vi][2]
                    vi += 1
            assert vi == len(vpu)
            return carry
        lax.fori_loop(0, CH // 8, mac, 0)

        c_fi.wait()
        c_d.wait()
        dvec = dv[...].astype(F32).reshape(1, Dm)

        def inv(i, carry):
            r0 = pl.multiple_of(i * CH, CH)
            y = jnp.dot(fi[...], Ub[i].astype(BF16), preferred_element_type=F32)
            yb[pl.ds(r0, CH), :] = y + ub[pl.ds(r0, CH), :].astype(F32) * dvec
            return carry
        if 'i' not in skip:
            lax.fori_loop(0, NCH, inv, 0)

        hbuf[...] = jnp.zeros(hbuf.shape, U32)
        x2buf[0] = jnp.zeros(x2buf.shape[1:], F32)
        ox[...] = jnp.zeros(ox.shape, F32)
        c_bias.wait()
        c_mem0.wait()
        for c in c_wo:
            c.wait()
        c_xb.start()
        MB = M
        XB = seg // 2
        MO = 2 * XB
        hbuf[0, MO:MO + MB // 2, :] = _pack16(mem0[...].astype(F32))

        def finish(s, r0):
            x3 = x2buf[s + 1] + ox[seg:2 * seg, :]
            x4 = x3 + _ln(x3) * yb[pl.ds(r0, seg), :]
            ob[pl.ds(r0, seg), :] = x4.astype(BF16)

        def make_step(act1, act2, pre):
            rows = 2 * M + seg * (int(act1) + int(act2))
            b0 = 0 if (act1 and act2) else R if act1 else R + 2 * M + seg
            x1_in_lhs = act1 and not pre

            key = "b" if (act1 and act2 and not pre) else "bp" if (act1 and act2) else "1" if act1 else "2"
            lS, lP, lW, tail = cfg.get("lag_" + key, LAGS[key])

            def step(t, par):
                npar = 1 - par
                parts = []
                if x1_in_lhs:
                    parts.append(hbuf[par, 0:XB, :])
                if act2:
                    parts.append(hbuf[par, XB:2 * XB, :])
                parts.append(hbuf[par, MO:MO + MB, :])
                hh = pltpu.bitcast(parts[0] if len(parts) == 1 else jnp.concatenate(parts, axis=0), BF16)
                zpad = jnp.zeros((128 - rows, Dh), F32)

                def proj(h, j, padded):
                    r = jnp.dot(hh, pltpu.bitcast(wqkv[j, h], BF16), preferred_element_type=F32)
                    blocks = [r]
                    if pre:
                        x1p = qkvx[j, h, pl.ds(pl.multiple_of(t * seg, seg), seg), :]
                        blocks = [x1p, r]
                    if padded:
                        blocks.append(zpad)
                    u = blocks[0] if len(blocks) == 1 else jnp.concatenate(blocks, axis=0)
                    return u.astype(BF16)

                def scores(q, k):
                    s = lax.dot_general(q, k, (((1,), (1,)), ((), ())), preferred_element_type=F32)
                    s = s * qk_scale + bias[b0:b0 + rows, :]
                    m = jnp.max(s, axis=-1, keepdims=True)
                    p = jnp.exp2(s - m)
                    l = jnp.sum(p, axis=-1, keepdims=True)
                    r = pl.reciprocal(l, approx=True)
                    r = r * (2.0 - l * r)
                    return (p * r).astype(BF16)

                def pv(p, v):
                    z = jnp.dot(p, v, preferred_element_type=F32)
                    return jnp.concatenate([z[rows - 2 * M:], z[:rows - 2 * M]], axis=0).astype(BF16)

                def wout(h, z):
                    return jnp.dot(z, pltpu.bitcast(wo[h], BF16), preferred_element_type=F32)

                def post1():
                    s = jnp.minimum(jnp.maximum(t - 1, 0), NSEG - 1)
                    r0 = pl.multiple_of(s * seg, seg)
                    x1 = x0[pl.ds(r0, seg), :].astype(F32) + ox[0:seg, :]
                    x2 = x1 + _ln(x1) * yb[pl.ds(r0, seg), :]
                    x2buf[t] = x2
                    hbuf[npar, XB:2 * XB, :] = _pack16(_ln(x2))

                def post2():
                    s = jnp.maximum(t - 1 - LAG, 0)
                    finish(s, pl.multiple_of(s * seg, seg))

                def pre1():
                    s = jnp.minimum(t + 1, NSEG - 1)
                    r0 = pl.multiple_of(s * seg, seg)
                    hbuf[npar, 0:XB, :] = _pack16(_ln(x0[pl.ds(r0, seg), :].astype(F32)))
                extra = {extras[0]: post1}
                if act2:
                    extra[extras[1]] = post2
                if act1 and act2:
                    extra[extras[2]] = pre1

                q, k, v, p, z = {}, {}, {}, {}, {}
                s_at = {h: h + lS for h in range(H)}
                p_at = {h: h + lP for h in range(H)}
                w_at = {h: h + lW for h in range(H)}
                for d, extra_lag in enumerate(tail):
                    p_at[H - 1 - d] += extra_lag
                fin = []
                accv = acc.at[0:rows]
                for i in range(max(w_at.values()) + 1):
                    for op in order:
                        if op == 'q' and i < H:
                            q[i] = proj(i, 0, False)
                        if op == 'k' and i < H:
                            k[i] = proj(i, 1, True)
                        if op == 'v' and i < H:
                            v[i] = proj(i, 2, True)
                        for h in range(H):
                            if op == 'S' and s_at[h] == i:
                                p[h] = scores(q.pop(h), k.pop(h))
                            if op == 'P' and p_at[h] == i:
                                z[h] = pv(p.pop(h), v.pop(h))
                            if op == 'W' and w_at[h] == i:
                                r = wout(h, z.pop(h))
                                if h == 0:
                                    accv[...] = r
                                elif h == H - 1:
                                    fin.append(accv[...] + r)
                                else:
                                    accv[...] += r
                    if i in extra:
                        extra[i]()
                assert not (q or k or v or p or z)
                a = fin[0]
                mp = _pack16(a[0:2 * M, :])
                if act2:
                    hbuf[npar, MO:MO + MB, :] = mp
                else:
                    hbuf[npar, MO:MO + MB // 2, :] = mp[0:MB // 2]
                    hbuf[npar, MO + MB // 2:MO + MB, :] = _pack16(mem0[...].astype(F32))
                if act1 and act2:
                    ox[...] = a[2 * M:R, :]
                elif act1:
                    ox[0:seg, :] = a[2 * M:, :]
                else:
                    ox[seg:2 * seg, :] = a[2 * M:, :]
            return step

        def run_steps(t0, t1, step, unroll=1):
            if unroll == 1:
                lax.fori_loop(t0, t1, lambda t, c: step(t, t & 1), None)
                return
            assert unroll % 2 == 0 and (t1 - t0) % unroll == 0

            def body(i, c):
                for u in range(unroll):
                    step(t0 + i * unroll + u, (t0 + u) & 1)
            lax.fori_loop(0, (t1 - t0) // unroll, body, None)

        run_steps(0, LAG, make_step(True, False, True))
        c_xb.wait()
        nboth = nsteps - LAG
        run_steps(LAG, min(NS, nboth), make_step(True, True, True))
        if nboth > NS:
            run_steps(NS, nboth, make_step(True, True, False), cfg.get("unroll", 2))
        OA = (NSEG - LAG - 1) * seg
        c_oa = pltpu.make_async_copy(ob.at[pl.ds(0, OA)], o_hbm.at[pl.ds(0, OA)], sem_out.at[0])
        c_oa.start()
        run_steps(NSEG, NSEG + LAG, make_step(False, True, False))
        finish(NSEG - 1, (NSEG - 1) * seg)
        c_ob = pltpu.make_async_copy(ob.at[pl.ds(OA, S - OA)], o_hbm.at[pl.ds(OA, S - OA)],
                                     sem_out.at[1])
        c_ob.start()
        c_oa.wait()
        c_ob.wait()

    scratch = [
        pltpu.VMEM((3, H, Dm // 2, Dh), U32),
        pltpu.VMEM((3, HP, Dm, Dh), U32),
        pltpu.VMEM((H, Dh // 2, Dm), U32),
        pltpu.VMEM((S, Dm), BF16),
        pltpu.VMEM((KPAD + S, Dm), BF16),
        pltpu.VMEM((S, Dm), BF16),
        pltpu.VMEM((NCH, Dm, CH), BF16),
        pltpu.VMEM((S, Dm), BF16),
        pltpu.VMEM((NCH, 2 * CH, Dm), F32),
        pltpu.VMEM((NCH, 2 * CH, Dm), F32),
        pltpu.VMEM((2 * CH, Dm), F32),
        pltpu.VMEM((S, Dm), F32),
        pltpu.VMEM((2, R // 2, Dm), U32),
        pltpu.VMEM((NS * seg // 2, Dm), U32),
        pltpu.VMEM((3, H, NS * seg, Dh), F32),
        pltpu.VMEM((R, Dm), F32),
        pltpu.VMEM((NSEG + LAG + 1, seg, Dm), F32),
        pltpu.VMEM((2 * seg, Dm), F32),
        pltpu.VMEM((S, Dm), BF16),
        pltpu.VMEM((2 * CH, CH), BF16),
        pltpu.VMEM((CH, 2 * CH), BF16),
        pltpu.VMEM((R + 2 * (2 * M + seg), 128), F32),
        pltpu.VMEM((M, Dm), BF16),
        pltpu.VMEM((KS, Dm), BF16),
        pltpu.VMEM((Dm,), BF16),
        pltpu.SemaphoreType.DMA((6,)),
        pltpu.SemaphoreType.DMA((NCH,)),
        pltpu.SemaphoreType.DMA((NCH,)),
        pltpu.SemaphoreType.DMA((NCH,)),
        pltpu.SemaphoreType.DMA((3, HP)),
        pltpu.SemaphoreType.DMA((4,)),
        pltpu.SemaphoreType.DMA((2,)),
        pltpu.SemaphoreType.DMA((2,)),
    ]
    return kernel, scratch


def _run(A_x, A_mem0, A_Wq, A_Wk, A_Wv, A_Wo, A_seg_len, B_k, B_v, B_shift_k, B_ssm_k, B_ssm_D,
         cfg=None):
    B, S, Dm = A_x.shape
    assert B == 1
    _, H, Dh = A_Wq.shape
    M = A_mem0.shape[1]
    seg = int(A_seg_len)
    KS = B_shift_k.shape[-1]
    kernel, scratch = _build(S, Dm, H, Dh, M, seg, KS, cfg or {})
    fa_np, fi_np = _dft_mats()
    bias_np = _attn_bias(M, seg)
    args = (A_x.reshape(S, Dm), A_mem0.reshape(M, Dm), A_Wq, A_Wk, A_Wv, A_Wo,
            B_k.reshape(S, Dm), B_v.reshape(S, Dm), B_shift_k.T, B_ssm_k, B_ssm_D,
            fa_np, fi_np, bias_np)
    out = pl.pallas_call(
        kernel,
        out_shape=jax.ShapeDtypeStruct((S, Dm), BF16),
        in_specs=[pl.BlockSpec(memory_space=pl.ANY)] * len(args),
        out_specs=pl.BlockSpec(memory_space=pl.ANY),
        scratch_shapes=scratch,
        compiler_params=pltpu.CompilerParams(vmem_limit_bytes=110 * 1024 * 1024,
                                             flags=(cfg or {}).get("flags")),
    )(*args)
    return out.reshape(B, S, Dm)


@functools.partial(jax.jit, static_argnames=("A_seg_len",))
def pallas_interleave_layers__memory_aug_recurrent_mem_tr__ssm_conv_h3__prompt_kernel(
    A_x: jax.Array,
    A_mem0: jax.Array,
    A_Wq: jax.Array,
    A_Wk: jax.Array,
    A_Wv: jax.Array,
    A_Wo: jax.Array,
    A_seg_len: int,
    B_q: jax.Array,
    B_k: jax.Array,
    B_v: jax.Array,
    B_shift_k: jax.Array,
    B_ssm_k: jax.Array,
    B_ssm_D: jax.Array,
):
    del B_q
    return _run(A_x, A_mem0, A_Wq, A_Wk, A_Wv, A_Wo, A_seg_len, B_k, B_v, B_shift_k,
                B_ssm_k, B_ssm_D)
```

```python
import functools

import jax
import jax.numpy as jnp
import numpy as np
from jax import lax
from jax.experimental import pallas as pl
from jax.experimental.pallas import tpu as pltpu

F32, BF16, U32 = jnp.float32, jnp.bfloat16, jnp.uint32

LOG2E = 1.4426950408889634
LN_EPS = 1e-5
CH = 128
LAG = 2
KPAD = 16


def _np_bf16(a):
    return np.asarray(a, dtype=np.float32).astype(BF16)


def _dft_mats():
    n2 = 2 * CH
    karr = np.concatenate([np.arange(0, CH, 2), np.arange(1, CH, 2)])
    n = np.arange(CH)
    th = 2.0 * np.pi * n[None, :] * (karr[:, None] + 0.5) / n2
    fa = np.concatenate([np.cos(th), -np.sin(th)], axis=0)
    fi = np.concatenate([np.cos(th).T, -np.sin(th).T], axis=1) * (2.0 / n2)
    return _np_bf16(fa), _np_bf16(fi)


def _attn_bias(m, seg):
    stream = np.concatenate([np.zeros(seg), np.ones(seg), np.zeros(m), np.ones(m)])
    ismem = np.concatenate([np.zeros(2 * seg), np.ones(2 * m)]).astype(bool)
    pos = np.concatenate([np.arange(seg), np.arange(seg), np.zeros(2 * m)])
    same = stream[:, None] == stream[None, :]
    keep = ismem[:, None] | ismem[None, :] | (pos[:, None] >= pos[None, :])
    full = np.where(same & keep, 0.0, np.where(same, -1e9 * LOG2E, -1e30))
    s1, s2, mm = np.arange(seg), np.arange(seg, 2 * seg), np.arange(2 * seg, 2 * seg + 2 * m)
    out = []
    for sel in (np.concatenate([s1, s2, mm]), np.concatenate([s1, mm]), np.concatenate([s2, mm])):
        b = np.full((len(sel), 128), -1e30, np.float32)
        b[:, :len(sel)] = full[sel][:, sel]
        out.append(b)
    return np.concatenate(out, axis=0)


def _ln(x):
    m = jnp.mean(x, axis=-1, keepdims=True)
    xc = x - m
    v = jnp.mean(xc * xc, axis=-1, keepdims=True)
    return xc * lax.rsqrt(v + LN_EPS)


def _pack16(x):
    return pltpu.bitcast(x.astype(BF16), U32)


def _build(S, Dm, H, Dh, M, seg, KS, cfg):
    assert Dh == 128 and Dm % 128 == 0 and S % CH == 0 and H % 16 == 0
    assert M == 8 and seg == 32 and KS <= 8
    NSEG = S // seg
    NCH = S // CH
    NT = Dm // 128
    R = 2 * (M + seg)
    HP = H // 2
    qk_scale = float(Dh ** -0.5) * LOG2E
    LAGS = {"b": (2, 4, 12, (3, 2, 1)), "bp": (2, 4, 12, (3, 2, 1, 1)), "1": (2, 5, 14, (4, 3, 2, 1)),
            "2": (2, 4, 12, (4, 3, 2, 1))}
    order = cfg.get("order", "qSkPvW")
    extras = cfg.get("extras", (3, 11, 19))
    nsteps = cfg.get("nsteps", NSEG + LAG)
    skip = cfg.get("skip", "")
    NS = cfg.get("ns", 6)
    assert LAG < NS <= NSEG - 1

    def kernel(x_hbm, mem0_hbm, wq_hbm, wk_hbm, wv_hbm, wo_hbm, k_hbm, v_hbm, sh_hbm, h_hbm,
               d_hbm, fa_hbm, fi_hbm, bias_hbm, o_hbm,
               wqkv, wstage, wo, x0, kb, vb, hb, ub, Ub, Gb, Ap, yb,
               hbuf, hx, qkvx, acc, x2buf, ox, ob, fa, fi, bias, mem0, shv, dv,
               sem_c, sem_k, sem_v, sem_h, sem_w, sem_o, sem_x, sem_out):
        c_fa = pltpu.make_async_copy(fa_hbm, fa, sem_c.at[0])
        c_sh = pltpu.make_async_copy(sh_hbm, shv, sem_c.at[1])
        c_fi = pltpu.make_async_copy(fi_hbm, fi, sem_c.at[2])
        c_d = pltpu.make_async_copy(d_hbm, dv, sem_c.at[3])
        c_bias = pltpu.make_async_copy(bias_hbm, bias, sem_c.at[4])
        c_mem0 = pltpu.make_async_copy(mem0_hbm, mem0, sem_c.at[5])

        def cp_k(j):
            return pltpu.make_async_copy(
                k_hbm.at[pl.ds(j * CH, CH)], kb.at[pl.ds(KPAD + j * CH, CH)], sem_k.at[j])

        def cp_v(j):
            return pltpu.make_async_copy(
                v_hbm.at[pl.ds(j * CH, CH)], vb.at[pl.ds(j * CH, CH)], sem_v.at[j])

        def cp_h(j):
            return pltpu.make_async_copy(
                h_hbm.at[:, pl.ds(j * CH, CH)], hb.at[j], sem_h.at[j])

        w32 = [w.bitcast(U32) for w in (wq_hbm, wk_hbm, wv_hbm)]

        def cp_w(j, s):
            return pltpu.make_async_copy(w32[j].at[:, s, :], wstage.at[j, s], sem_w.at[j, s])

        wo32 = wo_hbm.bitcast(U32)
        NWO = 4
        c_wo = [pltpu.make_async_copy(wo32.at[pl.ds(i * (H // NWO), H // NWO)],
                                      wo.at[pl.ds(i * (H // NWO), H // NWO)], sem_o.at[i])
                for i in range(NWO)]
        XA = NS * seg
        c_xa = pltpu.make_async_copy(x_hbm.at[pl.ds(0, XA)], x0.at[pl.ds(0, XA)], sem_x.at[0])
        c_xb = pltpu.make_async_copy(x_hbm.at[pl.ds(XA, S - XA)], x0.at[pl.ds(XA, S - XA)],
                                     sem_x.at[1])

        WIN = cfg.get("win", 4)
        WST = cfg.get("wst", NCH - 4)
        WW = cfg.get("ww", 3)

        def start_chunk(j):
            cp_k(j).start()
            cp_v(j).start()
            cp_h(j).start()

        def start_slab(s):
            for j in range(3):
                cp_w(j, s).start()

        start_chunk(0)
        c_fa.start()
        c_sh.start()
        for j in range(1, WIN):
            start_chunk(j)
        c_fi.start()
        c_d.start()
        c_bias.start()
        c_mem0.start()
        c_xa.start()

        kb[0:KPAD, :] = jnp.zeros((KPAD, Dm), BF16)
        Ap[...] = jnp.zeros(Ap.shape, F32)
        c_fa.wait()
        c_sh.wait()
        sh = shv[...].astype(F32)

        def fwd(j, carry):
            cp_k(j).wait()
            cp_v(j).wait()
            cp_h(j).wait()

            @pl.when(j + WIN < NCH)
            def _():
                start_chunk(j + WIN)

            @pl.when(j >= WST)
            def _():
                @pl.when(j < WST + WW)
                def _():
                    start_slab(j - WST)
            r0 = pl.multiple_of(j * CH, CH)
            kf = kb[pl.ds(r0, CH + KPAD), :].astype(F32)
            ks = kf[KPAD:KPAD + CH] * sh[0:1]
            for dlt in range(1, KS):
                ks = ks + kf[KPAD - dlt:KPAD - dlt + CH] * sh[dlt:dlt + 1]
            u = (ks * vb[pl.ds(r0, CH), :].astype(F32)).astype(BF16)
            ub[pl.ds(r0, CH), :] = u
            fav = fa[...]
            Ub[j] = jnp.dot(fav, u, preferred_element_type=F32)
            a = lax.dot_general(fav, hb[j], (((1,), (1,)), ((), ())),
                                preferred_element_type=F32)
            p = Ap[...]
            hh = CH // 2
            Gb[j, 0:hh] = a[0:hh] - p[CH:CH + hh]
            Gb[j, hh:CH] = a[hh:CH] + p[CH + hh:2 * CH]
            Gb[j, CH:CH + hh] = a[CH:CH + hh] + p[0:hh]
            Gb[j, CH + hh:2 * CH] = a[CH + hh:2 * CH] - p[hh:CH]
            Ap[...] = a
            return carry
        lax.fori_loop(0, NCH, fwd, 0)

        BL = cfg.get("bl", 4)
        MCH = cfg.get("mch", 64)

        c_xa.wait()
        for i in range(NS):
            hx[i * seg // 2:(i + 1) * seg // 2, :] = _pack16(
                _ln(x0[i * seg:(i + 1) * seg, :].astype(F32)))

        def repack(s, j):
            a = wstage[j, s, pl.ds(0, Dm // 2, stride=2), :]
            b = wstage[j, s, pl.ds(1, Dm // 2, stride=2), :]
            wqkv[j, 2 * s] = (a & jnp.uint32(0xFFFF)) | (b << 16)
            wqkv[j, 2 * s + 1] = (a >> 16) | (b & jnp.uint32(0xFFFF0000))

        def run_ahead(s, j, hh, m0):
            w = pltpu.bitcast(wqkv[j, 2 * s + hh], BF16)
            lhs = pltpu.bitcast(hx[m0 // 2:(m0 + MCH) // 2, :], BF16)
            qkvx[j, 2 * s + hh, m0:m0 + MCH, :] = jnp.dot(lhs, w, preferred_element_type=F32)

        assert HP == CH // 8

        def mac(f, carry):
            for j in range(3):
                cp_w(j, f).wait()

            @pl.when(f + WW < HP)
            def _():
                start_slab(f + WW)

            @pl.when(f + WW == HP)
            def _():
                for c in c_wo:
                    c.start()
            rr = pl.multiple_of(f * 8, 8)
            ri = pl.multiple_of(CH + f * 8, 8)

            def mac_gen(c, ib):
                cs = slice(c * 128, (c + 1) * 128)
                yr = [None] * BL
                yi = [None] * BL
                for jb in range(ib + 1):
                    for jj in range(BL):
                        J = jb * BL + jj
                        ur = Ub[J, pl.ds(rr, 8), cs]
                        ui = Ub[J, pl.ds(ri, 8), cs]
                        n = 0
                        for ii in range(BL):
                            I = ib * BL + ii
                            if I < J:
                                continue
                            gr = Gb[I - J, pl.ds(rr, 8), cs]
                            gi = Gb[I - J, pl.ds(ri, 8), cs]
                            tr = gr * ur - gi * ui
                            ti = gr * ui + gi * ur
                            yr[ii] = tr if yr[ii] is None else yr[ii] + tr
                            yi[ii] = ti if yi[ii] is None else yi[ii] + ti
                            n += 1
                        yield n
                for ii in range(BL):
                    Ub[ib * BL + ii, pl.ds(rr, 8), cs] = yr[ii]
                    Ub[ib * BL + ii, pl.ds(ri, 8), cs] = yi[ii]
                yield 0

            def vpu_stream():
                for c in range(NT if 'm' not in skip else 0):
                    for ib in reversed(range(NCH // BL)):
                        yield from mac_gen(c, ib)
            vpu = vpu_stream()
            tot = NT * NCH * (NCH + 1) // 2
            mxu = []
            for j in range(3):
                mxu.append(((repack, f, j), 0))
                for hh in range(2):
                    for m0 in range(0, NS * seg, MCH):
                        mxu.append(((run_ahead, f, j, hh, m0), 1))
            nm = sum(w for _, w in mxu)
            done = dm = 0
            gran = cfg.get("gran", 1)
            for (fn, *args), w in mxu:
                fn(*args)
                dm += w
                while done < tot * dm / nm:
                    n = next(vpu, None)
                    if n is None:
                        break
                    done += n
            for _ in vpu:
                pass
            return carry
        lax.fori_loop(0, CH // 8, mac, 0)

        c_fi.wait()
        c_d.wait()
        dvec = dv[...].astype(F32).reshape(1, Dm)

        def inv(i, carry):
            r0 = pl.multiple_of(i * CH, CH)
            y = jnp.dot(fi[...], Ub[i].astype(BF16), preferred_element_type=F32)
            yb[pl.ds(r0, CH), :] = y + ub[pl.ds(r0, CH), :].astype(F32) * dvec
            return carry
        if 'i' not in skip:
            lax.fori_loop(0, NCH, inv, 0)

        hbuf[...] = jnp.zeros(hbuf.shape, U32)
        x2buf[0] = jnp.zeros(x2buf.shape[1:], F32)
        ox[...] = jnp.zeros(ox.shape, F32)
        c_bias.wait()
        c_mem0.wait()
        for c in c_wo:
            c.wait()
        c_xb.start()
        MB = M
        XB = seg // 2
        MO = 2 * XB
        hbuf[0, MO:MO + MB // 2, :] = _pack16(mem0[...].astype(F32))

        def finish(s, r0):
            x3 = x2buf[s + 1] + ox[seg:2 * seg, :]
            x4 = x3 + _ln(x3) * yb[pl.ds(r0, seg), :]
            ob[pl.ds(r0, seg), :] = x4.astype(BF16)

        def make_step(act1, act2, pre):
            rows = 2 * M + seg * (int(act1) + int(act2))
            b0 = 0 if (act1 and act2) else R if act1 else R + 2 * M + seg
            x1_in_lhs = act1 and not pre

            key = "b" if (act1 and act2 and not pre) else "bp" if (act1 and act2) else "1" if act1 else "2"
            lS, lP, lW, tail = cfg.get("lag_" + key, LAGS[key])

            def step(t, par):
                npar = 1 - par
                parts = []
                if x1_in_lhs:
                    parts.append(hbuf[par, 0:XB, :])
                if act2:
                    parts.append(hbuf[par, XB:2 * XB, :])
                parts.append(hbuf[par, MO:MO + MB, :])
                hh = pltpu.bitcast(parts[0] if len(parts) == 1 else jnp.concatenate(parts, axis=0), BF16)
                zpad = jnp.zeros((128 - rows, Dh), F32)

                def proj(h, j, padded):
                    r = jnp.dot(hh, pltpu.bitcast(wqkv[j, h], BF16), preferred_element_type=F32)
                    blocks = [r]
                    if pre:
                        x1p = qkvx[j, h, pl.ds(pl.multiple_of(t * seg, seg), seg), :]
                        blocks = [x1p, r]
                    if padded:
                        blocks.append(zpad)
                    u = blocks[0] if len(blocks) == 1 else jnp.concatenate(blocks, axis=0)
                    return u.astype(BF16)

                def scores(q, k):
                    s = lax.dot_general(q, k, (((1,), (1,)), ((), ())), preferred_element_type=F32)
                    s = s * qk_scale + bias[b0:b0 + rows, :]
                    m = jnp.max(s, axis=-1, keepdims=True)
                    p = jnp.exp2(s - m)
                    l = jnp.sum(p, axis=-1, keepdims=True)
                    r = pl.reciprocal(l, approx=True)
                    r = r * (2.0 - l * r)
                    return (p * r).astype(BF16)

                def pv(p, v):
                    z = jnp.dot(p, v, preferred_element_type=F32)
                    return jnp.concatenate([z[rows - 2 * M:], z[:rows - 2 * M]], axis=0).astype(BF16)

                def wout(h, z):
                    return jnp.dot(z, pltpu.bitcast(wo[h], BF16), preferred_element_type=F32)

                def post1():
                    s = jnp.minimum(jnp.maximum(t - 1, 0), NSEG - 1)
                    r0 = pl.multiple_of(s * seg, seg)
                    x1 = x0[pl.ds(r0, seg), :].astype(F32) + ox[0:seg, :]
                    x2 = x1 + _ln(x1) * yb[pl.ds(r0, seg), :]
                    x2buf[t] = x2
                    hbuf[npar, XB:2 * XB, :] = _pack16(_ln(x2))

                def post2():
                    s = jnp.maximum(t - 1 - LAG, 0)
                    finish(s, pl.multiple_of(s * seg, seg))

                def pre1():
                    s = jnp.minimum(t + 1, NSEG - 1)
                    r0 = pl.multiple_of(s * seg, seg)
                    hbuf[npar, 0:XB, :] = _pack16(_ln(x0[pl.ds(r0, seg), :].astype(F32)))
                extra = {extras[0]: post1}
                if act2:
                    extra[extras[1]] = post2
                if act1 and act2:
                    extra[extras[2]] = pre1

                q, k, v, p, z = {}, {}, {}, {}, {}
                s_at = {h: h + lS for h in range(H)}
                p_at = {h: h + lP for h in range(H)}
                w_at = {h: h + lW for h in range(H)}
                for d, extra_lag in enumerate(tail):
                    p_at[H - 1 - d] += extra_lag
                fin = []
                accv = acc.at[0:rows]
                for i in range(max(w_at.values()) + 1):
                    for op in order:
                        if op == 'q' and i < H:
                            q[i] = proj(i, 0, False)
                        if op == 'k' and i < H:
                            k[i] = proj(i, 1, True)
                        if op == 'v' and i < H:
                            v[i] = proj(i, 2, True)
                        for h in range(H):
                            if op == 'S' and s_at[h] == i:
                                p[h] = scores(q.pop(h), k.pop(h))
                            if op == 'P' and p_at[h] == i:
                                z[h] = pv(p.pop(h), v.pop(h))
                            if op == 'W' and w_at[h] == i:
                                r = wout(h, z.pop(h))
                                if h == 0:
                                    accv[...] = r
                                elif h == H - 1:
                                    fin.append(accv[...] + r)
                                else:
                                    accv[...] += r
                    if i in extra:
                        extra[i]()
                assert not (q or k or v or p or z)
                a = fin[0]
                mp = _pack16(a[0:2 * M, :])
                if act2:
                    hbuf[npar, MO:MO + MB, :] = mp
                else:
                    hbuf[npar, MO:MO + MB // 2, :] = mp[0:MB // 2]
                    hbuf[npar, MO + MB // 2:MO + MB, :] = _pack16(mem0[...].astype(F32))
                if act1 and act2:
                    ox[...] = a[2 * M:R, :]
                elif act1:
                    ox[0:seg, :] = a[2 * M:, :]
                else:
                    ox[seg:2 * seg, :] = a[2 * M:, :]
            return step

        def run_steps(t0, t1, step, unroll=1):
            if unroll == 1:
                lax.fori_loop(t0, t1, lambda t, c: step(t, t & 1), None)
                return
            assert unroll % 2 == 0 and (t1 - t0) % unroll == 0

            def body(i, c):
                for u in range(unroll):
                    step(t0 + i * unroll + u, (t0 + u) & 1)
            lax.fori_loop(0, (t1 - t0) // unroll, body, None)

        run_steps(0, LAG, make_step(True, False, True))
        c_xb.wait()
        nboth = nsteps - LAG
        run_steps(LAG, min(NS, nboth), make_step(True, True, True))
        if nboth > NS:
            run_steps(NS, nboth, make_step(True, True, False), cfg.get("unroll", 2))
        OA = (NSEG - LAG - 1) * seg
        c_oa = pltpu.make_async_copy(ob.at[pl.ds(0, OA)], o_hbm.at[pl.ds(0, OA)], sem_out.at[0])
        c_oa.start()
        run_steps(NSEG, NSEG + LAG, make_step(False, True, False))
        finish(NSEG - 1, (NSEG - 1) * seg)
        c_ob = pltpu.make_async_copy(ob.at[pl.ds(OA, S - OA)], o_hbm.at[pl.ds(OA, S - OA)],
                                     sem_out.at[1])
        c_ob.start()
        c_oa.wait()
        c_ob.wait()

    scratch = [
        pltpu.VMEM((3, H, Dm // 2, Dh), U32),
        pltpu.VMEM((3, HP, Dm, Dh), U32),
        pltpu.VMEM((H, Dh // 2, Dm), U32),
        pltpu.VMEM((S, Dm), BF16),
        pltpu.VMEM((KPAD + S, Dm), BF16),
        pltpu.VMEM((S, Dm), BF16),
        pltpu.VMEM((NCH, Dm, CH), BF16),
        pltpu.VMEM((S, Dm), BF16),
        pltpu.VMEM((NCH, 2 * CH, Dm), F32),
        pltpu.VMEM((NCH, 2 * CH, Dm), F32),
        pltpu.VMEM((2 * CH, Dm), F32),
        pltpu.VMEM((S, Dm), F32),
        pltpu.VMEM((2, R // 2, Dm), U32),
        pltpu.VMEM((NS * seg // 2, Dm), U32),
        pltpu.VMEM((3, H, NS * seg, Dh), F32),
        pltpu.VMEM((R, Dm), F32),
        pltpu.VMEM((NSEG + LAG + 1, seg, Dm), F32),
        pltpu.VMEM((2 * seg, Dm), F32),
        pltpu.VMEM((S, Dm), BF16),
        pltpu.VMEM((2 * CH, CH), BF16),
        pltpu.VMEM((CH, 2 * CH), BF16),
        pltpu.VMEM((R + 2 * (2 * M + seg), 128), F32),
        pltpu.VMEM((M, Dm), BF16),
        pltpu.VMEM((KS, Dm), BF16),
        pltpu.VMEM((Dm,), BF16),
        pltpu.SemaphoreType.DMA((6,)),
        pltpu.SemaphoreType.DMA((NCH,)),
        pltpu.SemaphoreType.DMA((NCH,)),
        pltpu.SemaphoreType.DMA((NCH,)),
        pltpu.SemaphoreType.DMA((3, HP)),
        pltpu.SemaphoreType.DMA((4,)),
        pltpu.SemaphoreType.DMA((2,)),
        pltpu.SemaphoreType.DMA((2,)),
    ]
    return kernel, scratch


def _run(A_x, A_mem0, A_Wq, A_Wk, A_Wv, A_Wo, A_seg_len, B_k, B_v, B_shift_k, B_ssm_k, B_ssm_D,
         cfg=None):
    B, S, Dm = A_x.shape
    assert B == 1
    _, H, Dh = A_Wq.shape
    M = A_mem0.shape[1]
    seg = int(A_seg_len)
    KS = B_shift_k.shape[-1]
    kernel, scratch = _build(S, Dm, H, Dh, M, seg, KS, cfg or {})
    fa_np, fi_np = _dft_mats()
    bias_np = _attn_bias(M, seg)
    args = (A_x.reshape(S, Dm), A_mem0.reshape(M, Dm), A_Wq, A_Wk, A_Wv, A_Wo,
            B_k.reshape(S, Dm), B_v.reshape(S, Dm), B_shift_k.T, B_ssm_k, B_ssm_D,
            fa_np, fi_np, bias_np)
    out = pl.pallas_call(
        kernel,
        out_shape=jax.ShapeDtypeStruct((S, Dm), BF16),
        in_specs=[pl.BlockSpec(memory_space=pl.ANY)] * len(args),
        out_specs=pl.BlockSpec(memory_space=pl.ANY),
        scratch_shapes=scratch,
        compiler_params=pltpu.CompilerParams(vmem_limit_bytes=110 * 1024 * 1024,
                                             flags=(cfg or {}).get("flags")),
    )(*args)
    return out.reshape(B, S, Dm)


@functools.partial(jax.jit, static_argnames=("A_seg_len",))
def pallas_interleave_layers__memory_aug_recurrent_mem_tr__ssm_conv_h3__prompt_kernel(
    A_x: jax.Array,
    A_mem0: jax.Array,
    A_Wq: jax.Array,
    A_Wk: jax.Array,
    A_Wv: jax.Array,
    A_Wo: jax.Array,
    A_seg_len: int,
    B_q: jax.Array,
    B_k: jax.Array,
    B_v: jax.Array,
    B_shift_k: jax.Array,
    B_ssm_k: jax.Array,
    B_ssm_D: jax.Array,
):
    del B_q
    return _run(A_x, A_mem0, A_Wq, A_Wk, A_Wv, A_Wo, A_seg_len, B_k, B_v, B_shift_k,
                B_ssm_k, B_ssm_D)
```

```python
import functools

import jax
import jax.numpy as jnp
import numpy as np
from jax import lax
from jax.experimental import pallas as pl
from jax.experimental.pallas import tpu as pltpu

F32, BF16, U32 = jnp.float32, jnp.bfloat16, jnp.uint32

LOG2E = 1.4426950408889634
LN_EPS = 1e-5
CH = 128
LAG = 2
KPAD = 16


def _np_bf16(a):
    return np.asarray(a, dtype=np.float32).astype(BF16)


def _dft_mats():
    n2 = 2 * CH
    karr = np.concatenate([np.arange(0, CH, 2), np.arange(1, CH, 2)])
    n = np.arange(CH)
    th = 2.0 * np.pi * n[None, :] * (karr[:, None] + 0.5) / n2
    fa = np.concatenate([np.cos(th), -np.sin(th)], axis=0)
    fi = np.concatenate([np.cos(th).T, -np.sin(th).T], axis=1) * (2.0 / n2)
    return _np_bf16(fa), _np_bf16(fi)


def _attn_bias(m, seg):
    stream = np.concatenate([np.zeros(seg), np.ones(seg), np.zeros(m), np.ones(m)])
    ismem = np.concatenate([np.zeros(2 * seg), np.ones(2 * m)]).astype(bool)
    pos = np.concatenate([np.arange(seg), np.arange(seg), np.zeros(2 * m)])
    same = stream[:, None] == stream[None, :]
    keep = ismem[:, None] | ismem[None, :] | (pos[:, None] >= pos[None, :])
    full = np.where(same & keep, 0.0, np.where(same, -1e9 * LOG2E, -1e30))
    s1, s2, mm = np.arange(seg), np.arange(seg, 2 * seg), np.arange(2 * seg, 2 * seg + 2 * m)
    out = []
    for sel in (np.concatenate([s1, s2, mm]), np.concatenate([s1, mm]), np.concatenate([s2, mm])):
        b = np.full((len(sel), 128), -1e30, np.float32)
        b[:, :len(sel)] = full[sel][:, sel]
        out.append(b)
    return np.concatenate(out, axis=0)


def _ln(x):
    m = jnp.mean(x, axis=-1, keepdims=True)
    xc = x - m
    v = jnp.mean(xc * xc, axis=-1, keepdims=True)
    return xc * lax.rsqrt(v + LN_EPS)


def _pack16(x):
    return pltpu.bitcast(x.astype(BF16), U32)


def _build(S, Dm, H, Dh, M, seg, KS, cfg):
    assert Dh == 128 and Dm % 128 == 0 and S % CH == 0 and H % 16 == 0
    assert M == 8 and seg == 32 and KS <= 8
    NSEG = S // seg
    NCH = S // CH
    NT = Dm // 128
    R = 2 * (M + seg)
    HP = H // 2
    qk_scale = float(Dh ** -0.5) * LOG2E
    LAGS = {"b": (2, 4, 12, (3, 2, 1)), "bp": (2, 4, 12, (3, 2, 1, 1)), "1": (2, 4, 12, (4, 3, 2, 1)),
            "2": (2, 4, 12, (4, 3, 2, 1))}
    order = cfg.get("order", "qSkPvW")
    extras = cfg.get("extras", (3, 11, 19))
    nsteps = cfg.get("nsteps", NSEG + LAG)
    skip = cfg.get("skip", "")
    NS = cfg.get("ns", 6)
    assert 0 < NS and LAG + NS <= NSEG - 1

    import contextlib
    scope = jax.named_scope if cfg.get("scopes") else (lambda n: contextlib.nullcontext())

    def kernel(x_hbm, mem0_hbm, wq_hbm, wk_hbm, wv_hbm, wo_hbm, k_hbm, v_hbm, sh_hbm, h_hbm,
               d_hbm, fa_hbm, fi_hbm, bias_hbm, o_hbm,
               wqkv, wstage, wo, x0, kb, vb, hb, ub, Ub, Gb, Ap, yb,
               hbuf, hx, qkvx, acc, x2buf, ox, ob, fa, fi, bias, mem0, shv, dv,
               sem_c, sem_k, sem_v, sem_h, sem_w, sem_o, sem_x, sem_out):
        c_fa = pltpu.make_async_copy(fa_hbm, fa, sem_c.at[0])
        c_sh = pltpu.make_async_copy(sh_hbm, shv, sem_c.at[1])
        c_fi = pltpu.make_async_copy(fi_hbm, fi, sem_c.at[2])
        c_d = pltpu.make_async_copy(d_hbm, dv, sem_c.at[3])
        c_bias = pltpu.make_async_copy(bias_hbm, bias, sem_c.at[4])
        c_mem0 = pltpu.make_async_copy(mem0_hbm, mem0, sem_c.at[5])

        def cp_k(j):
            return pltpu.make_async_copy(
                k_hbm.at[pl.ds(j * CH, CH)], kb.at[pl.ds(KPAD + j * CH, CH)], sem_k.at[j])

        def cp_v(j):
            return pltpu.make_async_copy(
                v_hbm.at[pl.ds(j * CH, CH)], vb.at[pl.ds(j * CH, CH)], sem_v.at[j])

        def cp_h(j):
            return pltpu.make_async_copy(
                h_hbm.at[:, pl.ds(j * CH, CH)], hb.at[j], sem_h.at[j])

        w32 = [w.bitcast(U32) for w in (wq_hbm, wk_hbm, wv_hbm)]

        def cp_w(j, s):
            return pltpu.make_async_copy(w32[j].at[:, s, :], wstage.at[j, s], sem_w.at[j, s])

        wo32 = wo_hbm.bitcast(U32)
        NWO = 4
        c_wo = [pltpu.make_async_copy(wo32.at[pl.ds(i * (H // NWO), H // NWO)],
                                      wo.at[pl.ds(i * (H // NWO), H // NWO)], sem_o.at[i])
                for i in range(NWO)]
        XA = (LAG + NS) * seg
        c_xa = pltpu.make_async_copy(x_hbm.at[pl.ds(0, XA)], x0.at[pl.ds(0, XA)], sem_x.at[0])
        c_xb = pltpu.make_async_copy(x_hbm.at[pl.ds(XA, S - XA)], x0.at[pl.ds(XA, S - XA)],
                                     sem_x.at[1])

        WIN = cfg.get("win", 4)
        WST = cfg.get("wst", NCH - 4)
        WW = cfg.get("ww", 3)

        def start_chunk(j):
            cp_k(j).start()
            cp_v(j).start()
            cp_h(j).start()

        def start_slab(s):
            for j in range(3):
                cp_w(j, s).start()

        start_chunk(0)
        c_fa.start()
        c_sh.start()
        for j in range(1, WIN):
            start_chunk(j)
        c_fi.start()
        c_d.start()
        c_bias.start()
        c_mem0.start()
        c_xa.start()

        kb[0:KPAD, :] = jnp.zeros((KPAD, Dm), BF16)
        Ap[...] = jnp.zeros(Ap.shape, F32)
        with scope('wait_fa'):
            c_fa.wait()
        c_sh.wait()
        sh = shv[...].astype(F32)

        def fwd(j, carry):
            cp_k(j).wait()
            cp_v(j).wait()
            cp_h(j).wait()

            @pl.when(j + WIN < NCH)
            def _():
                start_chunk(j + WIN)

            @pl.when(j >= WST)
            def _():
                @pl.when(j < WST + WW)
                def _():
                    start_slab(j - WST)
            r0 = pl.multiple_of(j * CH, CH)
            kf = kb[pl.ds(r0, CH + KPAD), :].astype(F32)
            ks = kf[KPAD:KPAD + CH] * sh[0:1]
            for dlt in range(1, KS):
                ks = ks + kf[KPAD - dlt:KPAD - dlt + CH] * sh[dlt:dlt + 1]
            u = (ks * vb[pl.ds(r0, CH), :].astype(F32)).astype(BF16)
            ub[pl.ds(r0, CH), :] = u
            fav = fa[...]
            Ub[j] = jnp.dot(fav, u, preferred_element_type=F32)
            a = lax.dot_general(fav, hb[j], (((1,), (1,)), ((), ())),
                                preferred_element_type=F32)
            p = Ap[...]
            hh = CH // 2
            Gb[j, 0:hh] = a[0:hh] - p[CH:CH + hh]
            Gb[j, hh:CH] = a[hh:CH] + p[CH + hh:2 * CH]
            Gb[j, CH:CH + hh] = a[CH:CH + hh] + p[0:hh]
            Gb[j, CH + hh:2 * CH] = a[CH + hh:2 * CH] - p[hh:CH]
            Ap[...] = a
            return carry
        with scope('fwd'):
            lax.fori_loop(0, NCH, fwd, 0)

        BL = cfg.get("bl", 4)
        MCH = cfg.get("mch", 64)

        with scope('wait_xa'):
            c_xa.wait()
        for i in range(NS):
            hx[i * seg // 2:(i + 1) * seg // 2, :] = _pack16(
                _ln(x0[(LAG + i) * seg:(LAG + i + 1) * seg, :].astype(F32)))

        def repack(s, j):
            a = wstage[j, s, pl.ds(0, Dm // 2, stride=2), :]
            b = wstage[j, s, pl.ds(1, Dm // 2, stride=2), :]
            wqkv[j, 2 * s] = (a & jnp.uint32(0xFFFF)) | (b << 16)
            wqkv[j, 2 * s + 1] = (a >> 16) | (b & jnp.uint32(0xFFFF0000))

        def run_ahead(s, j, hh, m0):
            w = pltpu.bitcast(wqkv[j, 2 * s + hh], BF16)
            lhs = pltpu.bitcast(hx[m0 // 2:(m0 + MCH) // 2, :], BF16)
            qkvx[j, 2 * s + hh, m0:m0 + MCH, :] = jnp.dot(lhs, w, preferred_element_type=F32)

        assert HP == CH // 8 == NCH
        CS = cfg.get("cs", 4)

        def mac_gen(f, c, ib):
            rr = pl.multiple_of(f * 8, 8)
            ri = pl.multiple_of(CH + f * 8, 8)
            cs = slice(c * 128, (c + 1) * 128)
            yr = [None] * BL
            yi = [None] * BL
            for jb in range(ib + 1):
                for jj in range(BL):
                    J = jb * BL + jj
                    ur = Ub[J, pl.ds(rr, 8), cs]
                    ui = Ub[J, pl.ds(ri, 8), cs]
                    n = 0
                    for ii in range(BL):
                        I = ib * BL + ii
                        if I < J:
                            continue
                        gr = Gb[I - J, pl.ds(rr, 8), cs]
                        gi = Gb[I - J, pl.ds(ri, 8), cs]
                        tr = gr * ur - gi * ui
                        ti = gr * ui + gi * ur
                        yr[ii] = tr if yr[ii] is None else yr[ii] + tr
                        yi[ii] = ti if yi[ii] is None else yi[ii] + ti
                        n += 1
                    yield n
            for ii in range(BL):
                Ub[ib * BL + ii, pl.ds(rr, 8), cs] = yr[ii]
                Ub[ib * BL + ii, pl.ds(ri, 8), cs] = yi[ii]
            yield 0

        def mac_stream(f, ctiles):
            for c in (ctiles if 'm' not in skip else []):
                for ib in reversed(range(NCH // BL)):
                    yield from mac_gen(f, c, ib)

        def interleave(mxu, vpu, tot):
            nm = sum(w for _, w in mxu)
            done = dm = 0
            for fn, w in mxu:
                fn()
                dm += w
                while done < tot * dm / nm:
                    n = next(vpu, None)
                    if n is None:
                        break
                    done += n
            for _ in vpu:
                pass

        def slab(f, carry):
            for j in range(3):
                cp_w(j, f).wait()

            @pl.when(f + WW < HP)
            def _():
                start_slab(f + WW)

            @pl.when(f + WW == HP)
            def _():
                for c in c_wo:
                    c.start()
            mxu = []
            for j in range(3):
                mxu.append((functools.partial(repack, f, j), 0))
                for hh in range(2):
                    for m0 in range(0, NS * seg, MCH):
                        mxu.append((functools.partial(run_ahead, f, j, hh, m0), 1))
            interleave(mxu, mac_stream(f, range(CS)), CS * NCH * (NCH + 1) // 2)
            return carry
        with scope('slab'):
            lax.fori_loop(0, HP, slab, 0)

        c_fi.wait()
        c_d.wait()
        dvec = dv[...].astype(F32).reshape(1, Dm)

        def inv(i, c):
            r0 = pl.multiple_of(i * CH, CH)
            cs = slice(c * 128, (c + 1) * 128)
            y = jnp.dot(fi[...], Ub[i, :, cs].astype(BF16), preferred_element_type=F32)
            yb[pl.ds(r0, CH), cs] = y + ub[pl.ds(r0, CH), cs].astype(F32) * dvec[:, cs]

        def inv_a(i, carry):
            interleave([(functools.partial(inv, i, c), 1) for c in range(CS)],
                       mac_stream(i, range(CS, NT)), (NT - CS) * NCH * (NCH + 1) // 2)
            return carry

        def inv_b(i, carry):
            for c in range(CS, NT):
                inv(i, c)
            return carry
        with scope('inv_a'):
            lax.fori_loop(0, NCH, inv_a, 0)
        if CS < NT:
            lax.fori_loop(0, NCH, inv_b, 0, unroll=4)

        hbuf[...] = jnp.zeros(hbuf.shape, U32)
        x2buf[0] = jnp.zeros(x2buf.shape[1:], F32)
        ox[...] = jnp.zeros(ox.shape, F32)
        c_bias.wait()
        c_mem0.wait()
        with scope('wait_wo'):
            for c in c_wo:
                c.wait()
        c_xb.start()
        MB = M
        XB = seg // 2
        MO = 2 * XB
        hbuf[0, MO:MO + MB // 2, :] = _pack16(mem0[...].astype(F32))
        hbuf[0, 0:XB, :] = _pack16(_ln(x0[0:seg, :].astype(F32)))

        def finish(s, r0):
            x3 = x2buf[s + 1] + ox[seg:2 * seg, :]
            x4 = x3 + _ln(x3) * yb[pl.ds(r0, seg), :]
            ob[pl.ds(r0, seg), :] = x4.astype(BF16)

        def make_step(act1, act2, pre):
            rows = 2 * M + seg * (int(act1) + int(act2))
            b0 = 0 if (act1 and act2) else R if act1 else R + 2 * M + seg
            x1_in_lhs = act1 and not pre

            key = "b" if (act1 and act2 and not pre) else "bp" if (act1 and act2) else "1" if act1 else "2"
            lS, lP, lW, tail = cfg.get("lag_" + key, LAGS[key])

            def step(t, par):
                npar = 1 - par
                parts = []
                if x1_in_lhs:
                    parts.append(hbuf[par, 0:XB, :])
                if act2:
                    parts.append(hbuf[par, XB:2 * XB, :])
                parts.append(hbuf[par, MO:MO + MB, :])
                hh = pltpu.bitcast(parts[0] if len(parts) == 1 else jnp.concatenate(parts, axis=0), BF16)
                zpad = jnp.zeros((128 - rows, Dh), F32)

                def proj(h, j, padded):
                    r = jnp.dot(hh, pltpu.bitcast(wqkv[j, h], BF16), preferred_element_type=F32)
                    blocks = [r]
                    if pre:
                        x1p = qkvx[j, h, pl.ds(pl.multiple_of((t - LAG) * seg, seg), seg), :]
                        blocks = [x1p, r]
                    if padded:
                        blocks.append(zpad)
                    u = blocks[0] if len(blocks) == 1 else jnp.concatenate(blocks, axis=0)
                    return u.astype(BF16)

                def scores(q, k):
                    s = lax.dot_general(q, k, (((1,), (1,)), ((), ())), preferred_element_type=F32)
                    s = s * qk_scale + bias[b0:b0 + rows, :]
                    m = jnp.max(s, axis=-1, keepdims=True)
                    p = jnp.exp2(s - m)
                    l = jnp.sum(p, axis=-1, keepdims=True)
                    r = pl.reciprocal(l, approx=True)
                    r = r * (2.0 - l * r)
                    return (p * r).astype(BF16)

                def pv(p, v):
                    z = jnp.dot(p, v, preferred_element_type=F32)
                    return jnp.concatenate([z[rows - 2 * M:], z[:rows - 2 * M]], axis=0).astype(BF16)

                def wout(h, z):
                    return jnp.dot(z, pltpu.bitcast(wo[h], BF16), preferred_element_type=F32)

                def post1():
                    s = jnp.minimum(jnp.maximum(t - 1, 0), NSEG - 1)
                    r0 = pl.multiple_of(s * seg, seg)
                    x1 = x0[pl.ds(r0, seg), :].astype(F32) + ox[0:seg, :]
                    x2 = x1 + _ln(x1) * yb[pl.ds(r0, seg), :]
                    x2buf[t] = x2
                    hbuf[npar, XB:2 * XB, :] = _pack16(_ln(x2))

                def post2():
                    s = jnp.maximum(t - 1 - LAG, 0)
                    finish(s, pl.multiple_of(s * seg, seg))

                def pre1():
                    s = jnp.minimum(t + 1, NSEG - 1)
                    r0 = pl.multiple_of(s * seg, seg)
                    hbuf[npar, 0:XB, :] = _pack16(_ln(x0[pl.ds(r0, seg), :].astype(F32)))
                extra = {extras[0]: post1}
                if act2:
                    extra[extras[1]] = post2
                if act1:
                    extra[extras[2]] = pre1

                q, k, v, p, z = {}, {}, {}, {}, {}
                s_at = {h: h + lS for h in range(H)}
                p_at = {h: h + lP for h in range(H)}
                w_at = {h: h + lW for h in range(H)}
                for d, extra_lag in enumerate(tail):
                    p_at[H - 1 - d] += extra_lag
                fin = []
                accv = acc.at[0:rows]
                for i in range(max(w_at.values()) + 1):
                    for op in order:
                        if op == 'q' and i < H:
                            q[i] = proj(i, 0, False)
                        if op == 'k' and i < H:
                            k[i] = proj(i, 1, True)
                        if op == 'v' and i < H:
                            v[i] = proj(i, 2, True)
                        for h in range(H):
                            if op == 'S' and s_at[h] == i:
                                p[h] = scores(q.pop(h), k.pop(h))
                            if op == 'P' and p_at[h] == i:
                                z[h] = pv(p.pop(h), v.pop(h))
                            if op == 'W' and w_at[h] == i:
                                r = wout(h, z.pop(h))
                                if h == 0:
                                    accv[...] = r
                                elif h == H - 1:
                                    fin.append(accv[...] + r)
                                else:
                                    accv[...] += r
                    if i in extra:
                        extra[i]()
                assert not (q or k or v or p or z)
                a = fin[0]
                mp = _pack16(a[0:2 * M, :])
                if act2:
                    hbuf[npar, MO:MO + MB, :] = mp
                else:
                    hbuf[npar, MO:MO + MB // 2, :] = mp[0:MB // 2]
                    hbuf[npar, MO + MB // 2:MO + MB, :] = _pack16(mem0[...].astype(F32))
                if act1 and act2:
                    ox[...] = a[2 * M:R, :]
                elif act1:
                    ox[0:seg, :] = a[2 * M:, :]
                else:
                    ox[seg:2 * seg, :] = a[2 * M:, :]
            return step

        def run_steps(t0, t1, step, unroll=1):
            if unroll == 1:
                lax.fori_loop(t0, t1, lambda t, c: step(t, t & 1), None)
                return
            assert unroll % 2 == 0 and (t1 - t0) % unroll == 0

            def body(i, c):
                for u in range(unroll):
                    step(t0 + i * unroll + u, (t0 + u) & 1)
            lax.fori_loop(0, (t1 - t0) // unroll, body, None)

        with scope('s1'):
            run_steps(0, LAG, make_step(True, False, False))
        c_xb.wait()
        nboth = nsteps - LAG
        with scope('bp'):
            run_steps(LAG, min(LAG + NS, nboth), make_step(True, True, True))
        if nboth > LAG + NS:
            run_steps(LAG + NS, nboth, make_step(True, True, False), cfg.get("unroll", 2))
        OA = (NSEG - LAG - 1) * seg
        c_oa = pltpu.make_async_copy(ob.at[pl.ds(0, OA)], o_hbm.at[pl.ds(0, OA)], sem_out.at[0])
        c_oa.start()
        with scope('s2'):
            run_steps(NSEG, NSEG + LAG, make_step(False, True, False))
        finish(NSEG - 1, (NSEG - 1) * seg)
        c_ob = pltpu.make_async_copy(ob.at[pl.ds(OA, S - OA)], o_hbm.at[pl.ds(OA, S - OA)],
                                     sem_out.at[1])
        c_ob.start()
        c_oa.wait()
        c_ob.wait()

    scratch = [
        pltpu.VMEM((3, H, Dm // 2, Dh), U32),
        pltpu.VMEM((3, HP, Dm, Dh), U32),
        pltpu.VMEM((H, Dh // 2, Dm), U32),
        pltpu.VMEM((S, Dm), BF16),
        pltpu.VMEM((KPAD + S, Dm), BF16),
        pltpu.VMEM((S, Dm), BF16),
        pltpu.VMEM((NCH, Dm, CH), BF16),
        pltpu.VMEM((S, Dm), BF16),
        pltpu.VMEM((NCH, 2 * CH, Dm), F32),
        pltpu.VMEM((NCH, 2 * CH, Dm), F32),
        pltpu.VMEM((2 * CH, Dm), F32),
        pltpu.VMEM((S, Dm), F32),
        pltpu.VMEM((2, R // 2, Dm), U32),
        pltpu.VMEM((NS * seg // 2, Dm), U32),
        pltpu.VMEM((3, H, NS * seg, Dh), F32),
        pltpu.VMEM((R, Dm), F32),
        pltpu.VMEM((NSEG + LAG + 1, seg, Dm), F32),
        pltpu.VMEM((2 * seg, Dm), F32),
        pltpu.VMEM((S, Dm), BF16),
        pltpu.VMEM((2 * CH, CH), BF16),
        pltpu.VMEM((CH, 2 * CH), BF16),
        pltpu.VMEM((R + 2 * (2 * M + seg), 128), F32),
        pltpu.VMEM((M, Dm), BF16),
        pltpu.VMEM((KS, Dm), BF16),
        pltpu.VMEM((Dm,), BF16),
        pltpu.SemaphoreType.DMA((6,)),
        pltpu.SemaphoreType.DMA((NCH,)),
        pltpu.SemaphoreType.DMA((NCH,)),
        pltpu.SemaphoreType.DMA((NCH,)),
        pltpu.SemaphoreType.DMA((3, HP)),
        pltpu.SemaphoreType.DMA((4,)),
        pltpu.SemaphoreType.DMA((2,)),
        pltpu.SemaphoreType.DMA((2,)),
    ]
    return kernel, scratch


def _run(A_x, A_mem0, A_Wq, A_Wk, A_Wv, A_Wo, A_seg_len, B_k, B_v, B_shift_k, B_ssm_k, B_ssm_D,
         cfg=None):
    B, S, Dm = A_x.shape
    assert B == 1
    _, H, Dh = A_Wq.shape
    M = A_mem0.shape[1]
    seg = int(A_seg_len)
    KS = B_shift_k.shape[-1]
    kernel, scratch = _build(S, Dm, H, Dh, M, seg, KS, cfg or {})
    fa_np, fi_np = _dft_mats()
    bias_np = _attn_bias(M, seg)
    args = (A_x.reshape(S, Dm), A_mem0.reshape(M, Dm), A_Wq, A_Wk, A_Wv, A_Wo,
            B_k.reshape(S, Dm), B_v.reshape(S, Dm), B_shift_k.T, B_ssm_k, B_ssm_D,
            fa_np, fi_np, bias_np)
    out = pl.pallas_call(
        kernel,
        out_shape=jax.ShapeDtypeStruct((S, Dm), BF16),
        in_specs=[pl.BlockSpec(memory_space=pl.ANY)] * len(args),
        out_specs=pl.BlockSpec(memory_space=pl.ANY),
        scratch_shapes=scratch,
        compiler_params=pltpu.CompilerParams(vmem_limit_bytes=110 * 1024 * 1024,
                                             flags=(cfg or {}).get("flags")),
    )(*args)
    return out.reshape(B, S, Dm)


@functools.partial(jax.jit, static_argnames=("A_seg_len",))
def pallas_interleave_layers__memory_aug_recurrent_mem_tr__ssm_conv_h3__prompt_kernel(
    A_x: jax.Array,
    A_mem0: jax.Array,
    A_Wq: jax.Array,
    A_Wk: jax.Array,
    A_Wv: jax.Array,
    A_Wo: jax.Array,
    A_seg_len: int,
    B_q: jax.Array,
    B_k: jax.Array,
    B_v: jax.Array,
    B_shift_k: jax.Array,
    B_ssm_k: jax.Array,
    B_ssm_D: jax.Array,
):
    del B_q
    return _run(A_x, A_mem0, A_Wq, A_Wk, A_Wv, A_Wo, A_seg_len, B_k, B_v, B_shift_k,
                B_ssm_k, B_ssm_D)
```

```python
import functools

import jax
import jax.numpy as jnp
import numpy as np
from jax import lax
from jax.experimental import pallas as pl
from jax.experimental.pallas import tpu as pltpu

F32, BF16, U32 = jnp.float32, jnp.bfloat16, jnp.uint32

LOG2E = 1.4426950408889634
LN_EPS = 1e-5
CH = 128
LAG = 2
KPAD = 16


def _np_pack16(a):
    h = np.asarray(a, dtype=np.float32).astype(BF16).view(np.uint16).astype(np.uint32)
    return h[0::2] | (h[1::2] << 16)


def _dft_mats():
    n2 = 2 * CH
    karr = np.concatenate([np.arange(0, CH, 2), np.arange(1, CH, 2)])
    n = np.arange(CH)
    th = 2.0 * np.pi * n[None, :] * (karr[:, None] + 0.5) / n2
    fa = np.concatenate([np.cos(th), -np.sin(th)], axis=0)
    fi = np.concatenate([np.cos(th).T, -np.sin(th).T], axis=1) * (2.0 / n2)
    return _np_pack16(fa), _np_pack16(fi)


def _attn_bias(m, seg):
    stream = np.concatenate([np.zeros(seg), np.ones(seg), np.zeros(m), np.ones(m)])
    ismem = np.concatenate([np.zeros(2 * seg), np.ones(2 * m)]).astype(bool)
    pos = np.concatenate([np.arange(seg), np.arange(seg), np.zeros(2 * m)])
    same = stream[:, None] == stream[None, :]
    keep = ismem[:, None] | ismem[None, :] | (pos[:, None] >= pos[None, :])
    full = np.where(same & keep, 0.0, np.where(same, -1e9 * LOG2E, -1e30))
    s1, s2, mm = np.arange(seg), np.arange(seg, 2 * seg), np.arange(2 * seg, 2 * seg + 2 * m)
    out = []
    for sel in (np.concatenate([s1, s2, mm]), np.concatenate([s1, mm]), np.concatenate([s2, mm])):
        b = np.full((len(sel), 128), -1e30, np.float32)
        b[:, :len(sel)] = full[sel][:, sel]
        out.append(b)
    return np.concatenate(out, axis=0)


def _ln(x):
    m = jnp.mean(x, axis=-1, keepdims=True)
    xc = x - m
    v = jnp.mean(xc * xc, axis=-1, keepdims=True)
    return xc * lax.rsqrt(v + LN_EPS)


def _pack16(x):
    return pltpu.bitcast(x.astype(BF16), U32)


def _build(S, Dm, H, Dh, M, seg, KS, cfg):
    assert Dh == 128 and Dm % 128 == 0 and S % CH == 0 and H % 16 == 0
    assert M == 8 and seg == 32 and KS <= 8
    NSEG = S // seg
    NCH = S // CH
    NT = Dm // 128
    R = 2 * (M + seg)
    HP = H // 2
    qk_scale = float(Dh ** -0.5) * LOG2E
    LAGS = {"b": (2, 4, 12, (3, 2, 1)), "bp": (2, 4, 12, (3, 2, 1, 1)), "1": (2, 4, 12, (4, 3, 2, 1)),
            "2": (2, 4, 12, (4, 3, 2, 1))}
    order = cfg.get("order", "qSkPvW")
    extras = cfg.get("extras", (3, 11, 19))
    nsteps = cfg.get("nsteps", NSEG + LAG)
    skip = cfg.get("skip", "")
    NS = cfg.get("ns", 10)
    assert 0 < NS and LAG + NS <= NSEG - 1

    import contextlib
    scope = jax.named_scope if cfg.get("scopes") else (lambda n: contextlib.nullcontext())

    def kernel(x_hbm, mem0_hbm, wq_hbm, wk_hbm, wv_hbm, wo_hbm, k_hbm, v_hbm, sh_hbm, h_hbm,
               d_hbm, fa_hbm, fi_hbm, bias_hbm, o_hbm,
               wqkv, wstage, wo, x0, kb, vb, hb, ub, Ub, Gb, Ap, yb,
               hbuf, hx, qkvx, acc, x2buf, ox, ob, fa, fi, bias, mem0, shv, dv,
               sem_c, sem_k, sem_v, sem_h, sem_w, sem_o, sem_x, sem_out):
        c_fa = pltpu.make_async_copy(fa_hbm, fa, sem_c.at[0])
        c_sh = pltpu.make_async_copy(sh_hbm, shv, sem_c.at[1])
        c_fi = pltpu.make_async_copy(fi_hbm, fi, sem_c.at[2])
        c_d = pltpu.make_async_copy(d_hbm, dv, sem_c.at[3])
        c_bias = pltpu.make_async_copy(bias_hbm, bias, sem_c.at[4])
        c_mem0 = pltpu.make_async_copy(mem0_hbm, mem0, sem_c.at[5])

        def cp_k(j):
            return pltpu.make_async_copy(
                k_hbm.at[pl.ds(j * CH, CH)], kb.at[pl.ds(KPAD + j * CH, CH)], sem_k.at[j])

        def cp_v(j):
            return pltpu.make_async_copy(
                v_hbm.at[pl.ds(j * CH, CH)], vb.at[pl.ds(j * CH, CH)], sem_v.at[j])

        def cp_h(j):
            return pltpu.make_async_copy(
                h_hbm.at[:, pl.ds(j * CH, CH)], hb.at[j], sem_h.at[j])

        w32 = [w.bitcast(U32) for w in (wq_hbm, wk_hbm, wv_hbm)]

        def cp_w(j, s):
            return pltpu.make_async_copy(w32[j].at[:, s, :], wstage.at[j, s], sem_w.at[j, s])

        wo32 = wo_hbm.bitcast(U32)
        NWO = 4
        c_wo = [pltpu.make_async_copy(wo32.at[pl.ds(i * (H // NWO), H // NWO)],
                                      wo.at[pl.ds(i * (H // NWO), H // NWO)], sem_o.at[i])
                for i in range(NWO)]
        XA = (LAG + NS) * seg
        c_xa = pltpu.make_async_copy(x_hbm.at[pl.ds(0, XA)], x0.at[pl.ds(0, XA)], sem_x.at[0])
        c_xb = pltpu.make_async_copy(x_hbm.at[pl.ds(XA, S - XA)], x0.at[pl.ds(XA, S - XA)],
                                     sem_x.at[1])

        WIN = cfg.get("win", 4)
        WST = cfg.get("wst", NCH - 4)
        WW = cfg.get("ww", 3)

        def start_chunk(j):
            cp_k(j).start()
            cp_v(j).start()
            cp_h(j).start()

        def start_slab(s):
            for j in range(3):
                cp_w(j, s).start()

        start_chunk(0)
        c_fa.start()
        c_sh.start()
        for j in range(1, WIN):
            start_chunk(j)
        c_fi.start()
        c_d.start()
        c_bias.start()
        c_mem0.start()
        c_xa.start()

        kb[0:KPAD, :] = jnp.zeros((KPAD, Dm), BF16)
        Ap[...] = jnp.zeros(Ap.shape, F32)
        with scope('wait_fa'):
            c_fa.wait()
        c_sh.wait()
        sh = shv[...].astype(F32)

        def fwd(j, carry):
            cp_k(j).wait()
            cp_v(j).wait()
            cp_h(j).wait()

            @pl.when(j + WIN < NCH)
            def _():
                start_chunk(j + WIN)

            @pl.when(j >= WST)
            def _():
                @pl.when(j < WST + WW)
                def _():
                    start_slab(j - WST)
            r0 = pl.multiple_of(j * CH, CH)
            kf = kb[pl.ds(r0, CH + KPAD), :].astype(F32)
            ks = kf[KPAD:KPAD + CH] * sh[0:1]
            for dlt in range(1, KS):
                ks = ks + kf[KPAD - dlt:KPAD - dlt + CH] * sh[dlt:dlt + 1]
            u = (ks * vb[pl.ds(r0, CH), :].astype(F32)).astype(BF16)
            ub[pl.ds(r0, CH), :] = u
            fav = pltpu.bitcast(fa[...], BF16)
            Ub[j] = jnp.dot(fav, u, preferred_element_type=F32)
            a = lax.dot_general(fav, hb[j], (((1,), (1,)), ((), ())),
                                preferred_element_type=F32)
            p = Ap[...]
            hh = CH // 2
            Gb[j, 0:hh] = a[0:hh] - p[CH:CH + hh]
            Gb[j, hh:CH] = a[hh:CH] + p[CH + hh:2 * CH]
            Gb[j, CH:CH + hh] = a[CH:CH + hh] + p[0:hh]
            Gb[j, CH + hh:2 * CH] = a[CH + hh:2 * CH] - p[hh:CH]
            Ap[...] = a
            return carry
        with scope('fwd'):
            lax.fori_loop(0, NCH, fwd, 0)

        BL = cfg.get("bl", 4)
        MCH = cfg.get("mch", 64)

        with scope('wait_xa'):
            c_xa.wait()
        for i in range(NS):
            hx[i * seg // 2:(i + 1) * seg // 2, :] = _pack16(
                _ln(x0[(LAG + i) * seg:(LAG + i + 1) * seg, :].astype(F32)))

        def repack(s, j):
            a = wstage[j, s, pl.ds(0, Dm // 2, stride=2), :]
            b = wstage[j, s, pl.ds(1, Dm // 2, stride=2), :]
            wqkv[j, 2 * s] = (a & jnp.uint32(0xFFFF)) | (b << 16)
            wqkv[j, 2 * s + 1] = (a >> 16) | (b & jnp.uint32(0xFFFF0000))

        def run_ahead(s, j, hh, m0):
            w = pltpu.bitcast(wqkv[j, 2 * s + hh], BF16)
            lhs = pltpu.bitcast(hx[m0 // 2:(m0 + MCH) // 2, :], BF16)
            qkvx[j, 2 * s + hh, m0:m0 + MCH, :] = jnp.dot(lhs, w, preferred_element_type=F32)

        assert HP == CH // 8 == NCH
        CS = cfg.get("cs", 5)

        def mac_gen(f, c, ib):
            rr = pl.multiple_of(f * 8, 8)
            ri = pl.multiple_of(CH + f * 8, 8)
            cs = slice(c * 128, (c + 1) * 128)
            yr = [None] * BL
            yi = [None] * BL
            for jb in range(ib + 1):
                for jj in range(BL):
                    J = jb * BL + jj
                    ur = Ub[J, pl.ds(rr, 8), cs]
                    ui = Ub[J, pl.ds(ri, 8), cs]
                    n = 0
                    for ii in range(BL):
                        I = ib * BL + ii
                        if I < J:
                            continue
                        gr = Gb[I - J, pl.ds(rr, 8), cs]
                        gi = Gb[I - J, pl.ds(ri, 8), cs]
                        tr = gr * ur - gi * ui
                        ti = gr * ui + gi * ur
                        yr[ii] = tr if yr[ii] is None else yr[ii] + tr
                        yi[ii] = ti if yi[ii] is None else yi[ii] + ti
                        n += 1
                    yield n
            for ii in range(BL):
                Ub[ib * BL + ii, pl.ds(rr, 8), cs] = yr[ii]
                Ub[ib * BL + ii, pl.ds(ri, 8), cs] = yi[ii]
            yield 0

        def mac_stream(f, ctiles):
            for c in (ctiles if 'm' not in skip else []):
                for ib in reversed(range(NCH // BL)):
                    yield from mac_gen(f, c, ib)

        def interleave(mxu, vpu, tot):
            nm = sum(w for _, w in mxu)
            done = dm = 0
            for fn, w in mxu:
                fn()
                dm += w
                while done < tot * dm / nm:
                    n = next(vpu, None)
                    if n is None:
                        break
                    done += n
            for _ in vpu:
                pass

        def slab(f, carry):
            for j in range(3):
                cp_w(j, f).wait()

            @pl.when(f + WW < HP)
            def _():
                start_slab(f + WW)

            @pl.when(f + WW == HP)
            def _():
                for c in c_wo:
                    c.start()
            mxu = []
            for j in range(3):
                mxu.append((functools.partial(repack, f, j), 0))
                for hh in range(2):
                    for m0 in range(0, NS * seg, MCH):
                        mxu.append((functools.partial(run_ahead, f, j, hh, m0), 1))
            interleave(mxu, mac_stream(f, range(CS)), CS * NCH * (NCH + 1) // 2)
            return carry
        with scope('slab'):
            lax.fori_loop(0, HP, slab, 0)

        c_fi.wait()
        c_d.wait()
        dvec = dv[...].astype(F32).reshape(1, Dm)

        def inv(i, c):
            r0 = pl.multiple_of(i * CH, CH)
            cs = slice(c * 128, (c + 1) * 128)
            y = jnp.dot(pltpu.bitcast(fi[...], BF16), Ub[i, :, cs].astype(BF16), preferred_element_type=F32)
            yb[pl.ds(r0, CH), cs] = y + ub[pl.ds(r0, CH), cs].astype(F32) * dvec[:, cs]

        def inv_a(i, carry):
            interleave([(functools.partial(inv, i, c), 1) for c in range(CS)],
                       mac_stream(i, range(CS, NT)), (NT - CS) * NCH * (NCH + 1) // 2)
            return carry

        def inv_b(i, carry):
            for c in range(CS, NT):
                inv(i, c)
            return carry
        with scope('inv_a'):
            lax.fori_loop(0, NCH, inv_a, 0, unroll=cfg.get("iu", 4))
        if CS < NT:
            lax.fori_loop(0, NCH, inv_b, 0, unroll=4)

        hbuf[...] = jnp.zeros(hbuf.shape, U32)
        x2buf[0] = jnp.zeros(x2buf.shape[1:], F32)
        ox[...] = jnp.zeros(ox.shape, F32)
        c_bias.wait()
        c_mem0.wait()
        with scope('wait_wo'):
            for c in c_wo:
                c.wait()
        c_xb.start()
        MB = M
        XB = seg // 2
        MO = 2 * XB
        hbuf[0, MO:MO + MB // 2, :] = _pack16(mem0[...].astype(F32))
        hbuf[0, 0:XB, :] = _pack16(_ln(x0[0:seg, :].astype(F32)))

        def finish(s, r0):
            x3 = x2buf[s + 1] + ox[seg:2 * seg, :]
            x4 = x3 + _ln(x3) * yb[pl.ds(r0, seg), :]
            ob[pl.ds(r0, seg), :] = x4.astype(BF16)

        def make_step(act1, act2, pre):
            rows = 2 * M + seg * (int(act1) + int(act2))
            b0 = 0 if (act1 and act2) else R if act1 else R + 2 * M + seg
            x1_in_lhs = act1 and not pre

            key = "b" if (act1 and act2 and not pre) else "bp" if (act1 and act2) else "1" if act1 else "2"
            lS, lP, lW, tail = cfg.get("lag_" + key, LAGS[key])

            def step(t, par):
                npar = 1 - par
                parts = []
                if x1_in_lhs:
                    parts.append(hbuf[par, 0:XB, :])
                if act2:
                    parts.append(hbuf[par, XB:2 * XB, :])
                parts.append(hbuf[par, MO:MO + MB, :])
                hh = pltpu.bitcast(parts[0] if len(parts) == 1 else jnp.concatenate(parts, axis=0), BF16)
                zpad = jnp.zeros((128 - rows, Dh), F32)

                def proj(h, j, padded):
                    r = jnp.dot(hh, pltpu.bitcast(wqkv[j, h], BF16), preferred_element_type=F32)
                    blocks = [r]
                    if pre:
                        x1p = qkvx[j, h, pl.ds(pl.multiple_of((t - LAG) * seg, seg), seg), :]
                        blocks = [x1p, r]
                    if padded:
                        blocks.append(zpad)
                    u = blocks[0] if len(blocks) == 1 else jnp.concatenate(blocks, axis=0)
                    return u.astype(BF16)

                def scores(q, k):
                    s = lax.dot_general(q, k, (((1,), (1,)), ((), ())), preferred_element_type=F32)
                    s = s * qk_scale + bias[b0:b0 + rows, :]
                    m = jnp.max(s, axis=-1, keepdims=True)
                    p = jnp.exp2(s - m)
                    l = jnp.sum(p, axis=-1, keepdims=True)
                    r = pl.reciprocal(l, approx=True)
                    r = r * (2.0 - l * r)
                    return (p * r).astype(BF16)

                def pv(p, v):
                    z = jnp.dot(p, v, preferred_element_type=F32)
                    return jnp.concatenate([z[rows - 2 * M:], z[:rows - 2 * M]], axis=0).astype(BF16)

                def wout(h, z):
                    return jnp.dot(z, pltpu.bitcast(wo[h], BF16), preferred_element_type=F32)

                def post1():
                    s = jnp.minimum(jnp.maximum(t - 1, 0), NSEG - 1)
                    r0 = pl.multiple_of(s * seg, seg)
                    x1 = x0[pl.ds(r0, seg), :].astype(F32) + ox[0:seg, :]
                    x2 = x1 + _ln(x1) * yb[pl.ds(r0, seg), :]
                    x2buf[t] = x2
                    hbuf[npar, XB:2 * XB, :] = _pack16(_ln(x2))

                def post2():
                    s = jnp.maximum(t - 1 - LAG, 0)
                    finish(s, pl.multiple_of(s * seg, seg))

                def pre1():
                    s = jnp.minimum(t + 1, NSEG - 1)
                    r0 = pl.multiple_of(s * seg, seg)
                    hbuf[npar, 0:XB, :] = _pack16(_ln(x0[pl.ds(r0, seg), :].astype(F32)))
                extra = {extras[0]: post1}
                if act2:
                    extra[extras[1]] = post2
                if act1:
                    extra[extras[2]] = pre1

                q, k, v, p, z = {}, {}, {}, {}, {}
                s_at = {h: h + lS for h in range(H)}
                p_at = {h: h + lP for h in range(H)}
                w_at = {h: h + lW for h in range(H)}
                for d, extra_lag in enumerate(tail):
                    p_at[H - 1 - d] += extra_lag
                fin = []
                accv = acc.at[0:rows]
                for i in range(max(w_at.values()) + 1):
                    for op in order:
                        if op == 'q' and i < H:
                            q[i] = proj(i, 0, False)
                        if op == 'k' and i < H:
                            k[i] = proj(i, 1, True)
                        if op == 'v' and i < H:
                            v[i] = proj(i, 2, True)
                        for h in range(H):
                            if op == 'S' and s_at[h] == i:
                                p[h] = scores(q.pop(h), k.pop(h))
                            if op == 'P' and p_at[h] == i:
                                z[h] = pv(p.pop(h), v.pop(h))
                            if op == 'W' and w_at[h] == i:
                                r = wout(h, z.pop(h))
                                if h == 0:
                                    accv[...] = r
                                elif h == H - 1:
                                    fin.append(accv[...] + r)
                                else:
                                    accv[...] += r
                    if i in extra:
                        extra[i]()
                assert not (q or k or v or p or z)
                a = fin[0]
                mp = _pack16(a[0:2 * M, :])
                if act2:
                    hbuf[npar, MO:MO + MB, :] = mp
                else:
                    hbuf[npar, MO:MO + MB // 2, :] = mp[0:MB // 2]
                    hbuf[npar, MO + MB // 2:MO + MB, :] = _pack16(mem0[...].astype(F32))
                if act1 and act2:
                    ox[...] = a[2 * M:R, :]
                elif act1:
                    ox[0:seg, :] = a[2 * M:, :]
                else:
                    ox[seg:2 * seg, :] = a[2 * M:, :]
            return step

        def run_steps(t0, t1, step, unroll=1):
            if unroll == 1:
                lax.fori_loop(t0, t1, lambda t, c: step(t, t & 1), None)
                return
            assert unroll % 2 == 0 and (t1 - t0) % unroll == 0

            def body(i, c):
                for u in range(unroll):
                    step(t0 + i * unroll + u, (t0 + u) & 1)
            lax.fori_loop(0, (t1 - t0) // unroll, body, None)

        with scope('s1'):
            run_steps(0, LAG, make_step(True, False, False), cfg.get("s1u", 1))
        c_xb.wait()
        nboth = nsteps - LAG
        with scope('bp'):
            run_steps(LAG, min(LAG + NS, nboth), make_step(True, True, True), cfg.get("bpu", 1))
        if nboth > LAG + NS:
            with scope('b'):
                run_steps(LAG + NS, nboth, make_step(True, True, False), cfg.get("unroll", 2))
        OA = (NSEG - LAG - 1) * seg
        c_oa = pltpu.make_async_copy(ob.at[pl.ds(0, OA)], o_hbm.at[pl.ds(0, OA)], sem_out.at[0])
        c_oa.start()
        with scope('s2'):
            run_steps(NSEG, NSEG + LAG, make_step(False, True, False), cfg.get("s2u", 1))
        finish(NSEG - 1, (NSEG - 1) * seg)
        c_ob = pltpu.make_async_copy(ob.at[pl.ds(OA, S - OA)], o_hbm.at[pl.ds(OA, S - OA)],
                                     sem_out.at[1])
        c_ob.start()
        c_oa.wait()
        c_ob.wait()

    scratch = [
        pltpu.VMEM((3, H, Dm // 2, Dh), U32),
        pltpu.VMEM((3, HP, Dm, Dh), U32),
        pltpu.VMEM((H, Dh // 2, Dm), U32),
        pltpu.VMEM((S, Dm), BF16),
        pltpu.VMEM((KPAD + S, Dm), BF16),
        pltpu.VMEM((S, Dm), BF16),
        pltpu.VMEM((NCH, Dm, CH), BF16),
        pltpu.VMEM((S, Dm), BF16),
        pltpu.VMEM((NCH, 2 * CH, Dm), F32),
        pltpu.VMEM((NCH, 2 * CH, Dm), F32),
        pltpu.VMEM((2 * CH, Dm), F32),
        pltpu.VMEM((S, Dm), F32),
        pltpu.VMEM((2, R // 2, Dm), U32),
        pltpu.VMEM((NS * seg // 2, Dm), U32),
        pltpu.VMEM((3, H, NS * seg, Dh), F32),
        pltpu.VMEM((R, Dm), F32),
        pltpu.VMEM((NSEG + LAG + 1, seg, Dm), F32),
        pltpu.VMEM((2 * seg, Dm), F32),
        pltpu.VMEM((S, Dm), BF16),
        pltpu.VMEM((CH, CH), U32),
        pltpu.VMEM((CH // 2, 2 * CH), U32),
        pltpu.VMEM((R + 2 * (2 * M + seg), 128), F32),
        pltpu.VMEM((M, Dm), BF16),
        pltpu.VMEM((KS, Dm), BF16),
        pltpu.VMEM((Dm,), BF16),
        pltpu.SemaphoreType.DMA((6,)),
        pltpu.SemaphoreType.DMA((NCH,)),
        pltpu.SemaphoreType.DMA((NCH,)),
        pltpu.SemaphoreType.DMA((NCH,)),
        pltpu.SemaphoreType.DMA((3, HP)),
        pltpu.SemaphoreType.DMA((4,)),
        pltpu.SemaphoreType.DMA((2,)),
        pltpu.SemaphoreType.DMA((2,)),
    ]
    return kernel, scratch


def _run(A_x, A_mem0, A_Wq, A_Wk, A_Wv, A_Wo, A_seg_len, B_k, B_v, B_shift_k, B_ssm_k, B_ssm_D,
         cfg=None):
    B, S, Dm = A_x.shape
    assert B == 1
    _, H, Dh = A_Wq.shape
    M = A_mem0.shape[1]
    seg = int(A_seg_len)
    KS = B_shift_k.shape[-1]
    kernel, scratch = _build(S, Dm, H, Dh, M, seg, KS, cfg or {})
    fa_np, fi_np = _dft_mats()
    bias_np = _attn_bias(M, seg)
    args = (A_x.reshape(S, Dm), A_mem0.reshape(M, Dm), A_Wq, A_Wk, A_Wv, A_Wo,
            B_k.reshape(S, Dm), B_v.reshape(S, Dm), B_shift_k.T, B_ssm_k, B_ssm_D,
            fa_np, fi_np, bias_np)
    out = pl.pallas_call(
        kernel,
        out_shape=jax.ShapeDtypeStruct((S, Dm), BF16),
        in_specs=[pl.BlockSpec(memory_space=pl.ANY)] * len(args),
        out_specs=pl.BlockSpec(memory_space=pl.ANY),
        scratch_shapes=scratch,
        compiler_params=pltpu.CompilerParams(vmem_limit_bytes=110 * 1024 * 1024,
                                             flags=(cfg or {}).get("flags")),
    )(*args)
    return out.reshape(B, S, Dm)


@functools.partial(jax.jit, static_argnames=("A_seg_len",))
def pallas_interleave_layers__memory_aug_recurrent_mem_tr__ssm_conv_h3__prompt_kernel(
    A_x: jax.Array,
    A_mem0: jax.Array,
    A_Wq: jax.Array,
    A_Wk: jax.Array,
    A_Wv: jax.Array,
    A_Wo: jax.Array,
    A_seg_len: int,
    B_q: jax.Array,
    B_k: jax.Array,
    B_v: jax.Array,
    B_shift_k: jax.Array,
    B_ssm_k: jax.Array,
    B_ssm_D: jax.Array,
):
    del B_q
    return _run(A_x, A_mem0, A_Wq, A_Wk, A_Wv, A_Wo, A_seg_len, B_k, B_v, B_shift_k,
                B_ssm_k, B_ssm_D)
```

```python
import functools

import jax
import jax.numpy as jnp
import numpy as np
from jax import lax
from jax.experimental import pallas as pl
from jax.experimental.pallas import tpu as pltpu

F32, BF16, U32 = jnp.float32, jnp.bfloat16, jnp.uint32

LOG2E = 1.4426950408889634
LN_EPS = 1e-5
CH = 128
LAG = 2
KPAD = 16


def _np_pack16(a):
    h = np.asarray(a, dtype=np.float32).astype(BF16).view(np.uint16).astype(np.uint32)
    return h[0::2] | (h[1::2] << 16)


def _dft_mats():
    n2 = 2 * CH
    karr = np.concatenate([np.arange(0, CH, 2), np.arange(1, CH, 2)])
    n = np.arange(CH)
    th = 2.0 * np.pi * n[None, :] * (karr[:, None] + 0.5) / n2
    fa = np.concatenate([np.cos(th), -np.sin(th)], axis=0)
    fi = np.concatenate([np.cos(th).T, -np.sin(th).T], axis=1) * (2.0 / n2)
    return _np_pack16(fa), _np_pack16(fi)


def _attn_bias(m, seg):
    stream = np.concatenate([np.zeros(seg), np.ones(seg), np.zeros(m), np.ones(m)])
    ismem = np.concatenate([np.zeros(2 * seg), np.ones(2 * m)]).astype(bool)
    pos = np.concatenate([np.arange(seg), np.arange(seg), np.zeros(2 * m)])
    same = stream[:, None] == stream[None, :]
    keep = ismem[:, None] | ismem[None, :] | (pos[:, None] >= pos[None, :])
    full = np.where(same & keep, 0.0, np.where(same, -1e9 * LOG2E, -1e30))
    s1, s2, mm = np.arange(seg), np.arange(seg, 2 * seg), np.arange(2 * seg, 2 * seg + 2 * m)
    out = []
    for sel in (np.concatenate([s1, s2, mm]), np.concatenate([s1, mm]), np.concatenate([s2, mm])):
        b = np.full((len(sel), 128), -1e30, np.float32)
        b[:, :len(sel)] = full[sel][:, sel]
        out.append(b)
    return np.concatenate(out, axis=0)


def _ln(x):
    m = jnp.mean(x, axis=-1, keepdims=True)
    xc = x - m
    v = jnp.mean(xc * xc, axis=-1, keepdims=True)
    return xc * lax.rsqrt(v + LN_EPS)


def _pack16(x):
    return pltpu.bitcast(x.astype(BF16), U32)


def _build(S, Dm, H, Dh, M, seg, KS, cfg):
    assert Dh == 128 and Dm % 128 == 0 and S % CH == 0 and H % 16 == 0
    assert M == 8 and seg == 32 and KS <= 8
    NSEG = S // seg
    NCH = S // CH
    NT = Dm // 128
    R = 2 * (M + seg)
    HP = H // 2
    qk_scale = float(Dh ** -0.5) * LOG2E
    LAGS = {"b": (2, 4, 12, (3, 2, 1)), "bp": (2, 4, 12, (3, 2, 1, 1)), "1": (2, 4, 12, (4, 3, 2, 1)),
            "2": (2, 4, 12, (4, 3, 2, 1))}
    order = cfg.get("order", "qSkPvW")
    extras = cfg.get("extras", (3, 11, 19))
    nsteps = cfg.get("nsteps", NSEG + LAG)
    skip = cfg.get("skip", "")
    NS = cfg.get("ns", 10)
    assert 0 < NS and LAG + NS <= NSEG - 1

    import contextlib
    scope = jax.named_scope if cfg.get("scopes") else (lambda n: contextlib.nullcontext())

    def kernel(x_hbm, mem0_hbm, wq_hbm, wk_hbm, wv_hbm, wo_hbm, k_hbm, v_hbm, sh_hbm, h_hbm,
               d_hbm, fa_hbm, fi_hbm, bias_hbm, o_hbm,
               wqkv, wstage, wo, x0, kb, vb, hb, ub, Ub, Gb, Ap, yb,
               hbuf, hx, qkvx, acc, x2buf, ox, ob, fa, fi, bias, mem0, shv, dv,
               sem_c, sem_k, sem_v, sem_h, sem_w, sem_o, sem_x, sem_out):
        c_fa = pltpu.make_async_copy(fa_hbm, fa, sem_c.at[0])
        c_sh = pltpu.make_async_copy(sh_hbm, shv, sem_c.at[1])
        c_fi = pltpu.make_async_copy(fi_hbm, fi, sem_c.at[2])
        c_d = pltpu.make_async_copy(d_hbm, dv, sem_c.at[3])
        c_bias = pltpu.make_async_copy(bias_hbm, bias, sem_c.at[4])
        c_mem0 = pltpu.make_async_copy(mem0_hbm, mem0, sem_c.at[5])

        def cp_k(j):
            return pltpu.make_async_copy(
                k_hbm.at[pl.ds(j * CH, CH)], kb.at[pl.ds(KPAD + j * CH, CH)], sem_k.at[j])

        def cp_v(j):
            return pltpu.make_async_copy(
                v_hbm.at[pl.ds(j * CH, CH)], vb.at[pl.ds(j * CH, CH)], sem_v.at[j])

        def cp_h(j):
            return pltpu.make_async_copy(
                h_hbm.at[:, pl.ds(j * CH, CH)], hb.at[j], sem_h.at[j])

        w32 = [w.bitcast(U32) for w in (wq_hbm, wk_hbm, wv_hbm)]

        def cp_w(j, s):
            return pltpu.make_async_copy(w32[j].at[:, s, :], wstage.at[j, s], sem_w.at[j, s])

        wo32 = wo_hbm.bitcast(U32)
        NWO = 4
        c_wo = [pltpu.make_async_copy(wo32.at[pl.ds(i * (H // NWO), H // NWO)],
                                      wo.at[pl.ds(i * (H // NWO), H // NWO)], sem_o.at[i])
                for i in range(NWO)]
        XA = (LAG + NS) * seg
        c_xa = pltpu.make_async_copy(x_hbm.at[pl.ds(0, XA)], x0.at[pl.ds(0, XA)], sem_x.at[0])
        c_xb = pltpu.make_async_copy(x_hbm.at[pl.ds(XA, S - XA)], x0.at[pl.ds(XA, S - XA)],
                                     sem_x.at[1])

        WIN = cfg.get("win", 4)
        WST = cfg.get("wst", NCH - 4)
        WW = cfg.get("ww", 3)
        assert 0 <= WST and WST + WW <= NCH

        def start_chunk(j):
            cp_k(j).start()
            cp_v(j).start()
            cp_h(j).start()

        def start_slab(s):
            for j in range(3):
                cp_w(j, s).start()

        start_chunk(0)
        c_fa.start()
        c_sh.start()
        for j in range(1, WIN):
            start_chunk(j)
        c_fi.start()
        c_d.start()
        c_bias.start()
        c_mem0.start()
        c_xa.start()

        kb[0:KPAD, :] = jnp.zeros((KPAD, Dm), BF16)
        Ap[...] = jnp.zeros(Ap.shape, F32)
        with scope('wait_fa'):
            c_fa.wait()
        c_sh.wait()
        sh = shv[...].astype(F32)

        def fwd(j, carry):
            cp_k(j).wait()
            cp_v(j).wait()
            cp_h(j).wait()

            @pl.when(j + WIN < NCH)
            def _():
                start_chunk(j + WIN)

            @pl.when(j >= WST)
            def _():
                @pl.when(j < WST + WW)
                def _():
                    start_slab(j - WST)
            r0 = pl.multiple_of(j * CH, CH)
            kf = kb[pl.ds(r0, CH + KPAD), :].astype(F32)
            ks = kf[KPAD:KPAD + CH] * sh[0:1]
            for dlt in range(1, KS):
                ks = ks + kf[KPAD - dlt:KPAD - dlt + CH] * sh[dlt:dlt + 1]
            u = (ks * vb[pl.ds(r0, CH), :].astype(F32)).astype(BF16)
            ub[pl.ds(r0, CH), :] = u
            fav = pltpu.bitcast(fa[...], BF16)
            Ub[j] = jnp.dot(fav, u, preferred_element_type=F32)
            a = lax.dot_general(fav, hb[j], (((1,), (1,)), ((), ())),
                                preferred_element_type=F32)
            p = Ap[...]
            hh = CH // 2
            Gb[j, 0:hh] = a[0:hh] - p[CH:CH + hh]
            Gb[j, hh:CH] = a[hh:CH] + p[CH + hh:2 * CH]
            Gb[j, CH:CH + hh] = a[CH:CH + hh] + p[0:hh]
            Gb[j, CH + hh:2 * CH] = a[CH + hh:2 * CH] - p[hh:CH]
            Ap[...] = a
            return carry
        with scope('fwd'):
            lax.fori_loop(0, NCH, fwd, 0)

        BL = cfg.get("bl", 4)
        MCH = cfg.get("mch", 64)

        with scope('wait_xa'):
            c_xa.wait()
        for i in range(NS):
            hx[i * seg // 2:(i + 1) * seg // 2, :] = _pack16(
                _ln(x0[(LAG + i) * seg:(LAG + i + 1) * seg, :].astype(F32)))

        def repack(s, j):
            src = jnp.minimum(s, HP - 1)
            a = wstage[j, src, pl.ds(0, Dm // 2, stride=2), :]
            b = wstage[j, src, pl.ds(1, Dm // 2, stride=2), :]
            wqkv[j, 2 * s] = (a & jnp.uint32(0xFFFF)) | (b << 16)
            wqkv[j, 2 * s + 1] = (a >> 16) | (b & jnp.uint32(0xFFFF0000))

        def run_ahead(s, j, hh, m0):
            w = pltpu.bitcast(wqkv[j, 2 * s + hh], BF16)
            lhs = pltpu.bitcast(hx[m0 // 2:(m0 + MCH) // 2, :], BF16)
            qkvx[j, 2 * s + hh, m0:m0 + MCH, :] = jnp.dot(lhs, w, preferred_element_type=F32)

        assert HP == CH // 8 == NCH
        CS = cfg.get("cs", 5)

        def mac_gen(f, c, ib):
            rr = pl.multiple_of(f * 8, 8)
            ri = pl.multiple_of(CH + f * 8, 8)
            cs = slice(c * 128, (c + 1) * 128)
            yr = [None] * BL
            yi = [None] * BL
            for jb in range(ib + 1):
                for jj in range(BL):
                    J = jb * BL + jj
                    ur = Ub[J, pl.ds(rr, 8), cs]
                    ui = Ub[J, pl.ds(ri, 8), cs]
                    n = 0
                    for ii in range(BL):
                        I = ib * BL + ii
                        if I < J:
                            continue
                        gr = Gb[I - J, pl.ds(rr, 8), cs]
                        gi = Gb[I - J, pl.ds(ri, 8), cs]
                        tr = gr * ur - gi * ui
                        ti = gr * ui + gi * ur
                        yr[ii] = tr if yr[ii] is None else yr[ii] + tr
                        yi[ii] = ti if yi[ii] is None else yi[ii] + ti
                        n += 1
                    yield n
            for ii in range(BL):
                Ub[ib * BL + ii, pl.ds(rr, 8), cs] = yr[ii]
                Ub[ib * BL + ii, pl.ds(ri, 8), cs] = yi[ii]
            yield 0

        def mac_stream(f, ctiles):
            for c in (ctiles if 'm' not in skip else []):
                for ib in reversed(range(NCH // BL)):
                    yield from mac_gen(f, c, ib)

        def interleave(mxu, vpu, tot):
            nm = sum(w for _, w in mxu)
            done = dm = 0
            for fn, w in mxu:
                fn()
                dm += w
                while done < tot * dm / nm:
                    n = next(vpu, None)
                    if n is None:
                        break
                    done += n
            for _ in vpu:
                pass

        def slab_arrived(s):
            for j in range(3):
                cp_w(j, s).wait()

            @pl.when(s + WW < HP)
            def _():
                start_slab(s + WW)

            @pl.when(s + WW == HP)
            def _():
                for c in c_wo:
                    c.start()

        PIPE = cfg.get("pipe", 0)
        SU = cfg.get("su", 2)

        def slab(f):
            mxu = []
            for j in range(3):
                if not PIPE:
                    mxu.append((functools.partial(repack, f, j), 0))
                for hh in range(2):
                    for m0 in range(0, NS * seg, MCH):
                        mxu.append((functools.partial(run_ahead, f, j, hh, m0), 1))
                if PIPE:
                    mxu.append((functools.partial(repack, f + 1, j), 0))
            interleave(mxu, mac_stream(f, range(CS)), CS * NCH * (NCH + 1) // 2)

        def slab_body(i, carry):
            for u in range(SU):
                f = i * SU + u
                if PIPE:
                    @pl.when(f + 1 < HP)
                    def _():
                        slab_arrived(f + 1)
                else:
                    slab_arrived(f)
            for u in range(SU):
                slab(i * SU + u)
            return carry
        with scope('slab'):
            if PIPE:
                slab_arrived(0)
                for j in range(3):
                    repack(0, j)
            lax.fori_loop(0, HP // SU, slab_body, 0)

        c_fi.wait()
        c_d.wait()
        dvec = dv[...].astype(F32).reshape(1, Dm)

        def inv(i, c):
            r0 = pl.multiple_of(i * CH, CH)
            cs = slice(c * 128, (c + 1) * 128)
            y = jnp.dot(pltpu.bitcast(fi[...], BF16), Ub[i, :, cs].astype(BF16), preferred_element_type=F32)
            yb[pl.ds(r0, CH), cs] = y + ub[pl.ds(r0, CH), cs].astype(F32) * dvec[:, cs]

        def inv_a(i, carry):
            interleave([(functools.partial(inv, i, c), 1) for c in range(CS)],
                       mac_stream(i, range(CS, NT)), (NT - CS) * NCH * (NCH + 1) // 2)
            return carry

        def inv_b(i, carry):
            for c in range(CS, NT):
                inv(i, c)
            return carry
        with scope('inv_a'):
            lax.fori_loop(0, NCH, inv_a, 0, unroll=cfg.get("iu", 4))
        if CS < NT:
            lax.fori_loop(0, NCH, inv_b, 0, unroll=4)

        hbuf[...] = jnp.zeros(hbuf.shape, U32)
        x2buf[0] = jnp.zeros(x2buf.shape[1:], F32)
        ox[...] = jnp.zeros(ox.shape, F32)
        c_bias.wait()
        c_mem0.wait()
        with scope('wait_wo'):
            for c in c_wo:
                c.wait()
        c_xb.start()
        MB = M
        XB = seg // 2
        MO = 2 * XB
        hbuf[0, MO:MO + MB // 2, :] = _pack16(mem0[...].astype(F32))
        hbuf[0, 0:XB, :] = _pack16(_ln(x0[0:seg, :].astype(F32)))

        def finish(s, r0):
            x3 = x2buf[s + 1] + ox[seg:2 * seg, :]
            x4 = x3 + _ln(x3) * yb[pl.ds(r0, seg), :]
            ob[pl.ds(r0, seg), :] = x4.astype(BF16)

        def make_step(act1, act2, pre):
            rows = 2 * M + seg * (int(act1) + int(act2))
            b0 = 0 if (act1 and act2) else R if act1 else R + 2 * M + seg
            x1_in_lhs = act1 and not pre

            key = "b" if (act1 and act2 and not pre) else "bp" if (act1 and act2) else "1" if act1 else "2"
            lS, lP, lW, tail = cfg.get("lag_" + key, LAGS[key])

            def step(t, par):
                npar = 1 - par
                parts = []
                if x1_in_lhs:
                    parts.append(hbuf[par, 0:XB, :])
                if act2:
                    parts.append(hbuf[par, XB:2 * XB, :])
                parts.append(hbuf[par, MO:MO + MB, :])
                hh = pltpu.bitcast(parts[0] if len(parts) == 1 else jnp.concatenate(parts, axis=0), BF16)
                zpad = jnp.zeros((128 - rows, Dh), F32)

                def proj(h, j, padded):
                    r = jnp.dot(hh, pltpu.bitcast(wqkv[j, h], BF16), preferred_element_type=F32)
                    blocks = [r]
                    if pre:
                        x1p = qkvx[j, h, pl.ds(pl.multiple_of((t - LAG) * seg, seg), seg), :]
                        blocks = [x1p, r]
                    if padded:
                        blocks.append(zpad)
                    u = blocks[0] if len(blocks) == 1 else jnp.concatenate(blocks, axis=0)
                    return u.astype(BF16)

                def scores(q, k):
                    s = lax.dot_general(q, k, (((1,), (1,)), ((), ())), preferred_element_type=F32)
                    s = s * qk_scale + bias[b0:b0 + rows, :]
                    m = jnp.max(s, axis=-1, keepdims=True)
                    p = jnp.exp2(s - m)
                    l = jnp.sum(p, axis=-1, keepdims=True)
                    r = pl.reciprocal(l, approx=True)
                    r = r * (2.0 - l * r)
                    return (p * r).astype(BF16)

                def pv(p, v):
                    z = jnp.dot(p, v, preferred_element_type=F32)
                    return jnp.concatenate([z[rows - 2 * M:], z[:rows - 2 * M]], axis=0).astype(BF16)

                def wout(h, z):
                    return jnp.dot(z, pltpu.bitcast(wo[h], BF16), preferred_element_type=F32)

                def post1():
                    s = jnp.minimum(jnp.maximum(t - 1, 0), NSEG - 1)
                    r0 = pl.multiple_of(s * seg, seg)
                    x1 = x0[pl.ds(r0, seg), :].astype(F32) + ox[0:seg, :]
                    x2 = x1 + _ln(x1) * yb[pl.ds(r0, seg), :]
                    x2buf[t] = x2
                    hbuf[npar, XB:2 * XB, :] = _pack16(_ln(x2))

                def post2():
                    s = jnp.maximum(t - 1 - LAG, 0)
                    finish(s, pl.multiple_of(s * seg, seg))

                def pre1():
                    s = jnp.minimum(t + 1, NSEG - 1)
                    r0 = pl.multiple_of(s * seg, seg)
                    hbuf[npar, 0:XB, :] = _pack16(_ln(x0[pl.ds(r0, seg), :].astype(F32)))
                extra = {extras[0]: post1}
                if act2:
                    extra[extras[1]] = post2
                if act1:
                    extra[extras[2]] = pre1

                q, k, v, p, z = {}, {}, {}, {}, {}
                s_at = {h: h + lS for h in range(H)}
                p_at = {h: h + lP for h in range(H)}
                w_at = {h: h + lW for h in range(H)}
                for d, extra_lag in enumerate(tail):
                    p_at[H - 1 - d] += extra_lag
                fin = []
                accv = acc.at[0:rows]
                for i in range(max(w_at.values()) + 1):
                    for op in order:
                        if op == 'q' and i < H:
                            q[i] = proj(i, 0, False)
                        if op == 'k' and i < H:
                            k[i] = proj(i, 1, True)
                        if op == 'v' and i < H:
                            v[i] = proj(i, 2, True)
                        for h in range(H):
                            if op == 'S' and s_at[h] == i:
                                p[h] = scores(q.pop(h), k.pop(h))
                            if op == 'P' and p_at[h] == i:
                                z[h] = pv(p.pop(h), v.pop(h))
                            if op == 'W' and w_at[h] == i:
                                r = wout(h, z.pop(h))
                                if h == 0:
                                    accv[...] = r
                                elif h == H - 1:
                                    fin.append(accv[...] + r)
                                else:
                                    accv[...] += r
                    if i in extra:
                        extra[i]()
                assert not (q or k or v or p or z)
                a = fin[0]
                mp = _pack16(a[0:2 * M, :])
                if act2:
                    hbuf[npar, MO:MO + MB, :] = mp
                else:
                    hbuf[npar, MO:MO + MB // 2, :] = mp[0:MB // 2]
                    hbuf[npar, MO + MB // 2:MO + MB, :] = _pack16(mem0[...].astype(F32))
                if act1 and act2:
                    ox[...] = a[2 * M:R, :]
                elif act1:
                    ox[0:seg, :] = a[2 * M:, :]
                else:
                    ox[seg:2 * seg, :] = a[2 * M:, :]
            return step

        def run_steps(t0, t1, step, unroll=1):
            if unroll == 1:
                lax.fori_loop(t0, t1, lambda t, c: step(t, t & 1), None)
                return
            assert unroll % 2 == 0 and (t1 - t0) % unroll == 0

            def body(i, c):
                for u in range(unroll):
                    step(t0 + i * unroll + u, (t0 + u) & 1)
            lax.fori_loop(0, (t1 - t0) // unroll, body, None)

        with scope('s1'):
            run_steps(0, LAG, make_step(True, False, False), cfg.get("s1u", 1))
        c_xb.wait()
        nboth = nsteps - LAG
        with scope('bp'):
            run_steps(LAG, min(LAG + NS, nboth), make_step(True, True, True), cfg.get("bpu", 1))
        if nboth > LAG + NS:
            with scope('b'):
                run_steps(LAG + NS, nboth, make_step(True, True, False), cfg.get("unroll", 2))
        OA = (NSEG - LAG - 1) * seg
        c_oa = pltpu.make_async_copy(ob.at[pl.ds(0, OA)], o_hbm.at[pl.ds(0, OA)], sem_out.at[0])
        c_oa.start()
        with scope('s2'):
            run_steps(NSEG, NSEG + LAG, make_step(False, True, False), cfg.get("s2u", 1))
        finish(NSEG - 1, (NSEG - 1) * seg)
        c_ob = pltpu.make_async_copy(ob.at[pl.ds(OA, S - OA)], o_hbm.at[pl.ds(OA, S - OA)],
                                     sem_out.at[1])
        c_ob.start()
        c_oa.wait()
        c_ob.wait()

    scratch = [
        pltpu.VMEM((3, H + 2, Dm // 2, Dh), U32),
        pltpu.VMEM((3, HP, Dm, Dh), U32),
        pltpu.VMEM((H, Dh // 2, Dm), U32),
        pltpu.VMEM((S, Dm), BF16),
        pltpu.VMEM((KPAD + S, Dm), BF16),
        pltpu.VMEM((S, Dm), BF16),
        pltpu.VMEM((NCH, Dm, CH), BF16),
        pltpu.VMEM((S, Dm), BF16),
        pltpu.VMEM((NCH, 2 * CH, Dm), F32),
        pltpu.VMEM((NCH, 2 * CH, Dm), F32),
        pltpu.VMEM((2 * CH, Dm), F32),
        pltpu.VMEM((S, Dm), F32),
        pltpu.VMEM((2, R // 2, Dm), U32),
        pltpu.VMEM((NS * seg // 2, Dm), U32),
        pltpu.VMEM((3, H, NS * seg, Dh), F32),
        pltpu.VMEM((R, Dm), F32),
        pltpu.VMEM((NSEG + LAG + 1, seg, Dm), F32),
        pltpu.VMEM((2 * seg, Dm), F32),
        pltpu.VMEM((S, Dm), BF16),
        pltpu.VMEM((CH, CH), U32),
        pltpu.VMEM((CH // 2, 2 * CH), U32),
        pltpu.VMEM((R + 2 * (2 * M + seg), 128), F32),
        pltpu.VMEM((M, Dm), BF16),
        pltpu.VMEM((KS, Dm), BF16),
        pltpu.VMEM((Dm,), BF16),
        pltpu.SemaphoreType.DMA((6,)),
        pltpu.SemaphoreType.DMA((NCH,)),
        pltpu.SemaphoreType.DMA((NCH,)),
        pltpu.SemaphoreType.DMA((NCH,)),
        pltpu.SemaphoreType.DMA((3, HP)),
        pltpu.SemaphoreType.DMA((4,)),
        pltpu.SemaphoreType.DMA((2,)),
        pltpu.SemaphoreType.DMA((2,)),
    ]
    return kernel, scratch


def _run(A_x, A_mem0, A_Wq, A_Wk, A_Wv, A_Wo, A_seg_len, B_k, B_v, B_shift_k, B_ssm_k, B_ssm_D,
         cfg=None):
    B, S, Dm = A_x.shape
    assert B == 1
    _, H, Dh = A_Wq.shape
    M = A_mem0.shape[1]
    seg = int(A_seg_len)
    KS = B_shift_k.shape[-1]
    kernel, scratch = _build(S, Dm, H, Dh, M, seg, KS, cfg or {})
    fa_np, fi_np = _dft_mats()
    bias_np = _attn_bias(M, seg)
    args = (A_x.reshape(S, Dm), A_mem0.reshape(M, Dm), A_Wq, A_Wk, A_Wv, A_Wo,
            B_k.reshape(S, Dm), B_v.reshape(S, Dm), B_shift_k.T, B_ssm_k, B_ssm_D,
            fa_np, fi_np, bias_np)
    out = pl.pallas_call(
        kernel,
        out_shape=jax.ShapeDtypeStruct((S, Dm), BF16),
        in_specs=[pl.BlockSpec(memory_space=pl.ANY)] * len(args),
        out_specs=pl.BlockSpec(memory_space=pl.ANY),
        scratch_shapes=scratch,
        compiler_params=pltpu.CompilerParams(vmem_limit_bytes=110 * 1024 * 1024,
                                             flags=(cfg or {}).get("flags")),
    )(*args)
    return out.reshape(B, S, Dm)


@functools.partial(jax.jit, static_argnames=("A_seg_len",))
def pallas_interleave_layers__memory_aug_recurrent_mem_tr__ssm_conv_h3__prompt_kernel(
    A_x: jax.Array,
    A_mem0: jax.Array,
    A_Wq: jax.Array,
    A_Wk: jax.Array,
    A_Wv: jax.Array,
    A_Wo: jax.Array,
    A_seg_len: int,
    B_q: jax.Array,
    B_k: jax.Array,
    B_v: jax.Array,
    B_shift_k: jax.Array,
    B_ssm_k: jax.Array,
    B_ssm_D: jax.Array,
):
    del B_q
    return _run(A_x, A_mem0, A_Wq, A_Wk, A_Wv, A_Wo, A_seg_len, B_k, B_v, B_shift_k,
                B_ssm_k, B_ssm_D)
```

```python
import functools

import jax
import jax.numpy as jnp
import numpy as np
from jax import lax
from jax.experimental import pallas as pl
from jax.experimental.pallas import tpu as pltpu

F32, BF16, U32 = jnp.float32, jnp.bfloat16, jnp.uint32

LOG2E = 1.4426950408889634
LN_EPS = 1e-5
CH = 128
LAG = 2
KPAD = 16


def _np_pack16(a):
    h = np.asarray(a, dtype=np.float32).astype(BF16).view(np.uint16).astype(np.uint32)
    return h[0::2] | (h[1::2] << 16)


def _dft_mats():
    n2 = 2 * CH
    karr = np.concatenate([np.arange(0, CH, 2), np.arange(1, CH, 2)])
    n = np.arange(CH)
    th = 2.0 * np.pi * n[None, :] * (karr[:, None] + 0.5) / n2
    fa = np.concatenate([np.cos(th), -np.sin(th)], axis=0)
    fi = np.concatenate([np.cos(th).T, -np.sin(th).T], axis=1) * (2.0 / n2)
    return _np_pack16(fa), _np_pack16(fi)


def _attn_bias(m, seg):
    stream = np.concatenate([np.zeros(seg), np.ones(seg), np.zeros(m), np.ones(m)])
    ismem = np.concatenate([np.zeros(2 * seg), np.ones(2 * m)]).astype(bool)
    pos = np.concatenate([np.arange(seg), np.arange(seg), np.zeros(2 * m)])
    same = stream[:, None] == stream[None, :]
    keep = ismem[:, None] | ismem[None, :] | (pos[:, None] >= pos[None, :])
    full = np.where(same & keep, 0.0, np.where(same, -1e9 * LOG2E, -1e30))
    s1, s2, mm = np.arange(seg), np.arange(seg, 2 * seg), np.arange(2 * seg, 2 * seg + 2 * m)
    out = []
    for sel in (np.concatenate([s1, s2, mm]), np.concatenate([s1, mm]), np.concatenate([s2, mm])):
        b = np.full((len(sel), 128), -1e30, np.float32)
        b[:, :len(sel)] = full[sel][:, sel]
        out.append(b)
    return np.concatenate(out, axis=0)


def _ln(x):
    m = jnp.mean(x, axis=-1, keepdims=True)
    xc = x - m
    v = jnp.mean(xc * xc, axis=-1, keepdims=True)
    return xc * lax.rsqrt(v + LN_EPS)


def _pack16(x):
    return pltpu.bitcast(x.astype(BF16), U32)


def _build(S, Dm, H, Dh, M, seg, KS, cfg):
    assert Dh == 128 and Dm % 128 == 0 and S % CH == 0 and H % 16 == 0
    assert M == 8 and seg == 32 and KS <= 8
    NSEG = S // seg
    NCH = S // CH
    NT = Dm // 128
    R = 2 * (M + seg)
    HP = H // 2
    qk_scale = float(Dh ** -0.5) * LOG2E
    LAGS = {"b": (2, 4, 12, (3, 2, 1)), "bp": (2, 4, 12, (3, 2, 1, 1)), "1": (2, 4, 12, (4, 3, 2, 1)),
            "2": (2, 4, 12, (4, 3, 2, 1))}
    order = cfg.get("order", "qSkPvW")
    extras = cfg.get("extras", (3, 11, 19))
    nsteps = cfg.get("nsteps", NSEG + LAG)
    skip = cfg.get("skip", "")
    NS = cfg.get("ns", 10)
    assert 0 < NS and LAG + NS <= NSEG - 1

    import contextlib
    scope = jax.named_scope if cfg.get("scopes") else (lambda n: contextlib.nullcontext())

    def kernel(x_hbm, mem0_hbm, wq_hbm, wk_hbm, wv_hbm, wo_hbm, k_hbm, v_hbm, sh_hbm, h_hbm,
               d_hbm, fa_hbm, fi_hbm, bias_hbm, o_hbm,
               wqkv, wstage, wo, x0, kb, vb, hb, ub, Ub, Gb, Ap, yb,
               hbuf, hx, qkvx, acc, x2buf, ox, ob, fa, fi, bias, mem0, shv, dv,
               sem_c, sem_k, sem_v, sem_h, sem_w, sem_o, sem_x, sem_out):
        c_fa = pltpu.make_async_copy(fa_hbm, fa, sem_c.at[0])
        c_sh = pltpu.make_async_copy(sh_hbm, shv, sem_c.at[1])
        c_fi = pltpu.make_async_copy(fi_hbm, fi, sem_c.at[2])
        c_d = pltpu.make_async_copy(d_hbm, dv, sem_c.at[3])
        c_bias = pltpu.make_async_copy(bias_hbm, bias, sem_c.at[4])
        c_mem0 = pltpu.make_async_copy(mem0_hbm, mem0, sem_c.at[5])

        def cp_k(j):
            return pltpu.make_async_copy(
                k_hbm.at[pl.ds(j * CH, CH)], kb.at[pl.ds(KPAD + j * CH, CH)], sem_k.at[j])

        def cp_v(j):
            return pltpu.make_async_copy(
                v_hbm.at[pl.ds(j * CH, CH)], vb.at[pl.ds(j * CH, CH)], sem_v.at[j])

        def cp_h(j):
            return pltpu.make_async_copy(
                h_hbm.at[:, pl.ds(j * CH, CH)], hb.at[j], sem_h.at[j])

        w32 = [w.bitcast(U32) for w in (wq_hbm, wk_hbm, wv_hbm)]

        def cp_w(j, s):
            return pltpu.make_async_copy(w32[j].at[:, s, :], wstage.at[j, s], sem_w.at[j, s])

        wo32 = wo_hbm.bitcast(U32)
        NWO = 4
        c_wo = [pltpu.make_async_copy(wo32.at[pl.ds(i * (H // NWO), H // NWO)],
                                      wo.at[pl.ds(i * (H // NWO), H // NWO)], sem_o.at[i])
                for i in range(NWO)]
        XA = (LAG + NS) * seg
        c_xa = pltpu.make_async_copy(x_hbm.at[pl.ds(0, XA)], x0.at[pl.ds(0, XA)], sem_x.at[0])
        c_xb = pltpu.make_async_copy(x_hbm.at[pl.ds(XA, S - XA)], x0.at[pl.ds(XA, S - XA)],
                                     sem_x.at[1])

        WIN = cfg.get("win", 4)
        WST = cfg.get("wst", NCH - 4)
        WW = cfg.get("ww", 3)
        assert 0 <= WST and WST + WW <= NCH

        def start_chunk(j):
            cp_k(j).start()
            cp_v(j).start()
            cp_h(j).start()

        def start_slab(s):
            for j in range(3):
                cp_w(j, s).start()

        start_chunk(0)
        c_fa.start()
        c_sh.start()
        for j in range(1, WIN):
            start_chunk(j)
        c_fi.start()
        c_d.start()
        c_bias.start()
        c_mem0.start()
        c_xa.start()

        hbuf[...] = jnp.zeros(hbuf.shape, U32)
        x2buf[0] = jnp.zeros(x2buf.shape[1:], F32)
        ox[...] = jnp.zeros(ox.shape, F32)
        kb[0:KPAD, :] = jnp.zeros((KPAD, Dm), BF16)
        Ap[...] = jnp.zeros(Ap.shape, F32)
        with scope('wait_fa'):
            c_fa.wait()
        c_sh.wait()
        sh = shv[...].astype(F32)

        def fwd(j, carry):
            cp_k(j).wait()
            cp_v(j).wait()
            cp_h(j).wait()

            @pl.when(j + WIN < NCH)
            def _():
                start_chunk(j + WIN)

            @pl.when(j >= WST)
            def _():
                @pl.when(j < WST + WW)
                def _():
                    start_slab(j - WST)
            r0 = pl.multiple_of(j * CH, CH)
            kf = kb[pl.ds(r0, CH + KPAD), :].astype(F32)
            ks = kf[KPAD:KPAD + CH] * sh[0:1]
            for dlt in range(1, KS):
                ks = ks + kf[KPAD - dlt:KPAD - dlt + CH] * sh[dlt:dlt + 1]
            u = (ks * vb[pl.ds(r0, CH), :].astype(F32)).astype(BF16)
            ub[pl.ds(r0, CH), :] = u
            fav = pltpu.bitcast(fa[...], BF16)
            Ub[j] = jnp.dot(fav, u, preferred_element_type=F32)
            a = lax.dot_general(fav, hb[j], (((1,), (1,)), ((), ())),
                                preferred_element_type=F32)
            p = Ap[...]
            hh = CH // 2
            Gb[j, 0:hh] = a[0:hh] - p[CH:CH + hh]
            Gb[j, hh:CH] = a[hh:CH] + p[CH + hh:2 * CH]
            Gb[j, CH:CH + hh] = a[CH:CH + hh] + p[0:hh]
            Gb[j, CH + hh:2 * CH] = a[CH + hh:2 * CH] - p[hh:CH]
            Ap[...] = a
            return carry
        with scope('fwd'):
            lax.fori_loop(0, NCH, fwd, 0)

        BL = cfg.get("bl", 4)
        MCH = cfg.get("mch", 64)

        with scope('wait_xa'):
            c_xa.wait()
        for i in range(NS):
            hx[i * seg // 2:(i + 1) * seg // 2, :] = _pack16(
                _ln(x0[(LAG + i) * seg:(LAG + i + 1) * seg, :].astype(F32)))

        def repack(s, j):
            src = jnp.minimum(s, HP - 1)
            a = wstage[j, src, pl.ds(0, Dm // 2, stride=2), :]
            b = wstage[j, src, pl.ds(1, Dm // 2, stride=2), :]
            wqkv[j, 2 * s] = (a & jnp.uint32(0xFFFF)) | (b << 16)
            wqkv[j, 2 * s + 1] = (a >> 16) | (b & jnp.uint32(0xFFFF0000))

        def run_ahead(s, j, hh, m0):
            w = pltpu.bitcast(wqkv[j, 2 * s + hh], BF16)
            lhs = pltpu.bitcast(hx[m0 // 2:(m0 + MCH) // 2, :], BF16)
            qkvx[j, 2 * s + hh, m0:m0 + MCH, :] = jnp.dot(lhs, w, preferred_element_type=F32)

        assert HP == CH // 8 == NCH
        CS = cfg.get("cs", 5)

        def mac_gen(f, c, ib):
            rr = pl.multiple_of(f * 8, 8)
            ri = pl.multiple_of(CH + f * 8, 8)
            cs = slice(c * 128, (c + 1) * 128)
            yr = [None] * BL
            yi = [None] * BL
            for jb in range(ib + 1):
                for jj in range(BL):
                    J = jb * BL + jj
                    ur = Ub[J, pl.ds(rr, 8), cs]
                    ui = Ub[J, pl.ds(ri, 8), cs]
                    n = 0
                    for ii in range(BL):
                        I = ib * BL + ii
                        if I < J:
                            continue
                        gr = Gb[I - J, pl.ds(rr, 8), cs]
                        gi = Gb[I - J, pl.ds(ri, 8), cs]
                        tr = gr * ur - gi * ui
                        ti = gr * ui + gi * ur
                        yr[ii] = tr if yr[ii] is None else yr[ii] + tr
                        yi[ii] = ti if yi[ii] is None else yi[ii] + ti
                        n += 1
                    yield n
            for ii in range(BL):
                Ub[ib * BL + ii, pl.ds(rr, 8), cs] = yr[ii]
                Ub[ib * BL + ii, pl.ds(ri, 8), cs] = yi[ii]
            yield 0

        def mac_stream(f, ctiles):
            for c in (ctiles if 'm' not in skip else []):
                for ib in reversed(range(NCH // BL)):
                    yield from mac_gen(f, c, ib)

        def interleave(mxu, vpu, tot):
            nm = sum(w for _, w in mxu)
            done = dm = 0
            for fn, w in mxu:
                fn()
                dm += w
                while done < tot * dm / nm:
                    n = next(vpu, None)
                    if n is None:
                        break
                    done += n
            for _ in vpu:
                pass

        def slab_arrived(s):
            for j in range(3):
                cp_w(j, s).wait()

            @pl.when(s + WW < HP)
            def _():
                start_slab(s + WW)

            @pl.when(s + WW == HP)
            def _():
                for c in c_wo:
                    c.start()

        PIPE = cfg.get("pipe", 0)
        SU = cfg.get("su", 2)

        def slab(f):
            mxu = []
            for j in range(3):
                if not PIPE:
                    mxu.append((functools.partial(repack, f, j), 0))
                for hh in range(2):
                    for m0 in range(0, NS * seg, MCH):
                        mxu.append((functools.partial(run_ahead, f, j, hh, m0), 1))
                if PIPE:
                    mxu.append((functools.partial(repack, f + 1, j), 0))
            interleave(mxu, mac_stream(f, range(CS)), CS * NCH * (NCH + 1) // 2)

        def slab_body(i, carry):
            for u in range(SU):
                f = i * SU + u
                if PIPE:
                    @pl.when(f + 1 < HP)
                    def _():
                        slab_arrived(f + 1)
                else:
                    slab_arrived(f)
            for u in range(SU):
                slab(i * SU + u)
            return carry
        with scope('slab'):
            if PIPE:
                slab_arrived(0)
                for j in range(3):
                    repack(0, j)
            lax.fori_loop(0, HP // SU, slab_body, 0)

        c_fi.wait()
        c_d.wait()
        dvec = dv[...].astype(F32).reshape(1, Dm)

        def inv(i, c):
            r0 = pl.multiple_of(i * CH, CH)
            cs = slice(c * 128, (c + 1) * 128)
            y = jnp.dot(pltpu.bitcast(fi[...], BF16), Ub[i, :, cs].astype(BF16), preferred_element_type=F32)
            yb[pl.ds(r0, CH), cs] = y + ub[pl.ds(r0, CH), cs].astype(F32) * dvec[:, cs]

        def inv_a(i, carry):
            interleave([(functools.partial(inv, i, c), 1) for c in range(CS)],
                       mac_stream(i, range(CS, NT)), (NT - CS) * NCH * (NCH + 1) // 2)
            return carry

        def inv_b(i, carry):
            for c in range(CS, NT):
                inv(i, c)
            return carry
        with scope('inv_a'):
            lax.fori_loop(0, NCH, inv_a, 0, unroll=cfg.get("iu", 4))
        if CS < NT:
            lax.fori_loop(0, NCH, inv_b, 0, unroll=4)

        c_bias.wait()
        c_mem0.wait()
        with scope('wait_wo'):
            for c in c_wo:
                c.wait()
        c_xb.start()
        MB = M
        XB = seg // 2
        MO = 2 * XB
        hbuf[0, MO:MO + MB // 2, :] = _pack16(mem0[...].astype(F32))
        hbuf[0, 0:XB, :] = _pack16(_ln(x0[0:seg, :].astype(F32)))

        def finish(s, r0):
            x3 = x2buf[s + 1] + ox[seg:2 * seg, :]
            x4 = x3 + _ln(x3) * yb[pl.ds(r0, seg), :]
            ob[pl.ds(r0, seg), :] = x4.astype(BF16)

        def make_step(act1, act2, pre):
            rows = 2 * M + seg * (int(act1) + int(act2))
            b0 = 0 if (act1 and act2) else R if act1 else R + 2 * M + seg
            x1_in_lhs = act1 and not pre

            key = "b" if (act1 and act2 and not pre) else "bp" if (act1 and act2) else "1" if act1 else "2"
            lS, lP, lW, tail = cfg.get("lag_" + key, LAGS[key])

            def step(t, par):
                npar = 1 - par
                parts = []
                if x1_in_lhs:
                    parts.append(hbuf[par, 0:XB, :])
                if act2:
                    parts.append(hbuf[par, XB:2 * XB, :])
                parts.append(hbuf[par, MO:MO + MB, :])
                hh = pltpu.bitcast(parts[0] if len(parts) == 1 else jnp.concatenate(parts, axis=0), BF16)
                zpad = jnp.zeros((128 - rows, Dh), F32)

                def proj(h, j, padded):
                    r = jnp.dot(hh, pltpu.bitcast(wqkv[j, h], BF16), preferred_element_type=F32)
                    blocks = [r]
                    if pre:
                        x1p = qkvx[j, h, pl.ds(pl.multiple_of((t - LAG) * seg, seg), seg), :]
                        blocks = [x1p, r]
                    if padded:
                        blocks.append(zpad)
                    u = blocks[0] if len(blocks) == 1 else jnp.concatenate(blocks, axis=0)
                    return u.astype(BF16)

                def scores(q, k):
                    s = lax.dot_general(q, k, (((1,), (1,)), ((), ())), preferred_element_type=F32)
                    s = s * qk_scale + bias[b0:b0 + rows, :]
                    m = jnp.max(s, axis=-1, keepdims=True)
                    p = jnp.exp2(s - m)
                    l = jnp.sum(p, axis=-1, keepdims=True)
                    r = pl.reciprocal(l, approx=True)
                    r = r * (2.0 - l * r)
                    return (p * r).astype(BF16)

                def pv(p, v):
                    z = jnp.dot(p, v, preferred_element_type=F32)
                    return jnp.concatenate([z[rows - 2 * M:], z[:rows - 2 * M]], axis=0).astype(BF16)

                def wout(h, z):
                    return jnp.dot(z, pltpu.bitcast(wo[h], BF16), preferred_element_type=F32)

                def post1():
                    s = jnp.minimum(jnp.maximum(t - 1, 0), NSEG - 1)
                    r0 = pl.multiple_of(s * seg, seg)
                    x1 = x0[pl.ds(r0, seg), :].astype(F32) + ox[0:seg, :]
                    x2 = x1 + _ln(x1) * yb[pl.ds(r0, seg), :]
                    x2buf[t] = x2
                    hbuf[npar, XB:2 * XB, :] = _pack16(_ln(x2))

                def post2():
                    s = jnp.maximum(t - 1 - LAG, 0)
                    finish(s, pl.multiple_of(s * seg, seg))

                def pre1():
                    s = jnp.minimum(t + 1, NSEG - 1)
                    r0 = pl.multiple_of(s * seg, seg)
                    hbuf[npar, 0:XB, :] = _pack16(_ln(x0[pl.ds(r0, seg), :].astype(F32)))
                extra = {extras[0]: post1}
                if act2:
                    extra[extras[1]] = post2
                if act1:
                    extra[extras[2]] = pre1

                q, k, v, p, z = {}, {}, {}, {}, {}
                s_at = {h: h + lS for h in range(H)}
                p_at = {h: h + lP for h in range(H)}
                w_at = {h: h + lW for h in range(H)}
                for d, extra_lag in enumerate(tail):
                    p_at[H - 1 - d] += extra_lag
                fin = []
                accv = acc.at[0:rows]
                for i in range(max(w_at.values()) + 1):
                    for op in order:
                        if op == 'q' and i < H:
                            q[i] = proj(i, 0, False)
                        if op == 'k' and i < H:
                            k[i] = proj(i, 1, True)
                        if op == 'v' and i < H:
                            v[i] = proj(i, 2, True)
                        for h in range(H):
                            if op == 'S' and s_at[h] == i:
                                p[h] = scores(q.pop(h), k.pop(h))
                            if op == 'P' and p_at[h] == i:
                                z[h] = pv(p.pop(h), v.pop(h))
                            if op == 'W' and w_at[h] == i:
                                r = wout(h, z.pop(h))
                                if h == 0:
                                    accv[...] = r
                                elif h == H - 1:
                                    fin.append(accv[...] + r)
                                else:
                                    accv[...] += r
                    if i in extra:
                        extra[i]()
                assert not (q or k or v or p or z)
                a = fin[0]
                mp = _pack16(a[0:2 * M, :])
                if act2:
                    hbuf[npar, MO:MO + MB, :] = mp
                else:
                    hbuf[npar, MO:MO + MB // 2, :] = mp[0:MB // 2]
                    hbuf[npar, MO + MB // 2:MO + MB, :] = _pack16(mem0[...].astype(F32))
                if act1 and act2:
                    ox[...] = a[2 * M:R, :]
                elif act1:
                    ox[0:seg, :] = a[2 * M:, :]
                else:
                    ox[seg:2 * seg, :] = a[2 * M:, :]
            return step

        def run_steps(t0, t1, step, unroll=1):
            if unroll == 1:
                lax.fori_loop(t0, t1, lambda t, c: step(t, t & 1), None)
                return
            assert unroll % 2 == 0 and (t1 - t0) % unroll == 0

            def body(i, c):
                for u in range(unroll):
                    step(t0 + i * unroll + u, (t0 + u) & 1)
            lax.fori_loop(0, (t1 - t0) // unroll, body, None)

        with scope('s1'):
            run_steps(0, LAG, make_step(True, False, False), cfg.get("s1u", 1))
        c_xb.wait()
        nboth = nsteps - LAG
        with scope('bp'):
            run_steps(LAG, min(LAG + NS, nboth), make_step(True, True, True), cfg.get("bpu", 1))
        if nboth > LAG + NS:
            with scope('b'):
                run_steps(LAG + NS, nboth, make_step(True, True, False), cfg.get("unroll", 2))
        OA = (NSEG - LAG - 1) * seg
        c_oa = pltpu.make_async_copy(ob.at[pl.ds(0, OA)], o_hbm.at[pl.ds(0, OA)], sem_out.at[0])
        c_oa.start()
        with scope('s2'):
            run_steps(NSEG, NSEG + LAG, make_step(False, True, False), cfg.get("s2u", 1))
        OB = (NSEG - 1) * seg
        c_ob = pltpu.make_async_copy(ob.at[pl.ds(OA, OB - OA)], o_hbm.at[pl.ds(OA, OB - OA)],
                                     sem_out.at[1])
        c_ob.start()
        finish(NSEG - 1, OB)
        c_oc = pltpu.make_async_copy(ob.at[pl.ds(OB, S - OB)], o_hbm.at[pl.ds(OB, S - OB)],
                                     sem_out.at[2])
        c_oc.start()
        c_oa.wait()
        c_ob.wait()
        c_oc.wait()

    scratch = [
        pltpu.VMEM((3, H + 2, Dm // 2, Dh), U32),
        pltpu.VMEM((3, HP, Dm, Dh), U32),
        pltpu.VMEM((H, Dh // 2, Dm), U32),
        pltpu.VMEM((S, Dm), BF16),
        pltpu.VMEM((KPAD + S, Dm), BF16),
        pltpu.VMEM((S, Dm), BF16),
        pltpu.VMEM((NCH, Dm, CH), BF16),
        pltpu.VMEM((S, Dm), BF16),
        pltpu.VMEM((NCH, 2 * CH, Dm), F32),
        pltpu.VMEM((NCH, 2 * CH, Dm), F32),
        pltpu.VMEM((2 * CH, Dm), F32),
        pltpu.VMEM((S, Dm), F32),
        pltpu.VMEM((2, R // 2, Dm), U32),
        pltpu.VMEM((NS * seg // 2, Dm), U32),
        pltpu.VMEM((3, H, NS * seg, Dh), F32),
        pltpu.VMEM((R, Dm), F32),
        pltpu.VMEM((NSEG + LAG + 1, seg, Dm), F32),
        pltpu.VMEM((2 * seg, Dm), F32),
        pltpu.VMEM((S, Dm), BF16),
        pltpu.VMEM((CH, CH), U32),
        pltpu.VMEM((CH // 2, 2 * CH), U32),
        pltpu.VMEM((R + 2 * (2 * M + seg), 128), F32),
        pltpu.VMEM((M, Dm), BF16),
        pltpu.VMEM((KS, Dm), BF16),
        pltpu.VMEM((Dm,), BF16),
        pltpu.SemaphoreType.DMA((6,)),
        pltpu.SemaphoreType.DMA((NCH,)),
        pltpu.SemaphoreType.DMA((NCH,)),
        pltpu.SemaphoreType.DMA((NCH,)),
        pltpu.SemaphoreType.DMA((3, HP)),
        pltpu.SemaphoreType.DMA((4,)),
        pltpu.SemaphoreType.DMA((2,)),
        pltpu.SemaphoreType.DMA((3,)),
    ]
    return kernel, scratch


def _run(A_x, A_mem0, A_Wq, A_Wk, A_Wv, A_Wo, A_seg_len, B_k, B_v, B_shift_k, B_ssm_k, B_ssm_D,
         cfg=None):
    B, S, Dm = A_x.shape
    assert B == 1
    _, H, Dh = A_Wq.shape
    M = A_mem0.shape[1]
    seg = int(A_seg_len)
    KS = B_shift_k.shape[-1]
    kernel, scratch = _build(S, Dm, H, Dh, M, seg, KS, cfg or {})
    fa_np, fi_np = _dft_mats()
    bias_np = _attn_bias(M, seg)
    args = (A_x.reshape(S, Dm), A_mem0.reshape(M, Dm), A_Wq, A_Wk, A_Wv, A_Wo,
            B_k.reshape(S, Dm), B_v.reshape(S, Dm), B_shift_k.T, B_ssm_k, B_ssm_D,
            fa_np, fi_np, bias_np)
    out = pl.pallas_call(
        kernel,
        out_shape=jax.ShapeDtypeStruct((S, Dm), BF16),
        in_specs=[pl.BlockSpec(memory_space=pl.ANY)] * len(args),
        out_specs=pl.BlockSpec(memory_space=pl.ANY),
        scratch_shapes=scratch,
        compiler_params=pltpu.CompilerParams(vmem_limit_bytes=110 * 1024 * 1024,
                                             flags=(cfg or {}).get("flags")),
    )(*args)
    return out.reshape(B, S, Dm)


@functools.partial(jax.jit, static_argnames=("A_seg_len",))
def pallas_interleave_layers__memory_aug_recurrent_mem_tr__ssm_conv_h3__prompt_kernel(
    A_x: jax.Array,
    A_mem0: jax.Array,
    A_Wq: jax.Array,
    A_Wk: jax.Array,
    A_Wv: jax.Array,
    A_Wo: jax.Array,
    A_seg_len: int,
    B_q: jax.Array,
    B_k: jax.Array,
    B_v: jax.Array,
    B_shift_k: jax.Array,
    B_ssm_k: jax.Array,
    B_ssm_D: jax.Array,
):
    del B_q
    return _run(A_x, A_mem0, A_Wq, A_Wk, A_Wv, A_Wo, A_seg_len, B_k, B_v, B_shift_k,
                B_ssm_k, B_ssm_D)
```

```python
import functools

import jax
import jax.numpy as jnp
import numpy as np
from jax import lax
from jax.experimental import pallas as pl
from jax.experimental.pallas import tpu as pltpu

F32, BF16, U32 = jnp.float32, jnp.bfloat16, jnp.uint32

LOG2E = 1.4426950408889634
LN_EPS = 1e-5
CH = 128
LAG = 2
KPAD = 16


def _np_pack16(a):
    h = np.asarray(a, dtype=np.float32).astype(BF16).view(np.uint16).astype(np.uint32)
    return h[0::2] | (h[1::2] << 16)


def _dft_mats():
    n2 = 2 * CH
    karr = np.concatenate([np.arange(0, CH, 2), np.arange(1, CH, 2)])
    n = np.arange(CH)
    th = 2.0 * np.pi * n[None, :] * (karr[:, None] + 0.5) / n2
    fa = np.concatenate([np.cos(th), -np.sin(th)], axis=0)
    fi = np.concatenate([np.cos(th).T, -np.sin(th).T], axis=1) * (2.0 / n2)
    return _np_pack16(fa), _np_pack16(fi)


def _attn_bias(m, seg):
    stream = np.concatenate([np.zeros(seg), np.ones(seg), np.zeros(m), np.ones(m)])
    ismem = np.concatenate([np.zeros(2 * seg), np.ones(2 * m)]).astype(bool)
    pos = np.concatenate([np.arange(seg), np.arange(seg), np.zeros(2 * m)])
    same = stream[:, None] == stream[None, :]
    keep = ismem[:, None] | ismem[None, :] | (pos[:, None] >= pos[None, :])
    full = np.where(same & keep, 0.0, np.where(same, -1e9 * LOG2E, -1e30))
    s1, s2, mm = np.arange(seg), np.arange(seg, 2 * seg), np.arange(2 * seg, 2 * seg + 2 * m)
    out = []
    for sel in (np.concatenate([s1, s2, mm]), np.concatenate([s1, mm]), np.concatenate([s2, mm])):
        b = np.full((len(sel), 128), -1e30, np.float32)
        b[:, :len(sel)] = full[sel][:, sel]
        out.append(b)
    return np.concatenate(out, axis=0)


def _ln(x):
    m = jnp.mean(x, axis=-1, keepdims=True)
    xc = x - m
    v = jnp.mean(xc * xc, axis=-1, keepdims=True)
    return xc * lax.rsqrt(v + LN_EPS)


def _pack16(x):
    return pltpu.bitcast(x.astype(BF16), U32)


def _build(S, Dm, H, Dh, M, seg, KS, cfg):
    assert Dh == 128 and Dm % 128 == 0 and S % CH == 0 and H % 16 == 0
    assert M == 8 and seg == 32 and KS <= 8
    NSEG = S // seg
    NCH = S // CH
    NT = Dm // 128
    R = 2 * (M + seg)
    HP = H // 2
    qk_scale = float(Dh ** -0.5) * LOG2E
    LAGS = {"b": (2, 4, 12, (3, 2, 1)), "bp": (2, 4, 12, (3, 2, 1, 1)), "1": (2, 4, 12, (4, 3, 2, 1)),
            "2": (2, 4, 12, (4, 3, 2, 1))}
    order = cfg.get("order", "qSkPvW")
    extras = cfg.get("extras", (3, 11, 19))
    NS = cfg.get("ns", 10)
    assert 0 < NS and LAG + NS <= NSEG - 1 and (NSEG - LAG - NS) % 2 == 0

    def kernel(x_hbm, mem0_hbm, wq_hbm, wk_hbm, wv_hbm, wo_hbm, k_hbm, v_hbm, sh_hbm, h_hbm,
               d_hbm, fa_hbm, fi_hbm, bias_hbm, o_hbm,
               wqkv, wstage, wo, x0, kb, vb, hb, ub, Ub, Gb, Ap, yb,
               hbuf, hx, qkvx, acc, x2buf, ox, ob, fa, fi, bias, mem0, shv, dv,
               sem_c, sem_k, sem_v, sem_h, sem_w, sem_o, sem_x, sem_out):
        c_fa = pltpu.make_async_copy(fa_hbm, fa, sem_c.at[0])
        c_sh = pltpu.make_async_copy(sh_hbm, shv, sem_c.at[1])
        c_fi = pltpu.make_async_copy(fi_hbm, fi, sem_c.at[2])
        c_d = pltpu.make_async_copy(d_hbm, dv, sem_c.at[3])
        c_bias = pltpu.make_async_copy(bias_hbm, bias, sem_c.at[4])
        c_mem0 = pltpu.make_async_copy(mem0_hbm, mem0, sem_c.at[5])

        def cp_k(j):
            return pltpu.make_async_copy(
                k_hbm.at[pl.ds(j * CH, CH)], kb.at[pl.ds(KPAD + j * CH, CH)], sem_k.at[j])

        def cp_v(j):
            return pltpu.make_async_copy(
                v_hbm.at[pl.ds(j * CH, CH)], vb.at[pl.ds(j * CH, CH)], sem_v.at[j])

        def cp_h(j):
            return pltpu.make_async_copy(
                h_hbm.at[:, pl.ds(j * CH, CH)], hb.at[j], sem_h.at[j])

        w32 = [w.bitcast(U32) for w in (wq_hbm, wk_hbm, wv_hbm)]

        def cp_w(j, s):
            return pltpu.make_async_copy(w32[j].at[:, s, :], wstage.at[j, s], sem_w.at[j, s])

        wo32 = wo_hbm.bitcast(U32)
        NWO = 4
        c_wo = [pltpu.make_async_copy(wo32.at[pl.ds(i * (H // NWO), H // NWO)],
                                      wo.at[pl.ds(i * (H // NWO), H // NWO)], sem_o.at[i])
                for i in range(NWO)]
        XA = (LAG + NS) * seg
        c_xa = pltpu.make_async_copy(x_hbm.at[pl.ds(0, XA)], x0.at[pl.ds(0, XA)], sem_x.at[0])
        c_xb = pltpu.make_async_copy(x_hbm.at[pl.ds(XA, S - XA)], x0.at[pl.ds(XA, S - XA)],
                                     sem_x.at[1])

        WIN = cfg.get("win", 4)
        WST = cfg.get("wst", NCH - 5)
        WW = cfg.get("ww", 4)
        assert 0 <= WST and WST + WW <= NCH

        def start_chunk(j):
            cp_k(j).start()
            cp_v(j).start()
            cp_h(j).start()

        def start_slab(s):
            for j in range(3):
                cp_w(j, s).start()

        start_chunk(0)
        c_fa.start()
        c_sh.start()
        for j in range(1, WIN):
            start_chunk(j)
        c_fi.start()
        c_d.start()
        c_bias.start()
        c_mem0.start()
        c_xa.start()

        hbuf[...] = jnp.zeros(hbuf.shape, U32)
        x2buf[0] = jnp.zeros(x2buf.shape[1:], F32)
        ox[...] = jnp.zeros(ox.shape, F32)
        kb[0:KPAD, :] = jnp.zeros((KPAD, Dm), BF16)
        Ap[...] = jnp.zeros(Ap.shape, F32)
        c_fa.wait()
        c_sh.wait()
        sh = shv[...].astype(F32)

        def fwd(j, carry):
            cp_k(j).wait()
            cp_v(j).wait()
            cp_h(j).wait()

            @pl.when(j + WIN < NCH)
            def _():
                start_chunk(j + WIN)

            @pl.when(j >= WST)
            def _():
                @pl.when(j < WST + WW)
                def _():
                    start_slab(j - WST)
            r0 = pl.multiple_of(j * CH, CH)
            kf = kb[pl.ds(r0, CH + KPAD), :].astype(F32)
            ks = kf[KPAD:KPAD + CH] * sh[0:1]
            for dlt in range(1, KS):
                ks = ks + kf[KPAD - dlt:KPAD - dlt + CH] * sh[dlt:dlt + 1]
            u = (ks * vb[pl.ds(r0, CH), :].astype(F32)).astype(BF16)
            ub[pl.ds(r0, CH), :] = u
            fav = pltpu.bitcast(fa[...], BF16)
            Ub[j] = jnp.dot(fav, u, preferred_element_type=F32)
            a = lax.dot_general(fav, hb[j], (((1,), (1,)), ((), ())),
                                preferred_element_type=F32)
            p = Ap[...]
            hh = CH // 2
            Gb[j, 0:hh] = a[0:hh] - p[CH:CH + hh]
            Gb[j, hh:CH] = a[hh:CH] + p[CH + hh:2 * CH]
            Gb[j, CH:CH + hh] = a[CH:CH + hh] + p[0:hh]
            Gb[j, CH + hh:2 * CH] = a[CH + hh:2 * CH] - p[hh:CH]
            Ap[...] = a
            return carry
        lax.fori_loop(0, NCH, fwd, 0)

        BL = cfg.get("bl", 4)
        MCH = cfg.get("mch", 64)

        c_xa.wait()
        for i in range(NS):
            hx[i * seg // 2:(i + 1) * seg // 2, :] = _pack16(
                _ln(x0[(LAG + i) * seg:(LAG + i + 1) * seg, :].astype(F32)))

        def repack(s, j):
            a = wstage[j, s, pl.ds(0, Dm // 2, stride=2), :]
            b = wstage[j, s, pl.ds(1, Dm // 2, stride=2), :]
            wqkv[j, 2 * s] = (a & jnp.uint32(0xFFFF)) | (b << 16)
            wqkv[j, 2 * s + 1] = (a >> 16) | (b & jnp.uint32(0xFFFF0000))

        def run_ahead(s, j, hh, m0):
            w = pltpu.bitcast(wqkv[j, 2 * s + hh], BF16)
            lhs = pltpu.bitcast(hx[m0 // 2:(m0 + MCH) // 2, :], BF16)
            qkvx[j, 2 * s + hh, m0:m0 + MCH, :] = jnp.dot(lhs, w, preferred_element_type=F32)

        assert HP == CH // 8 == NCH

        def mac_gen(f, c, ib):
            rr = pl.multiple_of(f * 8, 8)
            ri = pl.multiple_of(CH + f * 8, 8)
            cs = slice(c * 128, (c + 1) * 128)
            yr = [None] * BL
            yi = [None] * BL
            for jb in range(ib + 1):
                for jj in range(BL):
                    J = jb * BL + jj
                    ur = Ub[J, pl.ds(rr, 8), cs]
                    ui = Ub[J, pl.ds(ri, 8), cs]
                    n = 0
                    for ii in range(BL):
                        I = ib * BL + ii
                        if I < J:
                            continue
                        gr = Gb[I - J, pl.ds(rr, 8), cs]
                        gi = Gb[I - J, pl.ds(ri, 8), cs]
                        tr = gr * ur - gi * ui
                        ti = gr * ui + gi * ur
                        yr[ii] = tr if yr[ii] is None else yr[ii] + tr
                        yi[ii] = ti if yi[ii] is None else yi[ii] + ti
                        n += 1
                    yield n
            for ii in range(BL):
                Ub[ib * BL + ii, pl.ds(rr, 8), cs] = yr[ii]
                Ub[ib * BL + ii, pl.ds(ri, 8), cs] = yi[ii]
            yield 0

        def mac_stream(f):
            for c in range(NT):
                for ib in reversed(range(NCH // BL)):
                    yield from mac_gen(f, c, ib)

        def interleave(mxu, vpu, tot):
            nm = sum(w for _, w in mxu)
            done = dm = 0
            for fn, w in mxu:
                fn()
                dm += w
                while done < tot * dm / nm:
                    n = next(vpu, None)
                    if n is None:
                        break
                    done += n
            for _ in vpu:
                pass

        def slab_arrived(s):
            for j in range(3):
                cp_w(j, s).wait()

            @pl.when(s + WW < HP)
            def _():
                start_slab(s + WW)

            @pl.when(s + WW == HP)
            def _():
                for c in c_wo:
                    c.start()

        def slab(f):
            mxu = []
            for j in range(3):
                mxu.append((functools.partial(repack, f, j), 0))
                for hh in range(2):
                    for m0 in range(0, NS * seg, MCH):
                        mxu.append((functools.partial(run_ahead, f, j, hh, m0), 1))
            interleave(mxu, mac_stream(f), NT * NCH * (NCH + 1) // 2)

        def slab_pair(i, carry):
            slab_arrived(2 * i)
            slab_arrived(2 * i + 1)
            slab(2 * i)
            slab(2 * i + 1)
            return carry
        lax.fori_loop(0, HP // 2, slab_pair, 0)

        c_fi.wait()
        c_d.wait()
        dvec = dv[...].astype(F32).reshape(1, Dm)

        def inv(i, carry):
            r0 = pl.multiple_of(i * CH, CH)
            for c in range(NT):
                cs = slice(c * 128, (c + 1) * 128)
                y = jnp.dot(pltpu.bitcast(fi[...], BF16), Ub[i, :, cs].astype(BF16),
                            preferred_element_type=F32)
                yb[pl.ds(r0, CH), cs] = y + ub[pl.ds(r0, CH), cs].astype(F32) * dvec[:, cs]
            return carry
        lax.fori_loop(0, NCH, inv, 0, unroll=4)

        c_bias.wait()
        c_mem0.wait()
        for c in c_wo:
            c.wait()
        c_xb.start()
        MB = M
        XB = seg // 2
        MO = 2 * XB
        hbuf[0, MO:MO + MB // 2, :] = _pack16(mem0[...].astype(F32))
        hbuf[0, 0:XB, :] = _pack16(_ln(x0[0:seg, :].astype(F32)))

        def finish(s, r0):
            x3 = x2buf[s + 1] + ox[seg:2 * seg, :]
            x4 = x3 + _ln(x3) * yb[pl.ds(r0, seg), :]
            ob[pl.ds(r0, seg), :] = x4.astype(BF16)

        def make_step(act1, act2, pre):
            rows = 2 * M + seg * (int(act1) + int(act2))
            b0 = 0 if (act1 and act2) else R if act1 else R + 2 * M + seg
            x1_in_lhs = act1 and not pre

            key = "b" if (act1 and act2 and not pre) else "bp" if (act1 and act2) else "1" if act1 else "2"
            lS, lP, lW, tail = cfg.get("lag_" + key, LAGS[key])

            def step(t, par):
                npar = 1 - par
                parts = []
                if x1_in_lhs:
                    parts.append(hbuf[par, 0:XB, :])
                if act2:
                    parts.append(hbuf[par, XB:2 * XB, :])
                parts.append(hbuf[par, MO:MO + MB, :])
                hh = pltpu.bitcast(parts[0] if len(parts) == 1 else jnp.concatenate(parts, axis=0), BF16)
                zpad = jnp.zeros((128 - rows, Dh), F32)

                def proj(h, j, padded):
                    r = jnp.dot(hh, pltpu.bitcast(wqkv[j, h], BF16), preferred_element_type=F32)
                    blocks = [r]
                    if pre:
                        x1p = qkvx[j, h, pl.ds(pl.multiple_of((t - LAG) * seg, seg), seg), :]
                        blocks = [x1p, r]
                    if padded:
                        blocks.append(zpad)
                    u = blocks[0] if len(blocks) == 1 else jnp.concatenate(blocks, axis=0)
                    return u.astype(BF16)

                def scores(q, k):
                    s = lax.dot_general(q, k, (((1,), (1,)), ((), ())), preferred_element_type=F32)
                    s = s * qk_scale + bias[b0:b0 + rows, :]
                    m = jnp.max(s, axis=-1, keepdims=True)
                    p = jnp.exp2(s - m)
                    l = jnp.sum(p, axis=-1, keepdims=True)
                    r = pl.reciprocal(l, approx=True)
                    r = r * (2.0 - l * r)
                    return (p * r).astype(BF16)

                def pv(p, v):
                    z = jnp.dot(p, v, preferred_element_type=F32)
                    return jnp.concatenate([z[rows - 2 * M:], z[:rows - 2 * M]], axis=0).astype(BF16)

                def wout(h, z):
                    return jnp.dot(z, pltpu.bitcast(wo[h], BF16), preferred_element_type=F32)

                def post1():
                    s = jnp.minimum(jnp.maximum(t - 1, 0), NSEG - 1)
                    r0 = pl.multiple_of(s * seg, seg)
                    x1 = x0[pl.ds(r0, seg), :].astype(F32) + ox[0:seg, :]
                    x2 = x1 + _ln(x1) * yb[pl.ds(r0, seg), :]
                    x2buf[t] = x2
                    hbuf[npar, XB:2 * XB, :] = _pack16(_ln(x2))

                def post2():
                    s = jnp.maximum(t - 1 - LAG, 0)
                    finish(s, pl.multiple_of(s * seg, seg))

                def pre1():
                    s = jnp.minimum(t + 1, NSEG - 1)
                    r0 = pl.multiple_of(s * seg, seg)
                    hbuf[npar, 0:XB, :] = _pack16(_ln(x0[pl.ds(r0, seg), :].astype(F32)))
                extra = {extras[0]: post1}
                if act2:
                    extra[extras[1]] = post2
                if act1:
                    extra[extras[2]] = pre1

                q, k, v, p, z = {}, {}, {}, {}, {}
                s_at = {h: h + lS for h in range(H)}
                p_at = {h: h + lP for h in range(H)}
                w_at = {h: h + lW for h in range(H)}
                for d, extra_lag in enumerate(tail):
                    p_at[H - 1 - d] += extra_lag
                fin = []
                accv = acc.at[0:rows]
                for i in range(max(w_at.values()) + 1):
                    for op in order:
                        if op == 'q' and i < H:
                            q[i] = proj(i, 0, False)
                        if op == 'k' and i < H:
                            k[i] = proj(i, 1, True)
                        if op == 'v' and i < H:
                            v[i] = proj(i, 2, True)
                        for h in range(H):
                            if op == 'S' and s_at[h] == i:
                                p[h] = scores(q.pop(h), k.pop(h))
                            if op == 'P' and p_at[h] == i:
                                z[h] = pv(p.pop(h), v.pop(h))
                            if op == 'W' and w_at[h] == i:
                                r = wout(h, z.pop(h))
                                if h == 0:
                                    accv[...] = r
                                elif h == H - 1:
                                    fin.append(accv[...] + r)
                                else:
                                    accv[...] += r
                    if i in extra:
                        extra[i]()
                assert not (q or k or v or p or z)
                a = fin[0]
                mp = _pack16(a[0:2 * M, :])
                if act2:
                    hbuf[npar, MO:MO + MB, :] = mp
                else:
                    hbuf[npar, MO:MO + MB // 2, :] = mp[0:MB // 2]
                    hbuf[npar, MO + MB // 2:MO + MB, :] = _pack16(mem0[...].astype(F32))
                if act1 and act2:
                    ox[...] = a[2 * M:R, :]
                elif act1:
                    ox[0:seg, :] = a[2 * M:, :]
                else:
                    ox[seg:2 * seg, :] = a[2 * M:, :]
            return step

        def run_steps(t0, t1, step, unroll=1):
            if unroll == 1:
                lax.fori_loop(t0, t1, lambda t, c: step(t, t & 1), None)
                return
            assert unroll % 2 == 0 and (t1 - t0) % unroll == 0

            def body(i, c):
                for u in range(unroll):
                    step(t0 + i * unroll + u, (t0 + u) & 1)
            lax.fori_loop(0, (t1 - t0) // unroll, body, None)

        run_steps(0, LAG, make_step(True, False, False))
        c_xb.wait()
        run_steps(LAG, LAG + NS, make_step(True, True, True))
        run_steps(LAG + NS, NSEG, make_step(True, True, False), unroll=2)
        OA = (NSEG - LAG - 1) * seg
        c_oa = pltpu.make_async_copy(ob.at[pl.ds(0, OA)], o_hbm.at[pl.ds(0, OA)], sem_out.at[0])
        c_oa.start()
        run_steps(NSEG, NSEG + LAG, make_step(False, True, False))
        OB = (NSEG - 1) * seg
        c_ob = pltpu.make_async_copy(ob.at[pl.ds(OA, OB - OA)], o_hbm.at[pl.ds(OA, OB - OA)],
                                     sem_out.at[1])
        c_ob.start()
        finish(NSEG - 1, OB)
        c_oc = pltpu.make_async_copy(ob.at[pl.ds(OB, S - OB)], o_hbm.at[pl.ds(OB, S - OB)],
                                     sem_out.at[2])
        c_oc.start()
        c_oa.wait()
        c_ob.wait()
        c_oc.wait()

    scratch = [
        pltpu.VMEM((3, H, Dm // 2, Dh), U32),
        pltpu.VMEM((3, HP, Dm, Dh), U32),
        pltpu.VMEM((H, Dh // 2, Dm), U32),
        pltpu.VMEM((S, Dm), BF16),
        pltpu.VMEM((KPAD + S, Dm), BF16),
        pltpu.VMEM((S, Dm), BF16),
        pltpu.VMEM((NCH, Dm, CH), BF16),
        pltpu.VMEM((S, Dm), BF16),
        pltpu.VMEM((NCH, 2 * CH, Dm), F32),
        pltpu.VMEM((NCH, 2 * CH, Dm), F32),
        pltpu.VMEM((2 * CH, Dm), F32),
        pltpu.VMEM((S, Dm), F32),
        pltpu.VMEM((2, R // 2, Dm), U32),
        pltpu.VMEM((NS * seg // 2, Dm), U32),
        pltpu.VMEM((3, H, NS * seg, Dh), F32),
        pltpu.VMEM((R, Dm), F32),
        pltpu.VMEM((NSEG + LAG + 1, seg, Dm), F32),
        pltpu.VMEM((2 * seg, Dm), F32),
        pltpu.VMEM((S, Dm), BF16),
        pltpu.VMEM((CH, CH), U32),
        pltpu.VMEM((CH // 2, 2 * CH), U32),
        pltpu.VMEM((R + 2 * (2 * M + seg), 128), F32),
        pltpu.VMEM((M, Dm), BF16),
        pltpu.VMEM((KS, Dm), BF16),
        pltpu.VMEM((Dm,), BF16),
        pltpu.SemaphoreType.DMA((6,)),
        pltpu.SemaphoreType.DMA((NCH,)),
        pltpu.SemaphoreType.DMA((NCH,)),
        pltpu.SemaphoreType.DMA((NCH,)),
        pltpu.SemaphoreType.DMA((3, HP)),
        pltpu.SemaphoreType.DMA((4,)),
        pltpu.SemaphoreType.DMA((2,)),
        pltpu.SemaphoreType.DMA((3,)),
    ]
    return kernel, scratch


def _run(A_x, A_mem0, A_Wq, A_Wk, A_Wv, A_Wo, A_seg_len, B_k, B_v, B_shift_k, B_ssm_k, B_ssm_D,
         cfg=None):
    B, S, Dm = A_x.shape
    assert B == 1
    _, H, Dh = A_Wq.shape
    M = A_mem0.shape[1]
    seg = int(A_seg_len)
    KS = B_shift_k.shape[-1]
    kernel, scratch = _build(S, Dm, H, Dh, M, seg, KS, cfg or {})
    fa_np, fi_np = _dft_mats()
    bias_np = _attn_bias(M, seg)
    args = (A_x.reshape(S, Dm), A_mem0.reshape(M, Dm), A_Wq, A_Wk, A_Wv, A_Wo,
            B_k.reshape(S, Dm), B_v.reshape(S, Dm), B_shift_k.T, B_ssm_k, B_ssm_D,
            fa_np, fi_np, bias_np)
    out = pl.pallas_call(
        kernel,
        out_shape=jax.ShapeDtypeStruct((S, Dm), BF16),
        in_specs=[pl.BlockSpec(memory_space=pl.ANY)] * len(args),
        out_specs=pl.BlockSpec(memory_space=pl.ANY),
        scratch_shapes=scratch,
        compiler_params=pltpu.CompilerParams(vmem_limit_bytes=110 * 1024 * 1024),
    )(*args)
    return out.reshape(B, S, Dm)


@functools.partial(jax.jit, static_argnames=("A_seg_len",))
def pallas_interleave_layers__memory_aug_recurrent_mem_tr__ssm_conv_h3__prompt_kernel(
    A_x: jax.Array,
    A_mem0: jax.Array,
    A_Wq: jax.Array,
    A_Wk: jax.Array,
    A_Wv: jax.Array,
    A_Wo: jax.Array,
    A_seg_len: int,
    B_q: jax.Array,
    B_k: jax.Array,
    B_v: jax.Array,
    B_shift_k: jax.Array,
    B_ssm_k: jax.Array,
    B_ssm_D: jax.Array,
):
    del B_q
    return _run(A_x, A_mem0, A_Wq, A_Wk, A_Wv, A_Wo, A_seg_len, B_k, B_v, B_shift_k,
                B_ssm_k, B_ssm_D)
```
